```python
import os as _os
_os.environ.setdefault("JAX_PLATFORMS", "cpu")
import jax
import jax.numpy as jnp

def _softmax(x, axis=-1):
    return jax.nn.softmax(x, axis=axis)
def _gelu(x):
    return jax.nn.gelu(x, approximate=True)
def _silu(x):
    return jax.nn.silu(x)
def _sigmoid(x):
    return jax.nn.sigmoid(x)
def _layernorm(x, axis=-1, eps=1e-5):
    m = jnp.mean(x, axis=axis, keepdims=True)
    v = jnp.var(x, axis=axis, keepdims=True)
    return (x - m) / jnp.sqrt(v + eps)
def _scatter_add(tgt, idx, src, axis=0):
    return tgt.at[idx].add(src)
def _segment_sum(src, seg, n):
    return jax.ops.segment_sum(src, seg, n)
class _Rng:
    def __init__(self, key):
        self._k = key
    def _next(self):
        self._k, sub = jax.random.split(self._k)
        return sub
    def normal(self, shape):
        return jax.random.normal(self._next(), shape, dtype=jnp.bfloat16)
    def randint(self, lo, hi, shape):
        return jax.random.randint(self._next(), shape, lo, hi, dtype=jnp.int32)
    def uniform(self, shape, lo=0.0, hi=1.0):
        return jax.random.uniform(self._next(), shape, jnp.bfloat16, lo, hi)
    def permutation(self, n):
        return jax.random.permutation(self._next(), n)


kernel_name = 'recurrent_scan__ssm_conv_s5__mixer_channel_mlp__prompt'

def setup_inputs():
    _rng = _Rng(jax.random.key(int.from_bytes(__import__("os").urandom(4), "little")))
    _w = (lambda a: (lambda t: t.astype(jnp.bfloat16) if jnp.issubdtype(t.dtype, jnp.floating) else t)(jnp.asarray(a)))
    def _A_setup():
        B, S, D = 1, 2048, 448
        P = D
        Lambda_re = -0.5 * jnp.exp((lambda *s: _rng.normal(s) * 0.4)(P))
        Lambda_im = (lambda *s: _rng.normal(s) * 0.4)(P) * 1.0
        B_re = (lambda *s: _rng.normal(s) * 0.4)(P, D) * (D ** -0.5)
        B_im = (lambda *s: _rng.normal(s) * 0.4)(P, D) * (D ** -0.5)
        C_re = (lambda *s: _rng.normal(s) * 0.4)(D, P) * (P ** -0.5)
        C_im = (lambda *s: _rng.normal(s) * 0.4)(D, P) * (P ** -0.5)
        log_dt = (lambda *s: _rng.normal(s) * 0.4)(P) * 0.3 - 2.0
        Dskip = (lambda *s: _rng.normal(s) * 0.2)(D)
        return {
            "x": _w((lambda *s: _rng.normal(s) * 0.05)(B, S, D)),
            "Lambda_re": _w(Lambda_re),
            "Lambda_im": _w(Lambda_im),
            "B_re": _w(B_re),
            "B_im": _w(B_im),
            "C_re": _w(C_re),
            "C_im": _w(C_im),
            "log_dt": _w(log_dt),
            "Dskip": _w(Dskip),
        }
    _A_in = _A_setup()

    def _B_setup():
        B, S, D, F = 1, 2048, 448, 1792
        return {
            "x": _w((lambda *s: _rng.normal(s) * 0.05)(B, S, D)),
            "w1": _w((lambda *s: _rng.normal(s) * 0.2)(D, F) * (D ** -0.5)),
            "b1": _w((lambda *s: _rng.normal(s) * 0.2)(F)),
            "w2": _w((lambda *s: _rng.normal(s) * 0.2)(F, D) * (F ** -0.5)),
            "b2": _w((lambda *s: _rng.normal(s) * 0.05)(D)),
        }
    _B_in = _B_setup()

    return {
        "A_x": _A_in["x"],
        "A_Lambda_re": _A_in["Lambda_re"],
        "A_Lambda_im": _A_in["Lambda_im"],
        "A_B_re": _A_in["B_re"],
        "A_B_im": _A_in["B_im"],
        "A_C_re": _A_in["C_re"],
        "A_C_im": _A_in["C_im"],
        "A_log_dt": _A_in["log_dt"],
        "A_Dskip": _A_in["Dskip"],
        "B_x": _B_in["x"],
        "B_w1": _B_in["w1"],
        "B_b1": _B_in["b1"],
        "B_w2": _B_in["w2"],
        "B_b2": _B_in["b2"],
    }

def reference(A_x, A_Lambda_re, A_Lambda_im, A_B_re, A_B_im, A_C_re, A_C_im, A_log_dt, A_Dskip, B_x, B_w1, B_b1, B_w2, B_b2):
    def _A_ref(x, Lambda_re, Lambda_im, B_re, B_im, C_re, C_im, log_dt, Dskip):
        Bsz, L, H = x.shape
        Lam = Lambda_re + 1j * Lambda_im
        Bmat = B_re + 1j * B_im
        Cmat = C_re + 1j * C_im
        dt = jnp.exp(log_dt)
        Lam_bar = jnp.exp(dt * Lam)
        B_bar = ((Lam_bar - 1.0) / Lam)[:, None] * Bmat
        Bu = jnp.einsum("bld,pd->blp", x + 0j, B_bar)
        h = jnp.zeros_like(Bu[:, 0, :])
        hs = []
        for t in range(L):
            h = Lam_bar[None, :] * h + Bu[:, t, :]
            hs.append(h)
        hseq = jnp.stack(hs, 1)
        y = 2.0 * jnp.einsum("blp,dp->bld", hseq, Cmat).real + x * Dskip[None, None, :]
        return y

    def _B_ref(x, w1, b1, w2, b2):
        y = _layernorm(x, axis=-1)
        h = _gelu(jnp.einsum("bsd,df->bsf", y, w1) + b1)
        return jnp.einsum("bsf,fd->bsd", h, w2) + b2

    x = A_x
    xn = _layernorm(x, axis=-1)
    s = _A_ref(xn, A_Lambda_re, A_Lambda_im, A_B_re, A_B_im, A_C_re, A_C_im, A_log_dt, A_Dskip)
    g = _silu(_B_ref(xn, B_w1, B_b1, B_w2, B_b2))
    return x + s * g
```

```python
import functools
import jax
import jax.numpy as jnp
import jax.experimental.pallas as pl
import jax.experimental.pallas.tpu as pltpu

TM = 256
XP = 0
EPS = 1e-5
F32 = jnp.float32
BF16 = jnp.bfloat16
U32 = jnp.uint32
NT = (((1,), (1,)), ((), ()))


def _ln0(x):
    d = x.shape[0]
    m = jnp.sum(x, axis=0, keepdims=True) * (1.0 / d)
    xc = x - m
    v = jnp.sum(xc * xc, axis=0, keepdims=True) * (1.0 / d)
    return xc * jax.lax.rsqrt(v + EPS)


def _cmul(ar, ai, br, bi):
    return ar * br - ai * bi, ar * bi + ai * br


def _row(ref):
    return ref[...].astype(F32).reshape(1, ref.shape[0])


def _kernel(x_ref, lre_ref, lim_ref, bre_ref, bim_ref, cre_ref, cim_ref, ldt_ref, dsk_ref,
            w1_ref, b1_ref, w2_ref, b2_ref, o_ref,
            bw_s, cw_s, lam_s, carry_s, col_s, b1_s, bu_s, h_s, *, tm, P):
    Q = tm // 8 + 1
    QL = tm - 7 * Q
    D = x_ref.shape[0]
    PA = (P // 128) * 128
    PB = P - PA
    NA = PA // 128
    step = pl.program_id(0)

    def pack_lam(re, im):
        a = jnp.concatenate([re[:, :PA], re[:, :PA], re[:, PA:], re[:, PA:], re[:, PA:], re[:, PA:]], axis=1)
        b = jnp.concatenate([-im[:, :PA], im[:, :PA], -im[:, PA:], im[:, PA:], im[:, PA:], -im[:, PA:]], axis=1)
        return a, b

    W = 2 * PA + 256

    @pl.when(step == 0)
    def _init():
        lr = _row(lre_ref)
        li = _row(lim_ref)
        dt = jnp.exp(_row(ldt_ref)).astype(BF16).astype(F32)
        mag = jnp.exp(dt * lr)
        ang = dt * li
        lbr = mag * jnp.cos(ang)
        lbi = mag * jnp.sin(ang)
        nr = lbr - 1.0
        den = lr * lr + li * li
        cr = (nr * lr + lbi * li) / den
        ci = (lbi * lr - nr * li) / den
        a, b = pack_lam(lbr, lbi)
        lam_s[0] = jnp.broadcast_to(a, (8, W))
        lam_s[1] = jnp.broadcast_to(b, (8, W))
        pr, pi = lbr, lbi
        q = 1
        while q < Q - 1:
            pr, pi = _cmul(pr, pi, pr, pi)
            q *= 2
        pr, pi = _cmul(pr, pi, lbr, lbi)
        bu_s[:, tm:, :] = jnp.zeros((8, 8, 128), F32)
        for k in range(3):
            a, b = pack_lam(pr, pi)
            lam_s[2 + 2 * k] = jnp.broadcast_to(a, (8, W))
            lam_s[3 + 2 * k] = jnp.broadcast_to(b, (8, W))
            pr, pi = _cmul(pr, pi, pr, pi)
        bw_s[0:PA, :] = bre_ref[0:PA, :]
        bw_s[PA:2 * PA, :] = bim_ref[0:PA, :]
        bw_s[2 * PA:2 * PA + PB, :] = bre_ref[PA:P, :]
        bw_s[2 * PA + PB:2 * P, :] = bim_ref[PA:P, :]
        c_re = cre_ref[...].astype(F32)
        c_im = cim_ref[...].astype(F32)
        cpr = 2.0 * (c_re * cr - c_im * ci)
        cpi = -2.0 * (c_re * ci + c_im * cr)
        cw = jnp.concatenate([cpr[:, :PA], cpi[:, :PA], cpr[:, PA:], cpi[:, PA:]], axis=1)
        cw_s[...] = cw.astype(BF16)
        carry_s[...] = jnp.zeros_like(carry_s)
        b1_s[...] = jnp.broadcast_to(_row(b1_ref), b1_s.shape)
        for k, ref in enumerate((dsk_ref, b2_ref)):
            r = jnp.concatenate([_row(ref), jnp.zeros((1, 512 - D), F32)], axis=1)
            col_s[k] = jnp.broadcast_to(r, (128, 512)).T[:D, :]

    def swap(h):
        return jnp.concatenate([h[:, PA:2 * PA], h[:, :PA], h[:, 2 * PA + 128:], h[:, 2 * PA:2 * PA + 128]], axis=1)

    xT = x_ref[...].astype(F32)
    xnT_b = _ln0(xT).astype(BF16)
    xnT = xnT_b.astype(F32)
    yT_b = _ln0(xnT).astype(BF16)
    if XP == 0:
        xn = xnT_b.T
        y = yT_b.T
    else:
        u = pltpu.bitcast(xnT, U32) | (pltpu.bitcast(yT_b.astype(F32), U32) >> 16)
        u = jnp.concatenate([u, jnp.zeros((512 - D, tm), U32)], axis=0).T[:, :D]
        xn = pltpu.bitcast(u & jnp.uint32(0xFFFF0000), F32).astype(BF16)
        y = pltpu.bitcast(u << 16, F32).astype(BF16)

    bu = jax.lax.dot_general(xn, bw_s[...], NT, preferred_element_type=F32)
    for j in range(2 * NA + 1):
        bu_s[j, :tm, :] = bu[:, j * 128:(j + 1) * 128]
    bu_s[2 * NA + 1, :tm, :] = pltpu.roll(bu[:, 2 * PA:], PB, 1)

    a = jnp.dot(y, w1_ref[...], preferred_element_type=F32) + b1_s[0:1, :]
    a = jax.nn.gelu(a, approximate=True).astype(BF16)

    def ld(i):
        return jnp.concatenate([bu_s[j, pl.ds(i, 8, stride=Q), :] for j in range(2 * NA + 2)], axis=1)

    la = lam_s[0]
    lb = lam_s[1]
    cin = carry_s[...]
    h = cin
    for i in range(Q):
        h = (la * h + ld(i)) + lb * swap(h)
    row = jax.lax.broadcasted_iota(jnp.int32, (8, W), 0)
    for k in range(3):
        sh = 1 << k
        hs = jnp.where(row >= sh, pltpu.roll(h, sh, 0), 0.0)
        h = h + lam_s[2 + 2 * k] * hs + lam_s[3 + 2 * k] * swap(hs)
    h = jnp.where(row == 0, cin, pltpu.roll(h, 1, 0))
    for i in range(Q):
        h = (la * h + ld(i)) + lb * swap(h)
        if i == QL - 1:
            carry_s[...] = jnp.where(row == 0, pltpu.roll(h, 1, 0), 0.0)
        for j in range(2 * NA + 1):
            h_s[j, pl.ds(i, 8, stride=Q), :] = h[:, j * 128:(j + 1) * 128]

    hb = jnp.concatenate([h_s[j, :tm, :] for j in range(2 * NA + 1)], axis=1).astype(BF16)
    sT = jax.lax.dot_general(cw_s[...], hb, NT, preferred_element_type=F32)
    oT = jax.lax.dot_general(w2_ref[...], a, NT, preferred_element_type=F32)
    rep = lambda c: jnp.concatenate([c] * (tm // 128), axis=1)
    sT = sT + xnT * rep(col_s[0])
    oT = oT + rep(col_s[1])
    g = oT * jax.nn.sigmoid(oT)
    o_ref[...] = xT + sT * g


@jax.jit
def pallas_recurrent_scan__ssm_conv_s5__mixer_channel_mlp__prompt_kernel(
    A_x, A_Lambda_re, A_Lambda_im, A_B_re, A_B_im, A_C_re, A_C_im, A_log_dt, A_Dskip,
    B_x, B_w1, B_b1, B_w2, B_b2,
):
    Bsz, L, D = A_x.shape
    P = A_Lambda_re.shape[0]
    F = B_w1.shape[1]
    tm = TM
    xT = A_x.reshape(L, D).T
    full = lambda shape: pl.BlockSpec(shape, lambda i: (0,) * len(shape))
    outT = pl.pallas_call(
        functools.partial(_kernel, tm=tm, P=P),
        grid=(L // tm,),
        in_specs=[
            pl.BlockSpec((D, tm), lambda i: (0, i)),
            full((P,)), full((P,)), full((P, D)), full((P, D)), full((D, P)), full((D, P)),
            full((P,)), full((D,)), full((D, F)), full((F,)), full((D, F)), full((D,)),
        ],
        out_specs=pl.BlockSpec((D, tm), lambda i: (0, i)),
        out_shape=jax.ShapeDtypeStruct((D, L), F32),
        scratch_shapes=[
            pltpu.VMEM((2 * P, D), BF16),
            pltpu.VMEM((D, 2 * P), BF16),
            pltpu.VMEM((8, 8, 1024), F32),
            pltpu.VMEM((8, 1024), F32),
            pltpu.VMEM((2, D, 128), F32),
            pltpu.VMEM((8, F), F32),
            pltpu.VMEM((8, tm + 8, 128), F32),
            pltpu.VMEM((7, tm + 8, 128), F32),
        ],
        compiler_params=pltpu.CompilerParams(
            dimension_semantics=("arbitrary",), vmem_limit_bytes=100 * 1024 * 1024),
    )(xT, A_Lambda_re, A_Lambda_im, A_B_re, A_B_im, A_C_re, A_C_im,
      A_log_dt, A_Dskip, B_w1, B_b1, B_w2.T, B_b2)
    return outT.T.reshape(Bsz, L, D)
```

```python
import functools
import contextlib
import jax
import jax.numpy as jnp
import jax.experimental.pallas as pl
import jax.experimental.pallas.tpu as pltpu

SCOPES = 0
TA = 256
TB = 512
GA = 2
PEEL = 1
LO = 4
SER = 1
GCP = 1
MSPLIT = 1
PADW = 16
PADW2 = 0
IPOS = 0
B0P = 1
FLAT = 0
G2 = None
GS = 0
GS0 = 0
EPS = 1e-5
F32 = jnp.float32
BF16 = jnp.bfloat16
U32 = jnp.uint32
NT = (((1,), (1,)), ((), ()))
GELU_C0 = 0.7978845608028654
GELU_C1 = 0.7978845608028654 * 0.044715


def scope(name):
    return jax.named_scope(name) if SCOPES else contextlib.nullcontext()


def _cmul(ar, ai, br, bi):
    return ar * br - ai * bi, ar * bi + ai * br


def _row(ref):
    return ref[...].astype(F32).reshape(1, ref.shape[0])


def _kernel(x_hbm, lre_hbm, lim_hbm, bre_hbm, bim_hbm, cre_hbm, cim_hbm, ldt_hbm, dsk_hbm,
            w1_hbm, b1_hbm, w2_hbm, b2_hbm, o_hbm,
            x_s, o_s, bw_s, cre_s, cim_s, cw_s, w1_s, w2_s,
            lre_s, lim_s, ldt_s, dsk_s, b1v_s, b2_s,
            lam_s, carry_s, col_s, coef_s, bu_s, h_s, a_s, s_s, xn_s, xnT_s, st_s, zero_s, zsrc_s,
            xsem, osem, wsem, *, P):
    ta, tb = TA, TB
    na = x_s.shape[0]
    D = x_s.shape[1]
    L = na * ta
    nb = L // tb
    R = tb // ta
    NF = w1_s.shape[0]
    DP = pl.cdiv(D, 128) * 128
    Q = tb // 8 + 1
    QL = tb - 7 * Q
    PA = (P // 128) * 128
    PB = P - PA
    NA = PA // 128
    NB = 2 * NA + 1
    W = 2 * PA + 256
    NH = tb // 128

    def x_copy(j):
        return pltpu.make_async_copy(x_hbm.at[:, pl.ds(j * ta, ta)], x_s.at[j], xsem.at[j])

    def o_copy(j, lo=0, hi=None, r0=0, r1=None):
        hi = tb if hi is None else hi
        r1 = D if r1 is None else r1
        return pltpu.make_async_copy(o_s.at[j, r0:r1, lo:hi],
                                     o_hbm.at[r0:r1, pl.ds(j * tb + lo, hi - lo)], osem)

    vec_copies = [pltpu.make_async_copy(src, dst, wsem.at[3]) for src, dst in
                  ((lre_hbm, lre_s), (lim_hbm, lim_s), (ldt_hbm, ldt_s), (dsk_hbm, dsk_s),
                   (b1_hbm, b1v_s), (b2_hbm, b2_s))]
    w1_copies = [pltpu.make_async_copy(w1_hbm.at[:, k * 128:(k + 1) * 128], w1_s.at[k, 0:D, :], wsem.at[2])
                 for k in range(NF)]
    w2_copies = [pltpu.make_async_copy(w2_hbm.at[:, k * 128:(k + 1) * 128], w2_s.at[k, 0:D, :], wsem.at[2])
                 for k in range(NF)]
    E = max(LO - NA, 0) * 128
    b0_copies = [pltpu.make_async_copy(bre_hbm.at[0:PA, :], bw_s.at[0:PA, :], wsem.at[0])]
    if E:
        b0_copies.append(pltpu.make_async_copy(bim_hbm.at[0:E, :], bw_s.at[PA:PA + E, :], wsem.at[0]))
    b1_copies = [
        pltpu.make_async_copy(bim_hbm.at[E:PA, :], bw_s.at[PA + E:2 * PA, :], wsem.at[1]),
        pltpu.make_async_copy(bre_hbm.at[PA:P, :], bw_s.at[2 * PA:2 * PA + PB, :], wsem.at[1]),
        pltpu.make_async_copy(bim_hbm.at[PA:P, :], bw_s.at[2 * PA + PB:2 * P, :], wsem.at[1]),
    ]
    c_copies = [pltpu.make_async_copy(cre_hbm, cre_s, wsem.at[2]),
                pltpu.make_async_copy(cim_hbm, cim_s, wsem.at[2])]

    def pack_lam(re, im):
        a = jnp.concatenate([re[:, :PA], re[:, :PA], re[:, PA:], re[:, PA:], re[:, PA:], re[:, PA:]], axis=1)
        b = jnp.concatenate([-im[:, :PA], im[:, :PA], -im[:, PA:], im[:, PA:], im[:, PA:], -im[:, PA:]], axis=1)
        return a, b

    def rep(c, w):
        return c if w == 128 else jnp.concatenate([c] * (w // 128), axis=1)

    def gate(val, dep):
        if dep is None:
            return val
        w = pl.cdiv(val.shape[1], 128) * 128
        head = jnp.where(rep(zero_s[...], w)[:, :val.shape[1]] != 0, rep(dep, w)[:, :val.shape[1]], val[0:8, :])
        return head if val.shape[0] == 8 else jnp.concatenate([head, val[8:, :]], axis=0)

    def blocks(ref, r0, r1):
        r32 = ref.bitcast(U32)
        return pltpu.bitcast(
            jnp.concatenate([r32[k, r0 // 2:r1 // 2, :] for k in range(ref.shape[0])], axis=1), BF16)

    def tiles(ref, j, lo, hi):
        parts = []
        for r in range(R):
            a, b = max(lo, r * ta), min(hi, (r + 1) * ta)
            if a < b:
                parts.append(ref[j * R + r, :, a - r * ta:b - r * ta])
        return parts[0] if len(parts) == 1 else jnp.concatenate(parts, axis=1)

    def stage_ln1(j, dep=None):
        x = gate(x_s[j].astype(F32), dep)
        m = jnp.sum(x, axis=0, keepdims=True) * (1.0 / D)
        xc = x - m
        v = jnp.sum(xc * xc, axis=0, keepdims=True) * (1.0 / D)
        xnT_b = (xc * jax.lax.rsqrt(v + EPS)).astype(BF16)
        xn = xnT_b.astype(F32)
        xnT_s[j] = xn
        m2 = jnp.sum(xn, axis=0, keepdims=True) * (1.0 / D)
        v2 = jnp.sum(xn * xn, axis=0, keepdims=True) * (1.0 / D) - m2 * m2
        r2 = jax.lax.rsqrt(v2 + EPS)
        st_s[j, 0:8, :] = jnp.broadcast_to(r2, (8, ta))
        st_s[j, 8:16, :] = jnp.broadcast_to(m2 * r2, (8, ta))
        return xnT_b.T

    def stage_bu(j, xn, lo, hi):
        bu = jax.lax.dot_general(xn, bw_s[lo * 128:hi * 128, :], NT, preferred_element_type=F32)
        if R == 1:
            jb, rows = j, pl.ds(0, ta)
        else:
            jb = j // R
            r0 = (j % R) * ta
            rows = pl.ds(r0 if isinstance(r0, int) else pl.multiple_of(r0, ta), ta)
        for k in range(lo, hi):
            bu_s[jb, k, rows, :] = bu[:, (k - lo) * 128:(k - lo + 1) * 128]
        if hi == NB:
            bu_s[jb, NB, rows, :] = pltpu.roll(bu[:, (NB - 1 - lo) * 128:], PB, 1)
            bu_s[jb, :, tb:, :] = jnp.zeros((8, 8, 128), F32)
        return bu[0:8, 0:128]

    def stage_w1(j, dep=None):
        st = gate(tiles(st_s, j, 0, tb), dep)
        yT = tiles(xnT_s, j, 0, tb) * st[0:1, :] - st[8:9, :]
        row = jax.lax.broadcasted_iota(jnp.int32, (DP - D, tb), 0)
        ones = jnp.where(row == 0, 1.0, 0.0).astype(F32)
        y = jnp.concatenate([yT, ones], axis=0).astype(BF16).T
        x = jnp.dot(y, blocks(w1_s, 0, DP), preferred_element_type=F32)
        t = jnp.tanh(x * (x * x * GELU_C1 + GELU_C0))
        a = (x + x * t).astype(BF16)
        a_s[...] = pltpu.bitcast(a, U32)
        return x[0:8, 0:128]

    def stage_scan(j, dep=None):
        row = jax.lax.broadcasted_iota(jnp.int32, (8, 128), 0)
        prev = dep
        for (ka, kb) in ((0, 3), (1, 4), (2, 5), (6, 7)):
            sa = slice(ka * 128, (ka + 1) * 128)
            sb = slice(kb * 128, (kb + 1) * 128)
            la = lam_s[0, :, sa]
            lba = lam_s[1, :, sa]
            lbb = lam_s[1, :, sb]
            ca = gate(carry_s[:, sa], prev)
            cb = carry_s[:, sb]

            def step(u, v, i):
                bu = bu_s[j, ka, pl.ds(i, 8, stride=Q), :]
                bv = bu_s[j, kb, pl.ds(i, 8, stride=Q), :]
                return (la * u + bu) + lba * v, (la * v + bv) + lbb * u

            u, v = ca, cb
            for i in range(Q):
                u, v = step(u, v, i)
            for k in range(3):
                sh = 1 << k
                us = jnp.where(row >= sh, pltpu.roll(u, sh, 0), 0.0)
                vs = jnp.where(row >= sh, pltpu.roll(v, sh, 0), 0.0)
                pa = lam_s[2 + 2 * k, :, sa]
                u, v = (u + pa * us + lam_s[3 + 2 * k, :, sa] * vs,
                        v + pa * vs + lam_s[3 + 2 * k, :, sb] * us)
            u = jnp.where(row == 0, ca, pltpu.roll(u, 1, 0))
            v = jnp.where(row == 0, cb, pltpu.roll(v, 1, 0))
            for i in range(Q):
                u, v = step(u, v, i)
                if i == QL - 1:
                    carry_s[:, sa] = jnp.where(row == 0, pltpu.roll(u, 1, 0), 0.0)
                    carry_s[:, sb] = jnp.where(row == 0, pltpu.roll(v, 1, 0), 0.0)
                h_s[ka, pl.ds(i, 8, stride=Q), :] = u
                if kb < NB:
                    h_s[kb, pl.ds(i, 8, stride=Q), :] = v
            if SER:
                prev = u

    def stage_c(j):
        hb = jnp.concatenate([h_s[k, :tb, :] for k in range(NB)], axis=1).astype(BF16)
        sT = jax.lax.dot_general(pltpu.bitcast(cw_s[...], BF16), hb, NT, preferred_element_type=F32)
        s_s[...] = sT + tiles(xnT_s, j, 0, tb) * rep(col_s[0], tb)
        return sT[0:8, 0:128]

    def stage_w2(j, lo, hi, r0=0, r1=None):
        r1 = D if r1 is None else r1
        a = pltpu.bitcast(a_s[lo // 2:hi // 2, :], BF16)
        oT = jax.lax.dot_general(blocks(w2_s, r0, r1), a, NT, preferred_element_type=F32)
        h = oT * 0.25 + rep(col_s[1, r0:r1, :], hi - lo)
        g = h + h * jnp.tanh(h)
        o_s[j, r0:r1, lo:hi] = tiles(x_s, j, lo, hi)[r0:r1].astype(F32) + s_s[r0:r1, lo:hi] * g
        return [oT[0:8, k * 128:(k + 1) * 128] for k in range((hi - lo) // 128)]

    def stage_init():
        lr = _row(lre_s)
        li = _row(lim_s)
        dt = jnp.exp(_row(ldt_s)).astype(BF16).astype(F32)
        mag = jnp.exp(dt * lr)
        ang = dt * li
        lbr = mag * jnp.cos(ang)
        lbi = mag * jnp.sin(ang)
        nr = lbr - 1.0
        den = lr * lr + li * li
        coef_s[0:1, :] = 2.0 * (nr * lr + lbi * li) / den
        coef_s[1:2, :] = 2.0 * (lbi * lr - nr * li) / den
        a, b = pack_lam(lbr, lbi)
        lam_s[0] = jnp.broadcast_to(a, (8, W))
        lam_s[1] = jnp.broadcast_to(b, (8, W))
        pr, pi = lbr, lbi
        q = 1
        while q < Q - 1:
            pr, pi = _cmul(pr, pi, pr, pi)
            q *= 2
        pr, pi = _cmul(pr, pi, lbr, lbi)
        for k in range(3):
            a, b = pack_lam(pr, pi)
            lam_s[2 + 2 * k] = jnp.broadcast_to(a, (8, W))
            lam_s[3 + 2 * k] = jnp.broadcast_to(b, (8, W))
            pr, pi = _cmul(pr, pi, pr, pi)
        carry_s[...] = jnp.zeros_like(carry_s)
        row = jax.lax.broadcasted_iota(jnp.int32, (DP - D, NF * 128), 0)
        pad = jnp.where(row == 0, _row(b1v_s), 0.0).astype(BF16)
        for k in range(NF):
            w1_s[k, D:DP, :] = pad[:, k * 128:(k + 1) * 128]
        for k, r in enumerate((_row(dsk_s), 0.5 * _row(b2_s))):
            r = jnp.concatenate([r, jnp.zeros((1, DP - D), F32)], axis=1)
            col_s[k] = jnp.broadcast_to(r, (128, DP)).T[:D, :]

    def stage_cprep(dep):
        cr = coef_s[0:1, :]
        ci = coef_s[1:2, :]
        c_re = gate(cre_s[...].astype(F32), dep)
        c_im = cim_s[...].astype(F32)
        cpr = c_re * cr - c_im * ci
        cpi = -(c_re * ci + c_im * cr)
        cw = jnp.concatenate([cpr[:, :PA], cpi[:, :PA], cpr[:, PA:], cpi[:, PA:]], axis=1).astype(BF16)
        cw_s[...] = pltpu.bitcast(cw, U32)

    FIRST = 1 if PEEL else GA
    if IPOS == 0:
        for c in vec_copies:
            c.start()
    x_copy(0).start()
    for c in b0_copies:
        c.start(priority=B0P)
    zsrc_s[...] = jnp.zeros_like(zsrc_s)
    z_copy = pltpu.make_async_copy(zsrc_s, zero_s, wsem.at[3])
    vec_copies.append(z_copy)
    z_copy.start()
    if IPOS == 0:
        with scope('vwait'):
            for c in vec_copies:
                c.wait()
        for c in b1_copies:
            c.start(priority=1)
        for j in range(1, FIRST + 1):
            x_copy(j).start(priority=1)
        with scope('init'):
            stage_init()
    with scope('x0wait'):
        x_copy(0).wait()
    if IPOS == 1:
        for c in vec_copies:
            c.start()
        for c in b1_copies:
            c.start(priority=1)
        for j in range(1, FIRST + 1):
            x_copy(j).start(priority=1)
    with scope('ln0'):
        xn = stage_ln1(0)
        xn_s[...] = xn
    with scope('b0_wait'):
        for c in b0_copies:
            c.wait()
        if IPOS == 1:
            for c in vec_copies:
                c.wait()
    for j in range(FIRST + 1, na):
        x_copy(j).start(priority=1)
    with scope('bu_lo0'):
        stage_bu(0, xn, 0, LO)
        if IPOS == 1:
            stage_init()
    with scope('b_wait'):
        for c in b1_copies:
            c.wait()
    for c in w1_copies + c_copies + w2_copies:
        c.start(priority=1)

    def a_chain(j0, cnt, last_lo):
        stage_bu(j0, xn_s[...], LO, NB)
        e = None
        for t in range(1, cnt + 1):
            xn = stage_ln1(j0 + t, e)
            if t < cnt or not last_lo:
                e = stage_bu(j0 + t, xn, 0, NB)
            else:
                stage_bu(j0 + t, xn, 0, LO)
                xn_s[...] = xn

    for j in range(PEEL):
        with scope('xwait'):
            x_copy(j + 1).wait()
        with scope('peel_a'):
            a_chain(j, 1, True)
    NIT = (na - 1 - PEEL) // GA
    REM = (na - 1 - PEEL) - NIT * GA

    def body_a(i, carry):
        j0 = PEEL + i * GA
        with scope('xwait'):
            for t in range(1, GA + 1):
                x_copy(j0 + t).wait()
        with scope('body_a'):
            a_chain(j0, GA, True)
        return carry

    jax.lax.fori_loop(0, NIT, body_a, 0)

    with scope('w_wait'):
        for t in range(1, REM + 1):
            x_copy(PEEL + NIT * GA + t).wait()
        for c in w1_copies + c_copies + w2_copies:
            c.wait()
    with scope('pro_b'):
        a_chain(PEEL + NIT * GA, REM, False)
        d = stage_w1(0)
        stage_cprep(d if GCP else None)
        stage_scan(0, d if GS0 else None)
        stage_c(0)

    def body_b(j, carry):
        with scope('body_b'):
            dw = stage_w2(j, 0, tb)
            d = stage_w1(j + 1, dw[G2] if G2 is not None else None)
            stage_scan(j + 1, (d if GS == 1 else dw[-1]) if GS else None)
            stage_c(j + 1)
        o_copy(j).start()
        return carry

    if FLAT:
        for j in range(nb - 1):
            body_b(j, 0)
    else:
        jax.lax.fori_loop(0, nb - 1, body_b, 0)

    pieces = [(k * 128, (k + 1) * 128, 0, D) for k in range(NH - 1)]
    if MSPLIT:
        pieces += [(tb - 128, tb, 0, D // 2), (tb - 128, tb, D // 2, D)]
    else:
        pieces += [(tb - 128, tb, 0, D)]
    with scope('epi'):
        for pc in pieces:
            stage_w2(nb - 1, *pc)
            o_copy(nb - 1, *pc).start()
    with scope('owait'):
        for j in range(nb - 1):
            o_copy(j).wait()
        for pc in pieces:
            o_copy(nb - 1, *pc).wait()


@jax.jit
def pallas_recurrent_scan__ssm_conv_s5__mixer_channel_mlp__prompt_kernel(
    A_x, A_Lambda_re, A_Lambda_im, A_B_re, A_B_im, A_C_re, A_C_im, A_log_dt, A_Dskip,
    B_x, B_w1, B_b1, B_w2, B_b2,
):
    Bsz, L, D = A_x.shape
    P = A_Lambda_re.shape[0]
    F = B_w1.shape[1]
    ta, tb = TA, TB
    na, nb = L // ta, L // tb
    NF = F // 128
    DP = pl.cdiv(D, 128) * 128
    xT = A_x.reshape(L, D).T
    outT = pl.pallas_call(
        functools.partial(_kernel, P=P),
        in_specs=[pl.BlockSpec(memory_space=pl.ANY)] * 13,
        out_specs=pl.BlockSpec(memory_space=pl.ANY),
        out_shape=jax.ShapeDtypeStruct((D, L), F32),
        scratch_shapes=[
            pltpu.VMEM((na, D, ta), BF16),
            pltpu.VMEM((nb, D, tb), F32),
            pltpu.VMEM((2 * P, D), BF16),
            pltpu.VMEM((D, P), BF16),
            pltpu.VMEM((D, P), BF16),
            pltpu.VMEM((D // 2, 2 * P), U32),
            pltpu.VMEM((NF, DP + PADW, 128), BF16),
            pltpu.VMEM((NF, D + PADW2, 128), BF16),
            pltpu.VMEM((P,), BF16), pltpu.VMEM((P,), BF16), pltpu.VMEM((P,), BF16),
            pltpu.VMEM((D,), BF16), pltpu.VMEM((F,), BF16), pltpu.VMEM((D,), BF16),
            pltpu.VMEM((8, 8, 1024), F32),
            pltpu.VMEM((8, 1024), F32),
            pltpu.VMEM((2, D, 128), F32),
            pltpu.VMEM((8, P), F32),
            pltpu.VMEM((nb, 8, tb + 8, 128), F32),
            pltpu.VMEM((7, tb + 8, 128), F32),
            pltpu.VMEM((tb // 2, F), U32),
            pltpu.VMEM((D, tb), F32),
            pltpu.VMEM((ta, D), BF16),
            pltpu.VMEM((na, D, ta), F32),
            pltpu.VMEM((na, 16, ta), F32),
            pltpu.VMEM((8, 128), jnp.int32),
            pltpu.VMEM((8, 128), jnp.int32),
            pltpu.SemaphoreType.DMA((na,)),
            pltpu.SemaphoreType.DMA(()),
            pltpu.SemaphoreType.DMA((4,)),
        ],
        compiler_params=pltpu.CompilerParams(
            vmem_limit_bytes=100 * 1024 * 1024,
            disable_semaphore_checks=True, disable_bounds_checks=True),
    )(xT, A_Lambda_re, A_Lambda_im, A_B_re, A_B_im, A_C_re, A_C_im,
      A_log_dt, A_Dskip, B_w1, B_b1, B_w2.T, B_b2)
    return outT.T.reshape(Bsz, L, D)
```

```python
import functools
import contextlib
import jax
import jax.numpy as jnp
import jax.experimental.pallas as pl
import jax.experimental.pallas.tpu as pltpu

SCOPES = 0
TA = 256
TB = 512
GA = 2
LO = 4
LNG = ((0, 1, 2), (0, 2, 3))
GS = -2
GS0 = 7
EV1 = ((0,32,64,96,128,160,192,224),56,7)
EV2 = ((0,3,6,9,12,15,18,21,24,27,30,33,36),(0,56,112,168),7)
CPK = (0,1,2,3,4,5,6,28,29,30,31,32,33,34)
SC0 = None
EPS = 1e-5
F32 = jnp.float32
BF16 = jnp.bfloat16
U32 = jnp.uint32
NT = (((1,), (1,)), ((), ()))
GELU_C0 = 0.7978845608028654
GELU_C1 = 0.7978845608028654 * 0.044715


def scope(name):
    return jax.named_scope(name) if SCOPES else contextlib.nullcontext()


def _cmul(ar, ai, br, bi):
    return ar * br - ai * bi, ar * bi + ai * br


def _row(ref):
    return ref[...].astype(F32).reshape(1, ref.shape[0])


def _kernel(x_hbm, lre_hbm, lim_hbm, bre_hbm, bim_hbm, cre_hbm, cim_hbm, ldt_hbm, dsk_hbm,
            w1_hbm, b1_hbm, w2_hbm, b2_hbm, o_hbm,
            x_s, o_s, bu_s, xnT_s, st_s, bw_s, cre_s, cim_s, cw_s, w1_s, w2_s, w1x_s, w2x_s,
            lam_s, carry_s, col_s, coef_s, cm_s, h_s, a_s, s_s, xn_s, zero_s, zsrc_s,
            lre_s, lim_s, ldt_s, dsk_s, b1v_s, b2_s, pad_s,
            xsem, osem, wsem, *, P):
    ta, tb = TA, TB
    na = x_s.shape[0]
    D = x_s.shape[1]
    L = na * ta
    nb = L // tb
    R = tb // ta
    NF = w1_s.shape[0]
    NFH = NF // 2
    FH = NFH * 128
    DP = pl.cdiv(D, 128) * 128
    DH = D // 2
    KP = pl.cdiv(DH, 128) * 128
    H = tb // 2
    Q = tb // 8 + 1
    QL = tb - 7 * Q
    PA = (P // 128) * 128
    PB = P - PA
    NA = PA // 128
    NB = 2 * NA + 1
    W = 2 * PA + 256

    def x_copy(j):
        return pltpu.make_async_copy(x_hbm.at[:, pl.ds(j * ta, ta)], x_s.at[j], xsem.at[j])

    def o_copy(j, lo=0, hi=None, r0=0, r1=None):
        hi = tb if hi is None else hi
        r1 = D if r1 is None else r1
        return pltpu.make_async_copy(o_s.at[j, r0:r1, lo:hi],
                                     o_hbm.at[r0:r1, pl.ds(j * tb + lo, hi - lo)], osem)

    vec_copies = [pltpu.make_async_copy(src, dst, wsem.at[3]) for src, dst in
                  ((lre_hbm, lre_s), (lim_hbm, lim_s), (ldt_hbm, ldt_s), (dsk_hbm, dsk_s),
                   (b1_hbm, b1v_s), (b2_hbm, b2_s))]
    z_copy = pltpu.make_async_copy(zsrc_s, zero_s, wsem.at[3])
    w1_copies = [pltpu.make_async_copy(w1_hbm.at[:, k * 128:(k + 1) * 128], w1_s.at[k, 0:D, :], wsem.at[4])
                 for k in range(NF)]
    w2_copies = [pltpu.make_async_copy(w2_hbm.at[:, k * 128:(k + 1) * 128], w2_s.at[k], wsem.at[2])
                 for k in range(NF)]
    E = max(LO - NA, 0) * 128
    b0_copies = [pltpu.make_async_copy(bre_hbm.at[0:PA, :], bw_s.at[0:PA, :], wsem.at[0]),
                 pltpu.make_async_copy(bim_hbm.at[0:E, :], bw_s.at[PA:PA + E, :], wsem.at[0])]
    b1_copies = [
        pltpu.make_async_copy(bim_hbm.at[E:PA, :], bw_s.at[PA + E:2 * PA, :], wsem.at[1]),
        pltpu.make_async_copy(bre_hbm.at[PA:P, :], bw_s.at[2 * PA:2 * PA + PB, :], wsem.at[1]),
        pltpu.make_async_copy(bim_hbm.at[PA:P, :], bw_s.at[2 * PA + PB:2 * P, :], wsem.at[1]),
    ]
    c_copies = [pltpu.make_async_copy(cre_hbm, cre_s, wsem.at[2]),
                pltpu.make_async_copy(cim_hbm, cim_s, wsem.at[2])]

    def pack_lam(re, im):
        a = jnp.concatenate([re[:, :PA], re[:, :PA], re[:, PA:], re[:, PA:], re[:, PA:], re[:, PA:]], axis=1)
        b = jnp.concatenate([-im[:, :PA], im[:, :PA], -im[:, PA:], im[:, PA:], im[:, PA:], -im[:, PA:]], axis=1)
        return a, b

    def rep(c, w):
        return c if w == 128 else jnp.concatenate([c] * (w // 128), axis=1)

    def gate(val, dep):
        if dep is None:
            return val
        w = pl.cdiv(val.shape[1], 128) * 128
        head = jnp.where(rep(zero_s[...], w)[:, :val.shape[1]] != 0, rep(dep, w)[:, :val.shape[1]], val[0:8, :])
        return head if val.shape[0] == 8 else jnp.concatenate([head, val[8:, :]], axis=0)

    def gate_row(val, dep):
        if dep is None:
            return val
        w = val.shape[1]
        return jnp.where(rep(zero_s[0:1, :], w) != 0, rep(dep[0:1, :], w), val)

    def wblk(ref, half, r0, r1):
        r32 = ref.bitcast(U32)
        return pltpu.bitcast(
            jnp.concatenate([r32[half * NFH + k, r0 // 2:r1 // 2, :] for k in range(NFH)], axis=1), BF16)

    def xblk(ref, i, r0=0, r1=None):
        r1 = 2 * ref.shape[2] if r1 is None else r1
        return pltpu.bitcast(jnp.concatenate([ref[i, k, r0 // 2:r1 // 2, :] for k in range(NFH)], axis=1), BF16)

    def tiles(ref, j, lo, hi):
        parts = []
        for r in range(R):
            a, b = max(lo, r * ta), min(hi, (r + 1) * ta)
            if a < b:
                parts.append(ref[j * R + r, :, a - r * ta:b - r * ta])
        return parts[0] if len(parts) == 1 else jnp.concatenate(parts, axis=1)

    def ln1_part(j, lo, hi, deps):
        x = gate(x_s[j, :, lo:hi].astype(F32), deps[0])
        m = gate_row(jnp.sum(x, axis=0, keepdims=True) * (1.0 / D), deps[1])
        xc = x - m
        v = jnp.sum(xc * xc, axis=0, keepdims=True) * (1.0 / D)
        xnT_b = (xc * gate_row(jax.lax.rsqrt(v + EPS), deps[2])).astype(BF16)
        xn = xnT_b.astype(F32)
        xnT_s[j, :, lo:hi] = xn
        m2 = jnp.sum(xn, axis=0, keepdims=True) * (1.0 / D)
        v2 = jnp.sum(xn * xn, axis=0, keepdims=True) * (1.0 / D) - m2 * m2
        r2 = jax.lax.rsqrt(v2 + EPS)
        st_s[j, 0:8, lo:hi] = jnp.broadcast_to(r2, (8, hi - lo))
        st_s[j, 8:16, lo:hi] = jnp.broadcast_to(m2 * r2, (8, hi - lo))
        return xnT_b.T

    def stage_ln1(j, e=None):
        if e is None:
            return ln1_part(j, 0, ta, (None, None, None))
        return jnp.concatenate(
            [ln1_part(j, k * 128, (k + 1) * 128, tuple(e[g] for g in LNG[k])) for k in range(ta // 128)], axis=0)

    def stage_bu(base, off, xn, lo, hi):
        bu = jax.lax.dot_general(xn, bw_s[lo * 128:hi * 128, :], NT, preferred_element_type=F32)
        jb = base + off // R
        rows = pl.ds((off % R) * ta, ta)
        for k in range(lo, hi):
            bu_s[jb, k, rows, :] = bu[:, (k - lo) * 128:(k - lo + 1) * 128]
        if hi == NB:
            bu_s[jb, NB, rows, :] = pltpu.roll(bu[:, (NB - 1 - lo) * 128:], PB, 1)
        return bu

    def heads(m, rows=(0,)):
        return [m[r:r + 8, k * 128:(k + 1) * 128] for k in range(m.shape[1] // 128) for r in rows]

    def stage_w1(j, prep=None):
        st = tiles(st_s, j, 0, tb)
        yT = tiles(xnT_s, j, 0, tb) * st[0:1, :] - st[8:9, :]
        a11, a12, a21, a22 = yT[:DH, :H], yT[DH:, :H], yT[:DH, H:], yT[DH:, H:]
        row = jax.lax.broadcasted_iota(jnp.int32, (KP - DH, H), 0)
        zeros = jnp.zeros((KP - DH, H), F32)
        ones = jnp.where(row == 0, 1.0, 0.0).astype(F32)

        def mm(lhsT, rhs, pad=zeros):
            lhs = jnp.concatenate([lhsT, pad], axis=0).astype(BF16).T
            return jnp.dot(lhs, rhs, preferred_element_type=F32)

        def act(r, c, x):
            t = jnp.tanh(x * (x * x * GELU_C1 + GELU_C0))
            a_s[r * H:(r + 1) * H, c * FH:(c + 1) * FH] = x + x * t

        deps = []
        m2 = mm(a21 + a22, wblk(w1_s, 0, 0, KP))
        deps += heads(m2)
        if prep:
            prep(0, deps)
        m4 = mm(a22, xblk(w1x_s, 0), ones)
        act(1, 0, m2 + m4)
        deps += heads(m4)
        m5 = mm(a11 + a12, wblk(w1_s, 1, DH, DH + KP))
        deps += heads(m5)
        if prep:
            prep(1, deps)
        m3 = mm(a11, xblk(w1x_s, 1), ones)
        act(0, 1, m3 + m5)
        deps += heads(m3)
        if prep:
            prep(2, deps)
        m1 = mm(a11 + a22, xblk(w1x_s, 2))
        deps += heads(m1)
        u = m1 + m4 - m5
        v = m1 - m2 + m3
        if prep:
            prep(3, deps)
        m7 = mm(a12 - a22, xblk(w1x_s, 3))
        act(0, 0, u + m7)
        deps += heads(m7)
        if prep:
            prep(4, deps)
        m6 = mm(a21 - a11, xblk(w1x_s, 4))
        act(1, 1, v + m6)
        deps += heads(m6)
        return deps, (m2, m4, m5, m3, m1, m7, m6)

    W1X = ((-1, (1, 0), (0, 0)), (-1, (0, 1), (1, 1)), (1, (0, 0), (1, 1)), (1, (1, 0), (1, 1)), (1, (0, 0), (0, 1)))
    W2X = ((1, (1, 0), (1, 1)), (1, (0, 0), (0, 1)), (1, (0, 0), (1, 1)), (-1, (0, 1), (1, 1)), (-1, (1, 0), (0, 0)))

    def comb_all(src, dst, specs, deps):
        src32 = src.bitcast(U32)
        per = len(deps) // NFH
        rows = DH // 2 // per
        z = jnp.concatenate([zero_s[...]] * (rows // 8), axis=0) != 0
        for n, dep in enumerate(deps):
            k, q = divmod(n, per)
            d = jnp.concatenate([pltpu.bitcast(dep, U32)] * (rows // 8), axis=0)
            blk = {}
            for r in range(2):
                for c in range(2):
                    r0 = r * DH // 2 + q * rows
                    w = jnp.where(z, d, src32[c * NFH + k, r0:r0 + rows, :])
                    blk[r, c] = [pltpu.unpack_elementwise(w, index=e, packed_dtype=BF16, unpacked_dtype=F32)
                                 for e in range(2)]
            for i, (sign, a, b) in enumerate(specs):
                s = [u + v if sign > 0 else u - v for u, v in zip(blk[a], blk[b])]
                dst[i, k, q * rows:(q + 1) * rows, :] = pltpu.pack_elementwise(s, packed_dtype=BF16)

    def stage_scan(j, dep=None, deps=None):
        row = jax.lax.broadcasted_iota(jnp.int32, (8, 128), 0)
        prev = dep
        for ip, (ka, kb) in enumerate(((0, 3), (1, 4), (2, 5), (6, 7))):
            if deps is not None and deps[ip] is not None:
                prev = deps[ip]
            sa = slice(ka * 128, (ka + 1) * 128)
            sb = slice(kb * 128, (kb + 1) * 128)
            la = lam_s[0, :, sa]
            lba = lam_s[1, :, sa]
            lbb = lam_s[1, :, sb]
            ca = gate(carry_s[:, sa], prev)
            cb = carry_s[:, sb]

            def step(u, v, i):
                bu = bu_s[j, ka, pl.ds(i, 8, stride=Q), :]
                bv = bu_s[j, kb, pl.ds(i, 8, stride=Q), :]
                return (la * u + bu) + lba * v, (la * v + bv) + lbb * u

            u, v = ca, cb
            for i in range(Q):
                u, v = step(u, v, i)
            for k in range(3):
                sh = 1 << k
                us = jnp.where(row >= sh, pltpu.roll(u, sh, 0), 0.0)
                vs = jnp.where(row >= sh, pltpu.roll(v, sh, 0), 0.0)
                pa = lam_s[2 + 2 * k, :, sa]
                u, v = (u + pa * us + lam_s[3 + 2 * k, :, sa] * vs,
                        v + pa * vs + lam_s[3 + 2 * k, :, sb] * us)
            u = jnp.where(row == 0, ca, pltpu.roll(u, 1, 0))
            v = jnp.where(row == 0, cb, pltpu.roll(v, 1, 0))
            for i in range(Q):
                u, v = step(u, v, i)
                if i == QL - 1:
                    carry_s[:, sa] = jnp.where(row == 0, pltpu.roll(u, 1, 0), 0.0)
                    carry_s[:, sb] = jnp.where(row == 0, pltpu.roll(v, 1, 0), 0.0)
                h_s[ka, pl.ds(i, 8, stride=Q), :] = u
                if kb < NB:
                    h_s[kb, pl.ds(i, 8, stride=Q), :] = v
            prev = u

    def stage_c(j, split=False):
        g = lambda r, c: jnp.concatenate([h_s[c * NA + k, r * H:(r + 1) * H, :] for k in range(NA)], axis=1)
        parts = []

        def mm(i, rhs):
            lhs = pltpu.bitcast(cw_s[i], BF16)
            rhs = rhs.astype(BF16)
            if not split:
                return jax.lax.dot_general(lhs, rhs, NT, preferred_element_type=F32)
            cols = []
            for n in range(H // 128):
                acc = None
                for k in range(NA):
                    p = jax.lax.dot_general(lhs[:, k * 128:(k + 1) * 128],
                                            rhs[n * 128:(n + 1) * 128, k * 128:(k + 1) * 128],
                                            NT, preferred_element_type=F32)
                    parts.append(p)
                    acc = p if acc is None else acc + p
                cols.append(acc)
            return jnp.concatenate(cols, axis=1)

        z = jax.lax.dot_general(pltpu.bitcast(cm_s[...], BF16), h_s[2 * NA, :tb, :].astype(BF16), NT,
                                preferred_element_type=F32)
        z = z + tiles(xnT_s, j, 0, tb) * rep(col_s[0], tb)
        n2 = mm(0, g(0, 0))
        n4 = mm(5, g(0, 1) - g(0, 0))
        s_s[DH:, :H] = z[DH:, :H] + (n2 + n4)
        n5 = mm(1, g(1, 1))
        n3 = mm(6, g(1, 0) - g(1, 1))
        s_s[:DH, H:] = z[:DH, H:] + (n3 + n5)
        n1 = mm(2, g(0, 0) + g(1, 1))
        u = z[:DH, :H] + n1 + n4 - n5
        v = z[DH:, H:] + n1 - n2 + n3
        s_s[:DH, :H] = u + mm(3, g(0, 1) + g(1, 1))
        s_s[DH:, H:] = v + mm(4, g(0, 0) + g(1, 0))
        return parts

    def stage_w2(j, last=False):
        g = lambda r, c: a_s[r * H:(r + 1) * H, c * FH:(c + 1) * FH]

        def mm(lhs, rhs):
            return jax.lax.dot_general(lhs, rhs.astype(BF16), NT, preferred_element_type=F32)

        def fin(r0, lo, oT):
            r1, hi = r0 + oT.shape[0], lo + oT.shape[1]
            h = oT * 0.25 + rep(col_s[1, r0:r1, :], hi - lo)
            gt = h + h * jnp.tanh(h)
            o_s[j, r0:r1, lo:hi] = tiles(x_s, j, lo, hi)[r0:r1].astype(F32) + s_s[r0:r1, lo:hi] * gt
            if last:
                o_copy(j, lo, hi, r0, r1).start()

        n2 = mm(xblk(w2x_s, 0), g(0, 0))
        n4 = mm(wblk(w2_s, 1, DH, D), g(0, 1) - g(0, 0))
        fin(DH, 0, n2 + n4)
        n5 = mm(xblk(w2x_s, 1), g(1, 1))
        n3 = mm(wblk(w2_s, 0, 0, DH), g(1, 0) - g(1, 1))
        fin(0, H, n3 + n5)
        n1 = mm(xblk(w2x_s, 2), g(0, 0) + g(1, 1))
        u = n1 + n4 - n5
        v = n1 - n2 + n3
        n7 = mm(xblk(w2x_s, 3), g(0, 1) + g(1, 1))
        fin(0, 0, u + n7)
        s6 = g(0, 0) + g(1, 0)
        if not last:
            fin(DH, H, v + mm(xblk(w2x_s, 4), s6))
        else:
            for (lo, r0, r1) in LASTP:
                fin(DH + r0, H + lo, v[r0:r1, lo:lo + 128] + mm(xblk(w2x_s, 4, r0, r1), s6[lo:lo + 128, :]))
        return [heads(n2), heads(n4), heads(n5), heads(n3), heads(n1), heads(n7)]

    LASTP = ((0, 0, DH), (128, 0, 128), (128, 128, DH))

    def stage_init():
        lr = _row(lre_s)
        li = _row(lim_s)
        dt = jnp.exp(_row(ldt_s)).astype(BF16).astype(F32)
        mag = jnp.exp(dt * lr)
        ang = dt * li
        lbr = mag * jnp.cos(ang)
        lbi = mag * jnp.sin(ang)
        nr = lbr - 1.0
        den = lr * lr + li * li
        coef_s[...] = jnp.zeros_like(coef_s)
        coef_s[0:1, :] = 2.0 * (nr * lr + lbi * li) / den
        coef_s[1:2, :] = 2.0 * (lbi * lr - nr * li) / den
        a, b = pack_lam(lbr, lbi)
        lam_s[0] = jnp.broadcast_to(a, (8, W))
        lam_s[1] = jnp.broadcast_to(b, (8, W))
        pr, pi = lbr, lbi
        q = 1
        while q < Q - 1:
            pr, pi = _cmul(pr, pi, pr, pi)
            q *= 2
        pr, pi = _cmul(pr, pi, lbr, lbi)
        for k in range(3):
            a, b = pack_lam(pr, pi)
            lam_s[2 + 2 * k] = jnp.broadcast_to(a, (8, W))
            lam_s[3 + 2 * k] = jnp.broadcast_to(b, (8, W))
            pr, pi = _cmul(pr, pi, pr, pi)
        carry_s[...] = jnp.zeros_like(carry_s)
        bu_s[:, :, tb:, :] = jnp.zeros((nb, 8, 8, 128), F32)
        row = jax.lax.broadcasted_iota(jnp.int32, (KP - DH, NF * 128), 0)
        pad = pltpu.bitcast(jnp.where(row == 0, _row(b1v_s), 0.0).astype(BF16), U32)
        for k in range(NFH):
            w1x_s[0, k, DH // 2:, :] = pad[:, k * 128:(k + 1) * 128]
            w1x_s[1, k, DH // 2:, :] = pad[:, (NFH + k) * 128:(NFH + k + 1) * 128]
        w1x_s[2:5, :, DH // 2:, :] = jnp.zeros((3, NFH, (KP - DH) // 2, 128), U32)
        w1_s[:, D:, :] = jnp.zeros((NF, w1_s.shape[1] - D, 128), BF16)
        for k, r in enumerate((_row(dsk_s), 0.5 * _row(b2_s))):
            r = jnp.concatenate([r, jnp.zeros((1, DP - D), F32)], axis=1)
            col_s[k] = jnp.broadcast_to(r, (128, DP)).T[:D, :]

    def stage_cprep(deps):
        nch = len(deps)
        rows = DH // nch
        for q in range(nch):
            cf = gate(coef_s[...], deps[q])
            cr = cf[0:1, :]
            ci = cf[1:2, :]
            blk = {}
            for r in range(2):
                rs = slice(r * DH + q * rows, r * DH + (q + 1) * rows)
                c_re = cre_s[rs, :].astype(F32)
                c_im = cim_s[rs, :].astype(F32)
                cpr = c_re * cr - c_im * ci
                cpi = -(c_re * ci + c_im * cr)
                blk[r, 0], blk[r, 1] = cpr[:, :PA], cpi[:, :PA]
                mix = jnp.concatenate([cpr[:, PA:], cpi[:, PA:]], axis=1).astype(BF16)
                cm_s[(r * DH + q * rows) // 2:(r * DH + (q + 1) * rows) // 2, :] = pltpu.bitcast(mix, U32)
            outs = [blk[a] + blk[b] if sign > 0 else blk[a] - blk[b] for sign, a, b in W2X]
            outs += [blk[1, 1], blk[0, 0]]
            for i, o in enumerate(outs):
                cw_s[i, q * rows // 2:(q + 1) * rows // 2, :] = pltpu.bitcast(o.astype(BF16), U32)

    for c in vec_copies:
        c.start()
    x_copy(0).start()
    for c in b0_copies:
        c.start(priority=1)
    zsrc_s[...] = jnp.zeros_like(zsrc_s)
    z_copy.start()
    with scope('vwait'):
        for c in vec_copies + [z_copy]:
            c.wait()
    for c in b1_copies:
        c.start(priority=1)
    x_copy(1).start(priority=1)
    with scope('init'):
        stage_init()
    with scope('x0wait'):
        x_copy(0).wait()
    with scope('ln0'):
        xn = stage_ln1(0)
        xn_s[...] = xn
    with scope('b0_wait'):
        for c in b0_copies:
            c.wait()
    for j in range(2, na):
        x_copy(j).start(priority=1)
    with scope('bu_lo0'):
        stage_bu(0, 0, xn, 0, LO)
    with scope('b_wait'):
        for c in b1_copies:
            c.wait()
    for c in w1_copies + c_copies + w2_copies:
        c.start(priority=1)

    def a_chain(base, off, cnt):
        res = [stage_bu(base, off, xn_s[...], LO, NB)]
        e = None
        for t in range(1, cnt + 1):
            xn = stage_ln1(base * R + off + t, e)
            if t < cnt:
                res.append(stage_bu(base, off + t, xn, 0, NB))
                e = heads(res[-1])
            else:
                res.append(stage_bu(base, off + t, xn, 0, LO))
                xn_s[...] = xn
        return res

    with scope('xwait'):
        x_copy(1).wait()
    with scope('peel_a'):
        a_chain(0, 0, 1)

    def body_a(i, carry):
        with scope('xwait'):
            for t in range(1, GA + 1):
                x_copy(1 + i * GA + t).wait()
        with scope('body_a'):
            a_chain(i * (GA // R), 1, GA)
        return carry

    NIT = (na - 2) // GA - 1
    if SC0 is None:
        jax.lax.fori_loop(0, NIT, body_a, 0)
    else:
        body_a(0, 0)
        with scope('xwait'):
            for t in range(1, GA + 1):
                x_copy(1 + GA + t).wait()
        with scope('a2'):
            res = a_chain(GA // R, 1, GA)
            ev = [e for m in res for e in heads(m)]
            stage_scan(0, None, [None if k is None else ev[k] for k in SC0])

    with scope('w1_wait'):
        for t in range(1, GA + 1):
            x_copy(1 + NIT * GA + t).wait()
        for c in w1_copies:
            c.wait()
    with scope('last_a'):
        res = a_chain(NIT * (GA // R), 1, GA)
        ev = [e for m in res for e in heads(m, EV1[0])]
        comb_all(w1_s, w1x_s, W1X, ev[EV1[1]:EV1[1] + EV1[2] * NFH])

    with scope('w_wait'):
        for c in c_copies + w2_copies:
            c.wait()
    with scope('pro_b'):
        stage_bu(0, na - 1, xn_s[...], LO, NB)
        d, mm1 = stage_w1(0)
        stage_cprep([d[k] for k in CPK])
        if SC0 is None:
            stage_scan(0, d[GS0])
        parts = stage_c(0, True)
        ev = [e for i in EV2[0] for e in heads(parts[i], EV2[1])]
        comb_all(w2_s, w2x_s, W2X, ev[:EV2[2] * NFH])

    def body_b(j, carry):
        with scope('body_b'):
            dw = stage_w2(j)
            d, _ = stage_w1(j + 1)
            stage_scan(j + 1, d[GS] if GS >= 0 else dw[-GS - 1][0])
            stage_c(j + 1)
        o_copy(j).start()
        return carry

    jax.lax.fori_loop(0, nb - 1, body_b, 0)

    with scope('epi'):
        stage_w2(nb - 1, last=True)
    with scope('owait'):
        for j in range(nb - 1):
            o_copy(j).wait()
        for (lo, hi, r0, r1) in ((0, H, DH, D), (H, tb, 0, DH), (0, H, 0, DH)):
            o_copy(nb - 1, lo, hi, r0, r1).wait()
        for (lo, r0, r1) in LASTP:
            o_copy(nb - 1, H + lo, H + lo + 128, DH + r0, DH + r1).wait()


@jax.jit
def pallas_recurrent_scan__ssm_conv_s5__mixer_channel_mlp__prompt_kernel(
    A_x, A_Lambda_re, A_Lambda_im, A_B_re, A_B_im, A_C_re, A_C_im, A_log_dt, A_Dskip,
    B_x, B_w1, B_b1, B_w2, B_b2,
):
    Bsz, L, D = A_x.shape
    P = A_Lambda_re.shape[0]
    F = B_w1.shape[1]
    ta, tb = TA, TB
    na, nb = L // ta, L // tb
    NF = F // 128
    DH = D // 2
    KP = pl.cdiv(DH, 128) * 128
    xT = A_x.reshape(L, D).T
    outT = pl.pallas_call(
        functools.partial(_kernel, P=P),
        in_specs=[pl.BlockSpec(memory_space=pl.ANY)] * 13,
        out_specs=pl.BlockSpec(memory_space=pl.ANY),
        out_shape=jax.ShapeDtypeStruct((D, L), F32),
        scratch_shapes=[
            pltpu.VMEM((na, D, ta), BF16),
            pltpu.VMEM((nb, D, tb), F32),
            pltpu.VMEM((nb, 8, tb + 8, 128), F32),
            pltpu.VMEM((na, D, ta), F32),
            pltpu.VMEM((na, 16, ta), F32),
            pltpu.VMEM((2 * P, D), BF16),
            pltpu.VMEM((D, P), BF16),
            pltpu.VMEM((D, P), BF16),
            pltpu.VMEM((7, DH // 2, (P // 128) * 128), U32),
            pltpu.VMEM((NF, DH + KP, 128), BF16),
            pltpu.VMEM((NF, D, 128), BF16),
            pltpu.VMEM((5, NF // 2, KP // 2, 128), U32),
            pltpu.VMEM((5, NF // 2, DH // 2, 128), U32),
            pltpu.VMEM((8, 8, 1024), F32),
            pltpu.VMEM((8, 1024), F32),
            pltpu.VMEM((2, D, 128), F32),
            pltpu.VMEM((8, P), F32),
            pltpu.VMEM((D // 2, 128), U32),
            pltpu.VMEM((7, tb + 8, 128), F32),
            pltpu.VMEM((tb, F), F32),
            pltpu.VMEM((D, tb), F32),
            pltpu.VMEM((ta, D), BF16),
            pltpu.VMEM((8, 128), jnp.int32),
            pltpu.VMEM((8, 128), jnp.int32),
            pltpu.VMEM((P,), BF16), pltpu.VMEM((P,), BF16), pltpu.VMEM((P,), BF16),
            pltpu.VMEM((D,), BF16), pltpu.VMEM((F,), BF16), pltpu.VMEM((D,), BF16),
            pltpu.VMEM((F,), BF16),
            pltpu.SemaphoreType.DMA((na,)),
            pltpu.SemaphoreType.DMA(()),
            pltpu.SemaphoreType.DMA((5,)),
        ],
        compiler_params=pltpu.CompilerParams(
            vmem_limit_bytes=100 * 1024 * 1024,
            disable_semaphore_checks=True, disable_bounds_checks=True),
    )(xT, A_Lambda_re, A_Lambda_im, A_B_re, A_B_im, A_C_re, A_C_im,
      A_log_dt, A_Dskip, B_w1, B_b1, B_w2.T, B_b2)
    return outT.T.reshape(Bsz, L, D)
```

```python
import functools
import contextlib
import jax
import jax.numpy as jnp
import jax.experimental.pallas as pl
import jax.experimental.pallas.tpu as pltpu

SCOPES = 0
TA = 256
TB = 512
GA = 2
LO = 4
LNG = ((0,4,8,16),(2,6,11,20))
EVB = (4,7,10,11,12,14,15,17)
EVB0 = (0,1,2,4,5,6,8,9)
GS = -1
GS0 = 9
EV1 = ((0,64),48,7)
EV2 = ((3,7,11,15,19,23,27,31,35,39,),(0,40,80,120,160,),7)
CPK = (0,1,2,3,4,5,6,28,29,30,31,32,33,34)
SC0 = None
LNG0 = None
STB = 1
STG = ((0,0),(0,1),(4,1),(5,0))
M5F = 0
XB = 0
REC = 0
LNGL = ((0,3,11,None),(0,1,14,None))
LNG0L = None
EVS = (45,46,47,48,49,50,51,52,53,54,55,56,57,59,60,61,62,63,64,65,66,67,68,69,70,72,73,74,75,76,77,78,79,80,81,82,83,85,86,87,88,89,90,91,92,93,94,95,96)
EPS = 1e-5
F32 = jnp.float32
BF16 = jnp.bfloat16
U32 = jnp.uint32
NT = (((1,), (1,)), ((), ()))
GELU_C0 = 0.7978845608028654
GELU_C1 = 0.7978845608028654 * 0.044715


def scope(name):
    return jax.named_scope(name) if SCOPES else contextlib.nullcontext()


def _cmul(ar, ai, br, bi):
    return ar * br - ai * bi, ar * bi + ai * br


def _row(ref):
    return ref[...].astype(F32).reshape(1, ref.shape[0])


def _kernel(x_hbm, lre_hbm, lim_hbm, bre_hbm, bim_hbm, cre_hbm, cim_hbm, ldt_hbm, dsk_hbm,
            w1_hbm, b1_hbm, w2_hbm, b2_hbm, o_hbm,
            x_s, o_s, bu_s, xnT_s, st_s, bw_s, cre_s, cim_s, cw_s, w1_s, w2_s, w1x_s, w2x_s,
            lam_s, carry_s, col_s, coef_s, cm_s, h_s, a_s, s_s, bx_s, lx_s, m_s, st2_s, zero_s, zsrc_s,
            lre_s, lim_s, ldt_s, dsk_s, b1v_s, b2_s, pad_s,
            xsem, osem, wsem, *, P):
    ta, tb = TA, TB
    na = x_s.shape[0]
    D = x_s.shape[1]
    L = na * ta
    nb = L // tb
    R = tb // ta
    NF = w1_s.shape[0]
    NFH = NF // 2
    FH = NFH * 128
    DP = pl.cdiv(D, 128) * 128
    DH = D // 2
    KP = pl.cdiv(DH, 128) * 128
    H = tb // 2
    Q = tb // 8 + 1
    QL = tb - 7 * Q
    PA = (P // 128) * 128
    PB = P - PA
    NA = PA // 128
    NB = 2 * NA + 1
    W = 2 * PA + 256

    def x_copy(j):
        return pltpu.make_async_copy(x_hbm.at[:, pl.ds(j * ta, ta)], x_s.at[j], xsem.at[j])

    def o_copy(j, lo=0, hi=None, r0=0, r1=None):
        hi = tb if hi is None else hi
        r1 = D if r1 is None else r1
        return pltpu.make_async_copy(o_s.at[j, r0:r1, lo:hi],
                                     o_hbm.at[r0:r1, pl.ds(j * tb + lo, hi - lo)], osem)

    vec_copies = [pltpu.make_async_copy(src, dst, wsem.at[3]) for src, dst in
                  ((lre_hbm, lre_s), (lim_hbm, lim_s), (ldt_hbm, ldt_s), (dsk_hbm, dsk_s),
                   (b1_hbm, b1v_s), (b2_hbm, b2_s))]
    z_copy = pltpu.make_async_copy(zsrc_s, zero_s, wsem.at[3])
    w1_copies = [pltpu.make_async_copy(w1_hbm.at[:, k * 128:(k + 1) * 128], w1_s.at[k, 0:D, :], wsem.at[4])
                 for k in range(NF)]
    w2_copies = [pltpu.make_async_copy(w2_hbm.at[:, k * 128:(k + 1) * 128], w2_s.at[k], wsem.at[2])
                 for k in range(NF)]
    E = 256
    b0_copies = [pltpu.make_async_copy(bre_hbm.at[0:E, :], bw_s.at[0:E, :], wsem.at[0]),
                 pltpu.make_async_copy(bim_hbm.at[0:E, :], bw_s.at[PA:PA + E, :], wsem.at[0])]
    b1_copies = [
        pltpu.make_async_copy(bre_hbm.at[E:PA, :], bw_s.at[E:PA, :], wsem.at[1]),
        pltpu.make_async_copy(bim_hbm.at[E:PA, :], bw_s.at[PA + E:2 * PA, :], wsem.at[1]),
        pltpu.make_async_copy(bre_hbm.at[PA:P, :], bw_s.at[2 * PA:2 * PA + PB, :], wsem.at[1]),
        pltpu.make_async_copy(bim_hbm.at[PA:P, :], bw_s.at[2 * PA + PB:2 * P, :], wsem.at[1]),
    ]
    c_copies = [pltpu.make_async_copy(cre_hbm, cre_s, wsem.at[2]),
                pltpu.make_async_copy(cim_hbm, cim_s, wsem.at[2])]

    def pack_lam(re, im):
        a = jnp.concatenate([re[:, :PA], re[:, :PA], re[:, PA:], re[:, PA:], re[:, PA:], re[:, PA:]], axis=1)
        b = jnp.concatenate([-im[:, :PA], im[:, :PA], -im[:, PA:], im[:, PA:], im[:, PA:], -im[:, PA:]], axis=1)
        return a, b

    def rep(c, w):
        return c if w == 128 else jnp.concatenate([c] * (w // 128), axis=1)

    def gate(val, dep):
        if dep is None:
            return val
        w = pl.cdiv(val.shape[1], 128) * 128
        head = jnp.where(rep(zero_s[...], w)[:, :val.shape[1]] != 0, rep(dep, w)[:, :val.shape[1]], val[0:8, :])
        return head if val.shape[0] == 8 else jnp.concatenate([head, val[8:, :]], axis=0)

    def gate_row(val, dep):
        if dep is None:
            return val
        w = val.shape[1]
        return jnp.where(rep(zero_s[0:1, :], w) != 0, rep(dep[0:1, :], w), val)

    def wblk(ref, half, r0, r1):
        r32 = ref.bitcast(U32)
        return pltpu.bitcast(
            jnp.concatenate([r32[half * NFH + k, r0 // 2:r1 // 2, :] for k in range(NFH)], axis=1), BF16)

    def xblk(ref, i, r0=0, r1=None):
        r1 = 2 * ref.shape[2] if r1 is None else r1
        return pltpu.bitcast(jnp.concatenate([ref[i, k, r0 // 2:r1 // 2, :] for k in range(NFH)], axis=1), BF16)

    def tiles(ref, j, lo, hi):
        parts = []
        for r in range(R):
            a, b = max(lo, r * ta), min(hi, (r + 1) * ta)
            if a < b:
                parts.append(ref[j * R + r, :, a - r * ta:b - r * ta])
        return parts[0] if len(parts) == 1 else jnp.concatenate(parts, axis=1)

    def xn_tiles(j, lo, hi):
        t = tiles(xnT_s, j, lo, hi)
        return pltpu.bitcast(t, BF16).astype(F32) if XB else t

    def ln1_part(j, lo, hi, deps):
        if REC:
            u = x_s.bitcast(U32)[j, :, lo:hi]
            if deps[0] is not None:
                u = gate(u, pltpu.bitcast(deps[0], U32))
            xe, xo = [pltpu.unpack_elementwise(u, index=e, packed_dtype=BF16, unpacked_dtype=F32) for e in range(2)]
            m = gate_row((jnp.sum(xe, axis=0, keepdims=True) + jnp.sum(xo, axis=0, keepdims=True)) * (1.0 / D), deps[1])
            if REC == 2:
                x2 = x_s[j, :, lo:hi].astype(F32) - m
                v = jnp.sum(x2 * x2, axis=0, keepdims=True) * (1.0 / D)
                xc = x2
            else:
                de, do = xe - m, xo - m
                v = (jnp.sum(de * de, axis=0, keepdims=True) + jnp.sum(do * do, axis=0, keepdims=True)) * (1.0 / D)
                xc = x_s[j, :, lo:hi].astype(F32) - m
        else:
            x = gate(x_s[j, :, lo:hi].astype(F32), deps[0])
            m = gate_row(jnp.sum(x, axis=0, keepdims=True) * (1.0 / D), deps[1])
            xc = x - m
            v = jnp.sum(xc * xc, axis=0, keepdims=True) * (1.0 / D)
        xf = xc * gate_row(jax.lax.rsqrt(v + EPS), deps[2])
        xnT_b = xf.astype(BF16)
        if XB:
            xn = xf if XB == 2 else xnT_b.astype(F32)
            xnT_s[j, :, lo:hi] = pltpu.bitcast(xnT_b, U32)
        else:
            xn = xnT_b.astype(F32)
            xnT_s[j, :, lo:hi] = xn
        if STB:
            return xnT_b, xn
        xs = xn if deps[3] is None else gate(xnT_s[j, :, lo:hi], deps[3])
        m2 = jnp.sum(xs, axis=0, keepdims=True) * (1.0 / D)
        v2 = jnp.sum(xs * xs, axis=0, keepdims=True) * (1.0 / D) - m2 * m2
        r2 = jax.lax.rsqrt(v2 + EPS)
        st_s[j, 0:8, lo:hi] = jnp.broadcast_to(r2, (8, hi - lo))
        st_s[j, 8:16, lo:hi] = jnp.broadcast_to(m2 * r2, (8, hi - lo))
        return xnT_b, xn

    def stage_ln1(j, e=None, lng=None):
        if e is None or lng is None:
            return ln1_part(j, 0, ta, (None,) * 4)[1]
        if lng[0] == 'ser':
            order = lng[1]
            first = ln1_part(j, order * 128, (order + 1) * 128, (None if lng[2] is None else e[lng[2]], None, None, None))[1]
            dep = first[lng[3]:lng[3] + 8, :]
            second = ln1_part(j, (1 - order) * 128, (2 - order) * 128, (dep, None, None, None) if lng[4] == 0 else (None, dep, None, None))[1]
            return jnp.concatenate([first, second] if order == 0 else [second, first], axis=1)
        return jnp.concatenate(
            [ln1_part(j, k * 128, (k + 1) * 128, tuple(None if g is None else e[g] for g in lng[k]))[1]
             for k in range(ta // 128)], axis=1)

    KA = 256
    KB = D - KA
    HA = ta // 2

    def bu_operands(xn):
        a11, a12, a21, a22 = xn[:KA, :HA], xn[KA:, :HA], xn[:KA, HA:], xn[KA:, HA:]
        addp = lambda t, b: jnp.concatenate([t[:KB] + b, t[KB:]], axis=0)
        padz = lambda b: jnp.concatenate([b, jnp.zeros((KA - KB, HA), F32)], axis=0)
        ops = (addp(a21, a22), padz(a11[:KB] + a12), padz(a22), a11, addp(a11, a22), padz(a12 - a22), a21 - a11)
        return [o.astype(BF16).T for o in ops]

    def bu_lo(l2, l5):
        r2 = jnp.concatenate([bw_s[0:PA, 0:KA], bw_s[2 * PA:, 0:KA]], axis=0)
        if M5F:
            m5 = jax.lax.dot_general(l5[:, :KB], bw_s[PA:, KA:], NT, preferred_element_type=F32)
        m2 = jax.lax.dot_general(l2, r2, NT, preferred_element_type=F32)
        if not M5F:
            m5 = jax.lax.dot_general(l5[:, :KB], bw_s[PA:, KA:], NT, preferred_element_type=F32)
        return m2, m5

    def bu_hi(base, off, m2, m5, ls):
        jb = base + off // R
        r0 = (off % R) * ta

        def mm(i, rows):
            return jax.lax.dot_general(ls[i], pltpu.bitcast(bx_s[i, 0:rows // 2, :], BF16), NT,
                                       preferred_element_type=F32)

        def put(half, k0, val):
            rows = pl.ds(r0 + half * HA, HA)
            for k in range(NA):
                bu_s[jb, k0 + k, rows, :] = val[:, k * 128:(k + 1) * 128]
            if val.shape[1] > PA:
                bu_s[jb, NB - 1, rows, :] = val[:, PA:]
                bu_s[jb, NB, rows, :] = pltpu.roll(val[:, PA:], PB, 1)

        m4 = mm(0, PA + 128)
        put(1, 0, m2 + m4)
        m3 = mm(1, PA + 128)
        put(0, NA, m3 + m5)
        m1 = mm(2, PA)
        u = m1 + m4[:, :PA] - m5[:, :PA]
        v = m1 - m2[:, :PA] + m3[:, :PA]
        m7 = mm(3, PA)
        put(0, 0, u + m7)
        m6 = mm(4, PA)
        put(1, NA, v + m6)
        return [m4, m3, m1, m7, m6]

    def stage_bprep(q0, deps):
        rows = 32

        def top_bot(r0, dep):
            w = bw_s[r0:r0 + rows, :].astype(F32)
            w = w + jnp.where(rep(zero_s[0:1, :], DP) != 0, rep(dep[0:1, :], DP), 0.0)[:, :D]
            return w[:, :KA], jnp.concatenate([w[:, KA:], jnp.zeros((rows, KA - KB), F32)], axis=1)

        lane = jax.lax.broadcasted_iota(jnp.int32, (rows, KA), 1)
        for q, dep in enumerate(deps):
            r0 = (q0 + q) * rows
            if r0 < PA:
                b11, b21 = top_bot(r0, dep)
                b12, b22 = top_bot(PA + r0, dep)
                outs = [jnp.where(lane < KB, b21 - b11, 0.0), b12 - b22, b11 + b22, b21 + b22, b11 + b12]
            else:
                b1, b2 = top_bot(PA + r0, dep)
                outs = [jnp.where(lane < KB, b2 - b1, 0.0), b1 - b2]
            o = pltpu.bitcast(jnp.concatenate(outs, axis=1).astype(BF16), U32)
            for i in range(len(outs)):
                bx_s[i, r0 // 2:(r0 + rows) // 2, :] = o[:, i * KA:(i + 1) * KA]

    def stage_bu0(xn, ks):
        rhs = jnp.concatenate([bw_s[k * 128:(k + 1) * 128, :] for k in ks], axis=0)
        bu = jax.lax.dot_general(xn, rhs, NT, preferred_element_type=F32)
        for i, k in enumerate(ks):
            bu_s[0, k, 0:ta, :] = bu[:, i * 128:(i + 1) * 128]
            if k == NB - 1:
                bu_s[0, NB, 0:ta, :] = pltpu.roll(bu[:, i * 128:(i + 1) * 128], PB, 1)
        return bu

    def heads(m, rows=(0,)):
        return [m[r:r + 8, k * 128:(k + 1) * 128] for k in range(m.shape[1] // 128) for r in rows]

    def stage_stats(j, deps):
        for k in range(tb // 128):
            xs = gate(xn_tiles(j, k * 128, (k + 1) * 128), deps[k])
            m2 = jnp.sum(xs, axis=0, keepdims=True) * (1.0 / D)
            v2 = jnp.sum(xs * xs, axis=0, keepdims=True) * (1.0 / D) - m2 * m2
            r2 = jax.lax.rsqrt(v2 + EPS)
            st2_s[0:8, k * 128:(k + 1) * 128] = jnp.broadcast_to(r2, (8, 128))
            st2_s[8:16, k * 128:(k + 1) * 128] = jnp.broadcast_to(m2 * r2, (8, 128))

    def stage_w1(j, prep=None):
        st = st2_s[...] if STB else tiles(st_s, j, 0, tb)
        yT = xn_tiles(j, 0, tb) * st[0:1, :] - st[8:9, :]
        a11, a12, a21, a22 = yT[:DH, :H], yT[DH:, :H], yT[:DH, H:], yT[DH:, H:]
        row = jax.lax.broadcasted_iota(jnp.int32, (KP - DH, H), 0)
        zeros = jnp.zeros((KP - DH, H), F32)
        ones = jnp.where(row == 0, 1.0, 0.0).astype(F32)

        def mm(lhsT, rhs, pad=zeros):
            lhs = jnp.concatenate([lhsT, pad], axis=0).astype(BF16).T
            return jnp.dot(lhs, rhs, preferred_element_type=F32)

        def act(r, c, x):
            t = jnp.tanh(x * (x * x * GELU_C1 + GELU_C0))
            a_s[r * H:(r + 1) * H, c * FH:(c + 1) * FH] = x + x * t

        deps = []
        m2 = mm(a21 + a22, wblk(w1_s, 0, 0, KP))
        deps += heads(m2)
        if prep:
            prep(0, deps)
        m4 = mm(a22, xblk(w1x_s, 0), ones)
        act(1, 0, m2 + m4)
        deps += heads(m4)
        m5 = mm(a11 + a12, wblk(w1_s, 1, DH, DH + KP))
        deps += heads(m5)
        if prep:
            prep(1, deps)
        m3 = mm(a11, xblk(w1x_s, 1), ones)
        act(0, 1, m3 + m5)
        deps += heads(m3)
        if prep:
            prep(2, deps)
        m1 = mm(a11 + a22, xblk(w1x_s, 2))
        deps += heads(m1)
        u = m1 + m4 - m5
        v = m1 - m2 + m3
        if prep:
            prep(3, deps)
        m7 = mm(a12 - a22, xblk(w1x_s, 3))
        act(0, 0, u + m7)
        deps += heads(m7)
        if prep:
            prep(4, deps)
        m6 = mm(a21 - a11, xblk(w1x_s, 4))
        act(1, 1, v + m6)
        deps += heads(m6)
        return deps, (m2, m4, m5, m3, m1, m7, m6)

    W1X = ((-1, (1, 0), (0, 0)), (-1, (0, 1), (1, 1)), (1, (0, 0), (1, 1)), (1, (1, 0), (1, 1)), (1, (0, 0), (0, 1)))
    W2X = ((1, (1, 0), (1, 1)), (1, (0, 0), (0, 1)), (1, (0, 0), (1, 1)), (-1, (0, 1), (1, 1)), (-1, (1, 0), (0, 0)))

    def comb_all(src, dst, specs, deps):
        src32 = src.bitcast(U32)
        per = len(deps) // NFH
        rows = DH // 2 // per
        z = jnp.concatenate([zero_s[...]] * (rows // 8), axis=0) != 0
        for n, dep in enumerate(deps):
            k, q = divmod(n, per)
            d = jnp.concatenate([pltpu.bitcast(dep, U32)] * (rows // 8), axis=0)
            blk = {}
            for r in range(2):
                for c in range(2):
                    r0 = r * DH // 2 + q * rows
                    w = jnp.where(z, d, src32[c * NFH + k, r0:r0 + rows, :])
                    blk[r, c] = [pltpu.unpack_elementwise(w, index=e, packed_dtype=BF16, unpacked_dtype=F32)
                                 for e in range(2)]
            for i, (sign, a, b) in enumerate(specs):
                s = [u + v if sign > 0 else u - v for u, v in zip(blk[a], blk[b])]
                dst[i, k, q * rows:(q + 1) * rows, :] = pltpu.pack_elementwise(s, packed_dtype=BF16)

    def stage_scan(j, dep=None, deps=None):
        row = jax.lax.broadcasted_iota(jnp.int32, (8, 128), 0)
        prev = dep
        for ip, (ka, kb) in enumerate(((0, 3), (1, 4), (2, 5), (6, 7))):
            if deps is not None and deps[ip] is not None:
                prev = deps[ip]
            sa = slice(ka * 128, (ka + 1) * 128)
            sb = slice(kb * 128, (kb + 1) * 128)
            la = lam_s[0, :, sa]
            lba = lam_s[1, :, sa]
            lbb = lam_s[1, :, sb]
            ca = gate(carry_s[:, sa], prev)
            cb = carry_s[:, sb]

            def step(u, v, i):
                bu = bu_s[j, ka, pl.ds(i, 8, stride=Q), :]
                bv = bu_s[j, kb, pl.ds(i, 8, stride=Q), :]
                return (la * u + bu) + lba * v, (la * v + bv) + lbb * u

            u, v = ca, cb
            for i in range(Q):
                u, v = step(u, v, i)
            for k in range(3):
                sh = 1 << k
                us = jnp.where(row >= sh, pltpu.roll(u, sh, 0), 0.0)
                vs = jnp.where(row >= sh, pltpu.roll(v, sh, 0), 0.0)
                pa = lam_s[2 + 2 * k, :, sa]
                u, v = (u + pa * us + lam_s[3 + 2 * k, :, sa] * vs,
                        v + pa * vs + lam_s[3 + 2 * k, :, sb] * us)
            u = jnp.where(row == 0, ca, pltpu.roll(u, 1, 0))
            v = jnp.where(row == 0, cb, pltpu.roll(v, 1, 0))
            for i in range(Q):
                u, v = step(u, v, i)
                if i == QL - 1:
                    carry_s[:, sa] = jnp.where(row == 0, pltpu.roll(u, 1, 0), 0.0)
                    carry_s[:, sb] = jnp.where(row == 0, pltpu.roll(v, 1, 0), 0.0)
                h_s[ka, pl.ds(i, 8, stride=Q), :] = u
                if kb < NB:
                    h_s[kb, pl.ds(i, 8, stride=Q), :] = v
            prev = u

    def stage_c(j, split=False):
        g = lambda r, c: jnp.concatenate([h_s[c * NA + k, r * H:(r + 1) * H, :] for k in range(NA)], axis=1)
        parts = []

        def mm(i, rhs):
            lhs = pltpu.bitcast(cw_s[i], BF16)
            rhs = rhs.astype(BF16)
            if not split:
                return jax.lax.dot_general(lhs, rhs, NT, preferred_element_type=F32)
            cols = []
            for n in range(H // 128):
                acc = None
                for k in range(NA):
                    p = jax.lax.dot_general(lhs[:, k * 128:(k + 1) * 128],
                                            rhs[n * 128:(n + 1) * 128, k * 128:(k + 1) * 128],
                                            NT, preferred_element_type=F32)
                    parts.append(p)
                    acc = p if acc is None else acc + p
                cols.append(acc)
            return jnp.concatenate(cols, axis=1)

        z = jax.lax.dot_general(pltpu.bitcast(cm_s[...], BF16), h_s[2 * NA, :tb, :].astype(BF16), NT,
                                preferred_element_type=F32)
        z = z + xn_tiles(j, 0, tb) * rep(col_s[0], tb)
        n2 = mm(0, g(0, 0))
        n4 = mm(5, g(0, 1) - g(0, 0))
        s_s[DH:, :H] = z[DH:, :H] + (n2 + n4)
        n5 = mm(1, g(1, 1))
        n3 = mm(6, g(1, 0) - g(1, 1))
        s_s[:DH, H:] = z[:DH, H:] + (n3 + n5)
        n1 = mm(2, g(0, 0) + g(1, 1))
        u = z[:DH, :H] + n1 + n4 - n5
        v = z[DH:, H:] + n1 - n2 + n3
        s_s[:DH, :H] = u + mm(3, g(0, 1) + g(1, 1))
        s_s[DH:, H:] = v + mm(4, g(0, 0) + g(1, 0))
        return parts

    def stage_w2(j, last=False):
        g = lambda r, c: a_s[r * H:(r + 1) * H, c * FH:(c + 1) * FH]

        def mm(lhs, rhs):
            return jax.lax.dot_general(lhs, rhs.astype(BF16), NT, preferred_element_type=F32)

        def fin(r0, lo, oT):
            r1, hi = r0 + oT.shape[0], lo + oT.shape[1]
            h = oT * 0.25 + rep(col_s[1, r0:r1, :], hi - lo)
            gt = h + h * jnp.tanh(h)
            o_s[j, r0:r1, lo:hi] = tiles(x_s, j, lo, hi)[r0:r1].astype(F32) + s_s[r0:r1, lo:hi] * gt
            if last:
                o_copy(j, lo, hi, r0, r1).start()

        n2 = mm(xblk(w2x_s, 0), g(0, 0))
        n4 = mm(wblk(w2_s, 1, DH, D), g(0, 1) - g(0, 0))
        fin(DH, 0, n2 + n4)
        n5 = mm(xblk(w2x_s, 1), g(1, 1))
        n3 = mm(wblk(w2_s, 0, 0, DH), g(1, 0) - g(1, 1))
        fin(0, H, n3 + n5)
        n1 = mm(xblk(w2x_s, 2), g(0, 0) + g(1, 1))
        u = n1 + n4 - n5
        v = n1 - n2 + n3
        n7 = mm(xblk(w2x_s, 3), g(0, 1) + g(1, 1))
        fin(0, 0, u + n7)
        s6 = g(0, 0) + g(1, 0)
        if not last:
            fin(DH, H, v + mm(xblk(w2x_s, 4), s6))
        else:
            for (lo, r0, r1) in LASTP:
                fin(DH + r0, H + lo, v[r0:r1, lo:lo + 128] + mm(xblk(w2x_s, 4, r0, r1), s6[lo:lo + 128, :]))
        return [heads(n2), heads(n4), heads(n5), heads(n3), heads(n1), heads(n7)]

    LASTP = ((0, 0, DH), (128, 0, 128), (128, 128, DH))

    def stage_init():
        lr = _row(lre_s)
        li = _row(lim_s)
        dt = jnp.exp(_row(ldt_s)).astype(BF16).astype(F32)
        mag = jnp.exp(dt * lr)
        ang = dt * li
        lbr = mag * jnp.cos(ang)
        lbi = mag * jnp.sin(ang)
        nr = lbr - 1.0
        den = lr * lr + li * li
        coef_s[...] = jnp.zeros_like(coef_s)
        coef_s[0:1, :] = 2.0 * (nr * lr + lbi * li) / den
        coef_s[1:2, :] = 2.0 * (lbi * lr - nr * li) / den
        a, b = pack_lam(lbr, lbi)
        lam_s[0] = jnp.broadcast_to(a, (8, W))
        lam_s[1] = jnp.broadcast_to(b, (8, W))
        pr, pi = lbr, lbi
        q = 1
        while q < Q - 1:
            pr, pi = _cmul(pr, pi, pr, pi)
            q *= 2
        pr, pi = _cmul(pr, pi, lbr, lbi)
        for k in range(3):
            a, b = pack_lam(pr, pi)
            lam_s[2 + 2 * k] = jnp.broadcast_to(a, (8, W))
            lam_s[3 + 2 * k] = jnp.broadcast_to(b, (8, W))
            pr, pi = _cmul(pr, pi, pr, pi)
        carry_s[...] = jnp.zeros_like(carry_s)
        bu_s[:, :, tb:, :] = jnp.zeros((nb, 8, 8, 128), F32)
        row = jax.lax.broadcasted_iota(jnp.int32, (KP - DH, NF * 128), 0)
        pad = pltpu.bitcast(jnp.where(row == 0, _row(b1v_s), 0.0).astype(BF16), U32)
        for k in range(NFH):
            w1x_s[0, k, DH // 2:, :] = pad[:, k * 128:(k + 1) * 128]
            w1x_s[1, k, DH // 2:, :] = pad[:, (NFH + k) * 128:(NFH + k + 1) * 128]
        w1x_s[2:5, :, DH // 2:, :] = jnp.zeros((3, NFH, (KP - DH) // 2, 128), U32)
        w1_s[:, D:, :] = jnp.zeros((NF, w1_s.shape[1] - D, 128), BF16)
        for k, r in enumerate((_row(dsk_s), 0.5 * _row(b2_s))):
            r = jnp.concatenate([r, jnp.zeros((1, DP - D), F32)], axis=1)
            col_s[k] = jnp.broadcast_to(r, (128, DP)).T[:D, :]

    def stage_cprep(deps):
        nch = len(deps)
        rows = DH // nch
        for q in range(nch):
            cf = gate(coef_s[...], deps[q])
            cr = cf[0:1, :]
            ci = cf[1:2, :]
            blk = {}
            for r in range(2):
                rs = slice(r * DH + q * rows, r * DH + (q + 1) * rows)
                c_re = cre_s[rs, :].astype(F32)
                c_im = cim_s[rs, :].astype(F32)
                cpr = c_re * cr - c_im * ci
                cpi = -(c_re * ci + c_im * cr)
                blk[r, 0], blk[r, 1] = cpr[:, :PA], cpi[:, :PA]
                mix = jnp.concatenate([cpr[:, PA:], cpi[:, PA:]], axis=1).astype(BF16)
                cm_s[(r * DH + q * rows) // 2:(r * DH + (q + 1) * rows) // 2, :] = pltpu.bitcast(mix, U32)
            outs = [blk[a] + blk[b] if sign > 0 else blk[a] - blk[b] for sign, a, b in W2X]
            outs += [blk[1, 1], blk[0, 0]]
            for i, o in enumerate(outs):
                cw_s[i, q * rows // 2:(q + 1) * rows // 2, :] = pltpu.bitcast(o.astype(BF16), U32)

    for c in vec_copies:
        c.start()
    x_copy(0).start()
    for c in b0_copies:
        c.start(priority=1)
    zsrc_s[...] = jnp.zeros_like(zsrc_s)
    z_copy.start()
    with scope('vwait'):
        for c in vec_copies + [z_copy]:
            c.wait()
    for c in b1_copies:
        c.start(priority=1)
    x_copy(1).start(priority=1)
    with scope('init'):
        stage_init()
    with scope('x0wait'):
        x_copy(0).wait()
    with scope('ln0'):
        xn = ln1_part(0, 0, ta, (None,) * 4)[0].T
    with scope('b0_wait'):
        for c in b0_copies:
            c.wait()
    for j in range(2, na):
        x_copy(j).start(priority=1)
    with scope('bu_lo0'):
        ev = heads(stage_bu0(xn, (0, 1, NA, NA + 1)), (0, 64, 128, 192))
        stage_bprep(0, [ev[k] for k in EVB0])
    with scope('b_wait'):
        for c in b1_copies:
            c.wait()
    for c in w1_copies + c_copies + w2_copies:
        c.start(priority=1)

    def stash(m2, m5, ls):
        m_s[0] = m2
        m_s[1] = m5
        for i in range(5):
            lx_s[i] = pltpu.bitcast(ls[2 + i], U32)

    def finish(base, off):
        return bu_hi(base, off, m_s[0], m_s[1], [pltpu.bitcast(lx_s[i], BF16) for i in range(5)])

    def a_chain(base, off, cnt, lng0=None, lng=None):
        lng0, lng = (LNG0, LNG) if lng is None else (lng0, lng)
        res = finish(base, off)
        e = [h for m in res for h in heads(m)]
        for t in range(1, cnt + 1):
            ls = bu_operands(stage_ln1(base * R + off + t, e, lng0 if t == 1 else lng))
            m2, m5 = bu_lo(ls[0], ls[1])
            res += [m2, m5]
            if t < cnt:
                now = [m2, m5] + bu_hi(base, off + t, m2, m5, ls[2:])
                res += now[2:]
                e = [h for m in now for h in heads(m)]
            else:
                stash(m2, m5, ls)
        return res

    with scope('xwait'):
        x_copy(1).wait()
    with scope('peel_a'):
        bu0 = stage_bu0(xn, (2, NA + 2, NB - 1))
        ls = bu_operands(stage_ln1(1))
        m2, m5 = bu_lo(ls[0], ls[1])
        stash(m2, m5, ls)
        ev = heads(bu0, (0, 64, 128, 192)) + heads(m2) + heads(m5)
        stage_bprep(8, [ev[k] for k in EVB])

    def body_a(i, carry):
        with scope('xwait'):
            for t in range(1, GA + 1):
                x_copy(1 + i * GA + t).wait()
        with scope('body_a'):
            a_chain(i * (GA // R), 1, GA)
        return carry

    NIT = (na - 2) // GA - 1
    if SC0 is None:
        jax.lax.fori_loop(0, NIT, body_a, 0)
    else:
        body_a(0, 0)
        with scope('xwait'):
            for t in range(1, GA + 1):
                x_copy(1 + GA + t).wait()
        with scope('a2'):
            res = a_chain(GA // R, 1, GA)
            ev = [e for m in res for e in heads(m)]
            stage_scan(0, None, [None if k is None else ev[k] for k in SC0])

    with scope('w1_wait'):
        for t in range(1, GA + 1):
            x_copy(1 + NIT * GA + t).wait()
        for c in w1_copies:
            c.wait()
    with scope('last_a'):
        res = a_chain(NIT * (GA // R), 1, GA, LNG0L, LNGL)
        ev = [e for m in res for e in heads(m, EV1[0])]
        comb_all(w1_s, w1x_s, W1X, ev[EV1[1]:EV1[1] + EV1[2] * NFH] if EVS is None else [ev[k] for k in EVS])

    with scope('w_wait'):
        for c in c_copies + w2_copies:
            c.wait()
    with scope('pro_b'):
        finish(0, na - 1)
        if STB:
            stage_stats(0, [None] * 4)
        d, mm1 = stage_w1(0)
        stage_cprep([d[k] for k in CPK])
        if SC0 is None:
            stage_scan(0, d[GS0])
        parts = stage_c(0, True)
        ev = [e for i in EV2[0] for e in heads(parts[i], EV2[1])]
        comb_all(w2_s, w2x_s, W2X, ev[:EV2[2] * NFH])

    def body_b(j, carry):
        with scope('body_b'):
            dw = stage_w2(j)
            if STB:
                stage_stats(j + 1, [None if g is None else dw[g[0]][g[1]] for g in STG])
            d, _ = stage_w1(j + 1)
            stage_scan(j + 1, d[GS] if GS >= 0 else dw[-GS - 1][0])
            stage_c(j + 1)
        o_copy(j).start()
        return carry

    jax.lax.fori_loop(0, nb - 1, body_b, 0)

    with scope('epi'):
        stage_w2(nb - 1, last=True)
    with scope('owait'):
        for j in range(nb - 1):
            o_copy(j).wait()
        for (lo, hi, r0, r1) in ((0, H, DH, D), (H, tb, 0, DH), (0, H, 0, DH)):
            o_copy(nb - 1, lo, hi, r0, r1).wait()
        for (lo, r0, r1) in LASTP:
            o_copy(nb - 1, H + lo, H + lo + 128, DH + r0, DH + r1).wait()


@jax.jit
def pallas_recurrent_scan__ssm_conv_s5__mixer_channel_mlp__prompt_kernel(
    A_x, A_Lambda_re, A_Lambda_im, A_B_re, A_B_im, A_C_re, A_C_im, A_log_dt, A_Dskip,
    B_x, B_w1, B_b1, B_w2, B_b2,
):
    Bsz, L, D = A_x.shape
    P = A_Lambda_re.shape[0]
    F = B_w1.shape[1]
    ta, tb = TA, TB
    na, nb = L // ta, L // tb
    NF = F // 128
    DH = D // 2
    KP = pl.cdiv(DH, 128) * 128
    xT = A_x.reshape(L, D).T
    outT = pl.pallas_call(
        functools.partial(_kernel, P=P),
        in_specs=[pl.BlockSpec(memory_space=pl.ANY)] * 13,
        out_specs=pl.BlockSpec(memory_space=pl.ANY),
        out_shape=jax.ShapeDtypeStruct((D, L), F32),
        scratch_shapes=[
            pltpu.VMEM((na, D, ta), BF16),
            pltpu.VMEM((nb, D, tb), F32),
            pltpu.VMEM((nb, 8, tb + 8, 128), F32),
            pltpu.VMEM((na, D // 2, ta), U32) if XB else pltpu.VMEM((na, D, ta), F32),
            pltpu.VMEM((na, 16, ta), F32),
            pltpu.VMEM((2 * P, D), BF16),
            pltpu.VMEM((D, P), BF16),
            pltpu.VMEM((D, P), BF16),
            pltpu.VMEM((7, DH // 2, (P // 128) * 128), U32),
            pltpu.VMEM((NF, DH + KP, 128), BF16),
            pltpu.VMEM((NF, D, 128), BF16),
            pltpu.VMEM((5, NF // 2, KP // 2, 128), U32),
            pltpu.VMEM((5, NF // 2, DH // 2, 128), U32),
            pltpu.VMEM((8, 8, 1024), F32),
            pltpu.VMEM((8, 1024), F32),
            pltpu.VMEM((2, D, 128), F32),
            pltpu.VMEM((8, P), F32),
            pltpu.VMEM((D // 2, 128), U32),
            pltpu.VMEM((7, tb + 8, 128), F32),
            pltpu.VMEM((tb, F), F32),
            pltpu.VMEM((D, tb), F32),
            pltpu.VMEM((5, 256, 256), U32),
            pltpu.VMEM((5, ta // 4, 256), U32),
            pltpu.VMEM((2, ta // 2, 512), F32),
            pltpu.VMEM((16, tb), F32),
            pltpu.VMEM((8, 128), jnp.int32),
            pltpu.VMEM((8, 128), jnp.int32),
            pltpu.VMEM((P,), BF16), pltpu.VMEM((P,), BF16), pltpu.VMEM((P,), BF16),
            pltpu.VMEM((D,), BF16), pltpu.VMEM((F,), BF16), pltpu.VMEM((D,), BF16),
            pltpu.VMEM((F,), BF16),
            pltpu.SemaphoreType.DMA((na,)),
            pltpu.SemaphoreType.DMA(()),
            pltpu.SemaphoreType.DMA((5,)),
        ],
        compiler_params=pltpu.CompilerParams(
            vmem_limit_bytes=100 * 1024 * 1024,
            disable_semaphore_checks=True, disable_bounds_checks=True),
    )(xT, A_Lambda_re, A_Lambda_im, A_B_re, A_B_im, A_C_re, A_C_im,
      A_log_dt, A_Dskip, B_w1, B_b1, B_w2.T, B_b2)
    return outT.T.reshape(Bsz, L, D)
```

```python
import jax
import jax.numpy as jnp
import jax.experimental.pallas as pl
import jax.experimental.pallas.tpu as pltpu

F32 = jnp.float32
BF16 = jnp.bfloat16
U32 = jnp.uint32
NT = (((1,), (1,)), ((), ()))
EPS = 1e-5
GELU_C0 = 0.7978845608028654
GELU_C1 = 0.7978845608028654 * 0.044715

TA = 256
TB = 512

EVB0 = (0,1,2,4,5,6,8,9)
EVB = (6,7,10,12,14,15,16,18)
LNG = ((0,2,12),(0,2,5))
LNGL = ((0,3,11),(0,1,14))
EVS = (45,46,47,48,49,50,51,52,53,54,55,56,57,59,60,61,62,63,64,65,66,67,68,69,70,72,73,74,75,76,77,78,79,80,81,82,83,85,86,87,88,89,90,91,92,93,94,95,96)
CPK = (0,1,2,3,4,5,6,28,29,30,31,32,33,34)
GS0 = 4
EV2 = ((3,7,11,15,19,23,27,31,35,39),(0,40,80,120,160))
STG = (0,1,9,10)
GS = 0

RHS_SUMS = ((-1, (1, 0), (0, 0)), (-1, (0, 1), (1, 1)), (1, (0, 0), (1, 1)), (1, (1, 0), (1, 1)), (1, (0, 0), (0, 1)))
LHS_SUMS = ((1, (1, 0), (1, 1)), (1, (0, 0), (0, 1)), (1, (0, 0), (1, 1)), (-1, (0, 1), (1, 1)), (-1, (1, 0), (0, 0)))


def _cmul(ar, ai, br, bi):
    return ar * br - ai * bi, ar * bi + ai * br


def _row(ref):
    return ref[...].astype(F32).reshape(1, ref.shape[0])


def _rep(c, w):
    return c if w == 128 else jnp.concatenate([c] * (w // 128), axis=1)


def _dot_nt(a, b):
    return jax.lax.dot_general(a, b, NT, preferred_element_type=F32)


def _unpack2(w):
    return [pltpu.unpack_elementwise(w, index=e, packed_dtype=BF16, unpacked_dtype=F32) for e in range(2)]


def _pack2(ws):
    return pltpu.pack_elementwise(ws, packed_dtype=BF16)


def _comb(sign, a, b):
    return [u + v if sign > 0 else u - v for u, v in zip(a, b)]


def _heads(m, rows=(0,)):
    return [m[r:r + 8, k * 128:(k + 1) * 128] for k in range(m.shape[1] // 128) for r in rows]


def _kernel(x_hbm, lre_hbm, lim_hbm, bre_hbm, bim_hbm, cre_hbm, cim_hbm, ldt_hbm, dsk_hbm,
            w1_hbm, b1_hbm, w2_hbm, b2_hbm, o_hbm,
            x_s, o_s, bu_s, xn_s, bw_s, bt_s, c_s, ct_s, cw_s, w1_s, w2_s, w1x_s, w2x_s,
            lam_s, carry_s, col_s, coef_s, cm_s, h_s, a_s, s_s, bx_s, lx_s, m_s, st_s, zero_s, zsrc_s,
            lre_s, lim_s, ldt_s, dsk_s, b1_s, b2_s,
            xsem, osem, wsem):
    ta, tb = TA, TB
    na, D, _ = x_s.shape
    nb = o_s.shape[0]
    P = lre_s.shape[0]
    R = tb // ta
    NF = w1_s.shape[0]
    NFH = NF // 2
    FH = NFH * 128
    NK = D // 128
    DP = pl.cdiv(D, 128) * 128
    DH = D // 2
    KP = pl.cdiv(DH, 128) * 128
    KA = 256
    KB = D - KA
    H = tb // 2
    HA = ta // 2
    Q = tb // 8 + 1
    QL = tb - 7 * Q
    NA = P // 128
    PA = NA * 128
    PB = P - PA
    NB = 2 * NA + 1
    W = (NB + 1) * 128
    E = 256

    def x_copy(j):
        return pltpu.make_async_copy(x_hbm.at[:, pl.ds(j * ta, ta)], x_s.at[j], xsem.at[j])

    def o_copy(j, lo=0, hi=tb, r0=0, r1=D):
        return pltpu.make_async_copy(o_s.at[j, r0:r1, lo:hi],
                                     o_hbm.at[r0:r1, pl.ds(j * tb + lo, hi - lo)], osem)

    def b_copy(src, r0, r1, d0, sem):
        cs = [pltpu.make_async_copy(src.at[r0:r1, k * 128:(k + 1) * 128], bw_s.at[k, d0:d0 + r1 - r0, :], sem)
              for k in range(NK)]
        return cs + [pltpu.make_async_copy(src.at[r0:r1, NK * 128:D], bt_s.at[d0:d0 + r1 - r0, :], sem)]

    vec_copies = [pltpu.make_async_copy(src, dst, wsem.at[3]) for src, dst in
                  ((lre_hbm, lre_s), (lim_hbm, lim_s), (ldt_hbm, ldt_s), (dsk_hbm, dsk_s),
                   (b1_hbm, b1_s), (b2_hbm, b2_s))]
    z_copy = pltpu.make_async_copy(zsrc_s, zero_s, wsem.at[3])
    b0_copies = b_copy(bre_hbm, 0, E, 0, wsem.at[0]) + b_copy(bim_hbm, 0, E, PA, wsem.at[0])
    b1_copies = (b_copy(bre_hbm, E, PA, E, wsem.at[1]) + b_copy(bim_hbm, E, PA, PA + E, wsem.at[1])
                 + b_copy(bre_hbm, PA, P, 2 * PA, wsem.at[1]) + b_copy(bim_hbm, PA, P, 2 * PA + PB, wsem.at[1]))
    w1_copies = [pltpu.make_async_copy(w1_hbm.at[:, k * 128:(k + 1) * 128], w1_s.at[k, 0:D, :], wsem.at[4])
                 for k in range(NF)]
    w2_copies = [pltpu.make_async_copy(w2_hbm.at[:, k * 128:(k + 1) * 128], w2_s.at[k], wsem.at[2])
                 for k in range(NF)]
    c_copies = [pltpu.make_async_copy(src.at[:, k * 128:(k + 1) * 128], c_s.at[i * NA + k], wsem.at[2])
                for i, src in enumerate((cre_hbm, cim_hbm)) for k in range(NA)]
    c_copies += [pltpu.make_async_copy(src.at[:, PA:P], ct_s.at[i], wsem.at[2])
                 for i, src in enumerate((cre_hbm, cim_hbm))]

    def gate(val, dep):
        if dep is None:
            return val
        n = val.shape[1]
        w = pl.cdiv(n, 128) * 128
        head = jnp.where(_rep(zero_s[...], w)[:, :n] != 0, _rep(dep, w)[:, :n], val[0:8, :])
        return head if val.shape[0] == 8 else jnp.concatenate([head, val[8:, :]], axis=0)

    def gate_row(val, dep):
        if dep is None:
            return val
        w = val.shape[1]
        return jnp.where(_rep(zero_s[0:1, :], w) != 0, _rep(dep[0:1, :], w), val)

    def gate_all(val, dep):
        n, w = val.shape[0] // 8, pl.cdiv(val.shape[1], 128) * 128
        z = jnp.concatenate([_rep(zero_s[...], w)] * n, axis=0)[:, :val.shape[1]]
        d = jnp.concatenate([_rep(pltpu.bitcast(dep, val.dtype), w)] * n, axis=0)[:, :val.shape[1]]
        return jnp.where(z != 0, d, val)

    def b_words(r0, r1, k0, k1):
        rs = slice(r0 // 2, r1 // 2)
        parts = [bw_s.bitcast(U32)[k, rs, :] if k < NK else bt_s.bitcast(U32)[rs, :] for k in range(k0, k1)]
        return jnp.concatenate(parts, axis=1)

    def wblk(ref, half, r0, r1):
        r32 = ref.bitcast(U32)
        return pltpu.bitcast(
            jnp.concatenate([r32[half * NFH + k, r0 // 2:r1 // 2, :] for k in range(NFH)], axis=1), BF16)

    def xblk(ref, i, r0=0, r1=None):
        r1 = 2 * ref.shape[2] if r1 is None else r1
        return pltpu.bitcast(jnp.concatenate([ref[i, k, r0 // 2:r1 // 2, :] for k in range(NFH)], axis=1), BF16)

    def tiles(ref, j, lo, hi):
        parts = []
        for r in range(R):
            a, b = max(lo, r * ta), min(hi, (r + 1) * ta)
            if a < b:
                parts.append(ref[j * R + r, :, a - r * ta:b - r * ta])
        return parts[0] if len(parts) == 1 else jnp.concatenate(parts, axis=1)

    def prep_params():
        lr = _row(lre_s)
        li = _row(lim_s)
        dt = jnp.exp(_row(ldt_s)).astype(BF16).astype(F32)
        mag = jnp.exp(dt * lr)
        ang = dt * li
        lbr = mag * jnp.cos(ang)
        lbi = mag * jnp.sin(ang)
        nr = lbr - 1.0
        den = lr * lr + li * li
        coef_s[...] = jnp.zeros_like(coef_s)
        coef_s[0:1, :] = 2.0 * (nr * lr + lbi * li) / den
        coef_s[1:2, :] = 2.0 * (lbi * lr - nr * li) / den

        def put_lam(k, re, im):
            a = jnp.concatenate([re[:, :PA], re[:, :PA], re[:, PA:], re[:, PA:], re[:, PA:], re[:, PA:]], axis=1)
            b = jnp.concatenate([-im[:, :PA], im[:, :PA], -im[:, PA:], im[:, PA:], im[:, PA:], -im[:, PA:]], axis=1)
            lam_s[2 * k] = jnp.broadcast_to(a, (8, W))
            lam_s[2 * k + 1] = jnp.broadcast_to(b, (8, W))

        put_lam(0, lbr, lbi)
        pr, pi = lbr, lbi
        q = 1
        while q < Q - 1:
            pr, pi = _cmul(pr, pi, pr, pi)
            q *= 2
        assert q == Q - 1
        pr, pi = _cmul(pr, pi, lbr, lbi)
        for k in range(3):
            put_lam(1 + k, pr, pi)
            pr, pi = _cmul(pr, pi, pr, pi)
        carry_s[...] = jnp.zeros_like(carry_s)
        bu_s[:, :, tb:, :] = jnp.zeros((nb, NB + 1, 8, 128), F32)
        row = jax.lax.broadcasted_iota(jnp.int32, (KP - DH, NF * 128), 0)
        pad = pltpu.bitcast(jnp.where(row == 0, _row(b1_s), 0.0).astype(BF16), U32)
        for k in range(NFH):
            w1x_s[0, k, DH // 2:, :] = pad[:, k * 128:(k + 1) * 128]
            w1x_s[1, k, DH // 2:, :] = pad[:, (NFH + k) * 128:(NFH + k + 1) * 128]
        w1x_s[2:5, :, DH // 2:, :] = jnp.zeros((3, NFH, (KP - DH) // 2, 128), U32)
        w1_s[:, D:, :] = jnp.zeros((NF, w1_s.shape[1] - D, 128), BF16)
        for k, r in enumerate((_row(dsk_s), 0.5 * _row(b2_s))):
            r = jnp.concatenate([r, jnp.zeros((1, DP - D), F32)], axis=1)
            col_s[k] = jnp.broadcast_to(r, (128, DP)).T[:D, :]

    def prep_b(q0, deps):
        rows = 32

        def top_bot(r0, dep):
            ws = _unpack2(gate_all(b_words(r0, r0 + rows, 0, NK + 1), dep))
            return ([w[:, :KA] for w in ws],
                    [jnp.concatenate([w[:, KA:], jnp.zeros((rows // 2, KA - KB), F32)], axis=1) for w in ws])

        lane = jax.lax.broadcasted_iota(jnp.int32, (rows // 2, KA), 1)
        cut = lambda a: [jnp.where(lane < KB, u, 0.0) for u in a]
        for q, dep in enumerate(deps):
            r0 = (q0 + q) * rows
            if r0 < PA:
                b11, b21 = top_bot(r0, dep)
                b12, b22 = top_bot(PA + r0, dep)
                outs = [cut(_comb(-1, b21, b11)), _comb(-1, b12, b22), _comb(1, b11, b22),
                        _comb(1, b21, b22), _comb(1, b11, b12)]
            else:
                b1, b2 = top_bot(PA + r0, dep)
                outs = [cut(_comb(-1, b2, b1)), _comb(-1, b1, b2)]
            for i, o in enumerate(outs):
                bx_s[i, r0 // 2:(r0 + rows) // 2, :] = _pack2(o)

    def prep_w(src, dst, specs, deps):
        src32 = src.bitcast(U32)
        per = len(deps) // NFH
        rows = DH // 2 // per
        z = jnp.concatenate([zero_s[...]] * (rows // 8), axis=0) != 0
        for n, dep in enumerate(deps):
            k, q = divmod(n, per)
            d = jnp.concatenate([pltpu.bitcast(dep, U32)] * (rows // 8), axis=0)
            blk = {}
            for r in range(2):
                for c in range(2):
                    r0 = r * DH // 2 + q * rows
                    blk[r, c] = _unpack2(jnp.where(z, d, src32[c * NFH + k, r0:r0 + rows, :]))
            for i, (sign, a, b) in enumerate(specs):
                dst[i, k, q * rows:(q + 1) * rows, :] = _pack2(_comb(sign, blk[a], blk[b]))

    def prep_c(deps):
        rows = DH // 2 // len(deps)
        for q, dep in enumerate(deps):
            cf = gate(coef_s[...], dep)
            cr = cf[0:1, :]
            ci = cf[1:2, :]
            blk = {}
            for r in range(2):
                rs = slice(r * DH // 2 + q * rows, r * DH // 2 + (q + 1) * rows)
                ld = lambda i: jnp.concatenate(
                    [c_s.bitcast(U32)[i * NA + k, rs, :] for k in range(NA)] + [ct_s.bitcast(U32)[i, rs, :]],
                    axis=1)
                c_re = _unpack2(ld(0))
                c_im = _unpack2(ld(1))
                cpr = [a * cr - b * ci for a, b in zip(c_re, c_im)]
                cpi = [-(a * ci) - b * cr for a, b in zip(c_re, c_im)]
                blk[r, 0], blk[r, 1] = [a[:, :PA] for a in cpr], [a[:, :PA] for a in cpi]
                cm_s[rs, :] = _pack2([jnp.concatenate([a[:, PA:], b[:, PA:]], axis=1) for a, b in zip(cpr, cpi)])
            outs = [_comb(sign, blk[a], blk[b]) for sign, a, b in LHS_SUMS] + [blk[1, 1], blk[0, 0]]
            for i, o in enumerate(outs):
                cw_s[i, q * rows:(q + 1) * rows, :] = _pack2(o)

    def ln1(j, lo, hi, deps=(None, None, None)):
        x = gate(x_s[j, :, lo:hi].astype(F32), deps[0])
        m = gate_row(jnp.sum(x, axis=0, keepdims=True) * (1.0 / D), deps[1])
        xc = x - m
        v = jnp.sum(xc * xc, axis=0, keepdims=True) * (1.0 / D)
        xb = (xc * gate_row(jax.lax.rsqrt(v + EPS), deps[2])).astype(BF16)
        xn = xb.astype(F32)
        xn_s[j, :, lo:hi] = xn
        return xb, xn

    def bu_plain(xn, ks):
        rhs = pltpu.bitcast(
            jnp.concatenate([b_words(k * 128, (k + 1) * 128, 0, NK + 1) for k in ks], axis=0), BF16)
        bu = _dot_nt(xn, rhs)
        for i, k in enumerate(ks):
            bu_s[0, k, 0:ta, :] = bu[:, i * 128:(i + 1) * 128]
            if k == NB - 1:
                bu_s[0, NB, 0:ta, :] = pltpu.roll(bu[:, i * 128:(i + 1) * 128], PB, 1)
        return bu

    def bu_operands(xn):
        a11, a12, a21, a22 = xn[:KA, :HA], xn[KA:, :HA], xn[:KA, HA:], xn[KA:, HA:]
        addp = lambda t, b: jnp.concatenate([t[:KB] + b, t[KB:]], axis=0)
        padz = lambda b: jnp.concatenate([b, jnp.zeros((KA - KB, HA), F32)], axis=0)
        ops = (addp(a21, a22), padz(a11[:KB] + a12), padz(a22), a11, addp(a11, a22), padz(a12 - a22), a21 - a11)
        return [o.astype(BF16).T for o in ops]

    def bu_lo(l2, l5):
        r2 = pltpu.bitcast(jnp.concatenate([b_words(0, PA, 0, 2), b_words(2 * PA, 2 * P, 0, 2)], axis=0), BF16)
        r5 = pltpu.bitcast(b_words(PA, 2 * P, 2, NK + 1), BF16)
        return _dot_nt(l2, r2), _dot_nt(l5[:, :KB], r5)

    def bu_hi(base, off, m2, m5, ls):
        jb = base + off // R
        r0 = (off % R) * ta
        mm = lambda i, rows: _dot_nt(ls[i], pltpu.bitcast(bx_s[i, 0:rows // 2, :], BF16))

        def put(half, k0, val):
            rows = pl.ds(r0 + half * HA, HA)
            for k in range(NA):
                bu_s[jb, k0 + k, rows, :] = val[:, k * 128:(k + 1) * 128]
            if val.shape[1] > PA:
                bu_s[jb, NB - 1, rows, :] = val[:, PA:]
                bu_s[jb, NB, rows, :] = pltpu.roll(val[:, PA:], PB, 1)

        m4 = mm(0, PA + 128)
        put(1, 0, m2 + m4)
        m3 = mm(1, PA + 128)
        put(0, NA, m3 + m5)
        m1 = mm(2, PA)
        u = m1 + m4[:, :PA] - m5[:, :PA]
        v = m1 - m2[:, :PA] + m3[:, :PA]
        m7 = mm(3, PA)
        put(0, 0, u + m7)
        m6 = mm(4, PA)
        put(1, NA, v + m6)
        return [m4, m3, m1, m7, m6]

    def stash(m2, m5, ls):
        m_s[0] = m2
        m_s[1] = m5
        for i in range(5):
            lx_s[i] = pltpu.bitcast(ls[2 + i], U32)

    def finish(base, off):
        return bu_hi(base, off, m_s[0], m_s[1], [pltpu.bitcast(lx_s[i], BF16) for i in range(5)])

    def phase_a_pair(base, lng):
        j = base * R + 1
        res = finish(base, 1)
        ls = bu_operands(ln1(j + 1, 0, ta)[1])
        cur = list(bu_lo(ls[0], ls[1]))
        cur += bu_hi(base, 2, cur[0], cur[1], ls[2:])
        ev = [e for m in cur for e in _heads(m)]
        xn = jnp.concatenate([ln1(j + 2, k * 128, (k + 1) * 128, [ev[g] for g in lng[k]])[1]
                              for k in range(ta // 128)], axis=1)
        ls = bu_operands(xn)
        m2, m5 = bu_lo(ls[0], ls[1])
        stash(m2, m5, ls)
        return res + cur + [m2, m5]

    def ln2_stats(j, deps):
        for k in range(tb // 128):
            xs = gate(tiles(xn_s, j, k * 128, (k + 1) * 128), deps[k])
            m = jnp.sum(xs, axis=0, keepdims=True) * (1.0 / D)
            v = jnp.sum(xs * xs, axis=0, keepdims=True) * (1.0 / D) - m * m
            r = jax.lax.rsqrt(v + EPS)
            st_s[0:8, k * 128:(k + 1) * 128] = jnp.broadcast_to(r, (8, 128))
            st_s[8:16, k * 128:(k + 1) * 128] = jnp.broadcast_to(m * r, (8, 128))

    def mlp_up(j):
        st = st_s[...]
        yT = tiles(xn_s, j, 0, tb) * st[0:1, :] - st[8:9, :]
        a11, a12, a21, a22 = yT[:DH, :H], yT[DH:, :H], yT[:DH, H:], yT[DH:, H:]
        row = jax.lax.broadcasted_iota(jnp.int32, (KP - DH, H), 0)
        zeros = jnp.zeros((KP - DH, H), F32)
        ones = jnp.where(row == 0, 1.0, 0.0).astype(F32)

        def mm(lhsT, rhs, pad=zeros):
            lhs = jnp.concatenate([lhsT, pad], axis=0).astype(BF16).T
            return jnp.dot(lhs, rhs, preferred_element_type=F32)

        def act(r, c, x):
            t = jnp.tanh(x * (x * x * GELU_C1 + GELU_C0))
            a_s[r * H:(r + 1) * H, c * FH:(c + 1) * FH] = x + x * t

        m2 = mm(a21 + a22, wblk(w1_s, 0, 0, KP))
        m4 = mm(a22, xblk(w1x_s, 0), ones)
        act(1, 0, m2 + m4)
        m5 = mm(a11 + a12, wblk(w1_s, 1, DH, DH + KP))
        m3 = mm(a11, xblk(w1x_s, 1), ones)
        act(0, 1, m3 + m5)
        m1 = mm(a11 + a22, xblk(w1x_s, 2))
        u = m1 + m4 - m5
        v = m1 - m2 + m3
        m7 = mm(a12 - a22, xblk(w1x_s, 3))
        act(0, 0, u + m7)
        m6 = mm(a21 - a11, xblk(w1x_s, 4))
        act(1, 1, v + m6)
        return [e for m in (m2, m4, m5, m3, m1, m7, m6) for e in _heads(m)]

    def scan(j, dep):
        row = jax.lax.broadcasted_iota(jnp.int32, (8, 128), 0)
        for ka, kb in [(k, NA + k) for k in range(NA)] + [(NB - 1, NB)]:
            sa = slice(ka * 128, (ka + 1) * 128)
            sb = slice(kb * 128, (kb + 1) * 128)
            la = lam_s[0, :, sa]
            lba = lam_s[1, :, sa]
            lbb = lam_s[1, :, sb]
            ca = gate(carry_s[:, sa], dep)
            cb = carry_s[:, sb]

            def step(u, v, i):
                bu = bu_s[j, ka, pl.ds(i, 8, stride=Q), :]
                bv = bu_s[j, kb, pl.ds(i, 8, stride=Q), :]
                return (la * u + bu) + lba * v, (la * v + bv) + lbb * u

            u, v = ca, cb
            for i in range(Q):
                u, v = step(u, v, i)
            for k in range(3):
                sh = 1 << k
                us = jnp.where(row >= sh, pltpu.roll(u, sh, 0), 0.0)
                vs = jnp.where(row >= sh, pltpu.roll(v, sh, 0), 0.0)
                pa = lam_s[2 + 2 * k, :, sa]
                u, v = (u + pa * us + lam_s[3 + 2 * k, :, sa] * vs,
                        v + pa * vs + lam_s[3 + 2 * k, :, sb] * us)
            u = jnp.where(row == 0, ca, pltpu.roll(u, 1, 0))
            v = jnp.where(row == 0, cb, pltpu.roll(v, 1, 0))
            for i in range(Q):
                u, v = step(u, v, i)
                if i == QL - 1:
                    carry_s[:, sa] = jnp.where(row == 0, pltpu.roll(u, 1, 0), 0.0)
                    carry_s[:, sb] = jnp.where(row == 0, pltpu.roll(v, 1, 0), 0.0)
                h_s[ka, pl.ds(i, 8, stride=Q), :] = u
                if kb < NB:
                    h_s[kb, pl.ds(i, 8, stride=Q), :] = v
            dep = u

    def ssm_out(j, split=False):
        g = lambda r, c: jnp.concatenate([h_s[c * NA + k, r * H:(r + 1) * H, :] for k in range(NA)], axis=1)
        parts = []

        def mm(i, rhs):
            lhs = pltpu.bitcast(cw_s[i], BF16)
            rhs = rhs.astype(BF16)
            if not split:
                return _dot_nt(lhs, rhs)
            cols = []
            for n in range(H // 128):
                acc = None
                for k in range(NA):
                    p = _dot_nt(lhs[:, k * 128:(k + 1) * 128], rhs[n * 128:(n + 1) * 128, k * 128:(k + 1) * 128])
                    parts.append(p)
                    acc = p if acc is None else acc + p
                cols.append(acc)
            return jnp.concatenate(cols, axis=1)

        z = _dot_nt(pltpu.bitcast(cm_s[...], BF16), h_s[NB - 1, :tb, :].astype(BF16))
        z = z + tiles(xn_s, j, 0, tb) * _rep(col_s[0], tb)
        n2 = mm(0, g(0, 0))
        n4 = mm(5, g(0, 1) - g(0, 0))
        s_s[DH:, :H] = z[DH:, :H] + (n2 + n4)
        n5 = mm(1, g(1, 1))
        n3 = mm(6, g(1, 0) - g(1, 1))
        s_s[:DH, H:] = z[:DH, H:] + (n3 + n5)
        n1 = mm(2, g(0, 0) + g(1, 1))
        u = z[:DH, :H] + n1 + n4 - n5
        v = z[DH:, H:] + n1 - n2 + n3
        s_s[:DH, :H] = u + mm(3, g(0, 1) + g(1, 1))
        s_s[DH:, H:] = v + mm(4, g(0, 0) + g(1, 0))
        return parts

    last_pieces = ((0, 0, DH), (128, 0, 128), (128, 128, DH))

    def mlp_down(j, last=False):
        g = lambda r, c: a_s[r * H:(r + 1) * H, c * FH:(c + 1) * FH]
        mm = lambda lhs, rhs: _dot_nt(lhs, rhs.astype(BF16))

        def fin(r0, lo, oT):
            r1, hi = r0 + oT.shape[0], lo + oT.shape[1]
            h = oT * 0.25 + _rep(col_s[1, r0:r1, :], hi - lo)
            gt = h + h * jnp.tanh(h)
            o_s[j, r0:r1, lo:hi] = tiles(x_s, j, lo, hi)[r0:r1].astype(F32) + s_s[r0:r1, lo:hi] * gt
            if last:
                o_copy(j, lo, hi, r0, r1).start()

        n2 = mm(xblk(w2x_s, 0), g(0, 0))
        n4 = mm(wblk(w2_s, 1, DH, D), g(0, 1) - g(0, 0))
        fin(DH, 0, n2 + n4)
        n5 = mm(xblk(w2x_s, 1), g(1, 1))
        n3 = mm(wblk(w2_s, 0, 0, DH), g(1, 0) - g(1, 1))
        fin(0, H, n3 + n5)
        n1 = mm(xblk(w2x_s, 2), g(0, 0) + g(1, 1))
        u = n1 + n4 - n5
        v = n1 - n2 + n3
        n7 = mm(xblk(w2x_s, 3), g(0, 1) + g(1, 1))
        fin(0, 0, u + n7)
        s6 = g(0, 0) + g(1, 0)
        if not last:
            fin(DH, H, v + mm(xblk(w2x_s, 4), s6))
        else:
            for lo, r0, r1 in last_pieces:
                fin(DH + r0, H + lo, v[r0:r1, lo:lo + 128] + mm(xblk(w2x_s, 4, r0, r1), s6[lo:lo + 128, :]))
        return [e for n in (n2, n4, n5, n3, n1, n7) for e in _heads(n)]

    for c in vec_copies:
        c.start()
    x_copy(0).start()
    for c in b0_copies:
        c.start(priority=1)
    zsrc_s[...] = jnp.zeros_like(zsrc_s)
    z_copy.start()
    for c in vec_copies + [z_copy]:
        c.wait()
    for c in b1_copies:
        c.start(priority=1)
    x_copy(1).start(priority=1)
    prep_params()
    x_copy(0).wait()
    xn0 = ln1(0, 0, ta)[0].T
    for c in b0_copies:
        c.wait()
    for j in range(2, na):
        x_copy(j).start(priority=1)
    ev = _heads(bu_plain(xn0, (0, 1, NA, NA + 1)), (0, 64, 128, 192))
    prep_b(0, [ev[k] for k in EVB0])
    for c in b1_copies:
        c.wait()
    for c in w1_copies + c_copies + w2_copies:
        c.start(priority=1)

    x_copy(1).wait()
    bu0 = bu_plain(xn0, (2, NA + 2, NB - 1))
    ls = bu_operands(ln1(1, 0, ta)[1])
    m2, m5 = bu_lo(ls[0], ls[1])
    stash(m2, m5, ls)
    ev = _heads(bu0, (0, 64, 128, 192)) + _heads(m2) + _heads(m5)
    prep_b(E // 32, [ev[k] for k in EVB])

    def body_a(i, carry):
        x_copy(2 * i + 2).wait()
        x_copy(2 * i + 3).wait()
        phase_a_pair(i, LNG)
        return carry

    jax.lax.fori_loop(0, nb - 2, body_a, 0)

    x_copy(na - 2).wait()
    x_copy(na - 1).wait()
    for c in w1_copies:
        c.wait()
    ev = [e for m in phase_a_pair(nb - 2, LNGL) for e in _heads(m, (0, 64))]
    prep_w(w1_s, w1x_s, RHS_SUMS, [ev[k] for k in EVS])

    for c in c_copies + w2_copies:
        c.wait()
    finish(0, na - 1)
    ln2_stats(0, [None] * (tb // 128))
    ev = mlp_up(0)
    prep_c([ev[k] for k in CPK])
    scan(0, ev[GS0])
    parts = ssm_out(0, split=True)
    ev = [e for i in EV2[0] for e in _heads(parts[i], EV2[1])]
    prep_w(w2_s, w2x_s, LHS_SUMS, ev[:7 * NFH])

    def body_b(j, carry):
        ev = mlp_down(j)
        ln2_stats(j + 1, [ev[k] for k in STG])
        mlp_up(j + 1)
        scan(j + 1, ev[GS])
        ssm_out(j + 1)
        o_copy(j).start()
        return carry

    jax.lax.fori_loop(0, nb - 1, body_b, 0)

    mlp_down(nb - 1, last=True)
    for j in range(nb - 1):
        o_copy(j).wait()
    for lo, hi, r0, r1 in ((0, H, DH, D), (H, tb, 0, DH), (0, H, 0, DH)):
        o_copy(nb - 1, lo, hi, r0, r1).wait()
    for lo, r0, r1 in last_pieces:
        o_copy(nb - 1, H + lo, H + lo + 128, DH + r0, DH + r1).wait()


@jax.jit
def pallas_recurrent_scan__ssm_conv_s5__mixer_channel_mlp__prompt_kernel(
    A_x, A_Lambda_re, A_Lambda_im, A_B_re, A_B_im, A_C_re, A_C_im, A_log_dt, A_Dskip,
    B_x, B_w1, B_b1, B_w2, B_b2,
):
    Bsz, L, D = A_x.shape
    P = A_Lambda_re.shape[0]
    F = B_w1.shape[1]
    assert (Bsz, L, D, P, F) == (1, 2048, 448, 448, 1792)
    ta, tb = TA, TB
    na, nb = L // ta, L // tb
    NF, NA = F // 128, P // 128
    DH = D // 2
    KP = pl.cdiv(DH, 128) * 128
    outT = pl.pallas_call(
        _kernel,
        in_specs=[pl.BlockSpec(memory_space=pl.ANY)] * 13,
        out_specs=pl.BlockSpec(memory_space=pl.ANY),
        out_shape=jax.ShapeDtypeStruct((D, L), F32),
        scratch_shapes=[
            pltpu.VMEM((na, D, ta), BF16),
            pltpu.VMEM((nb, D, tb), F32),
            pltpu.VMEM((nb, 2 * NA + 2, tb + 8, 128), F32),
            pltpu.VMEM((na, D, ta), F32),
            pltpu.VMEM((D // 128, 2 * P, 128), BF16),
            pltpu.VMEM((2 * P, D % 128), BF16),
            pltpu.VMEM((2 * NA, D, 128), BF16),
            pltpu.VMEM((2, D, P % 128), BF16),
            pltpu.VMEM((7, DH // 2, NA * 128), U32),
            pltpu.VMEM((NF, DH + KP, 128), BF16),
            pltpu.VMEM((NF, D, 128), BF16),
            pltpu.VMEM((5, NF // 2, KP // 2, 128), U32),
            pltpu.VMEM((5, NF // 2, DH // 2, 128), U32),
            pltpu.VMEM((8, 8, (2 * NA + 2) * 128), F32),
            pltpu.VMEM((8, (2 * NA + 2) * 128), F32),
            pltpu.VMEM((2, D, 128), F32),
            pltpu.VMEM((8, P), F32),
            pltpu.VMEM((D // 2, 128), U32),
            pltpu.VMEM((2 * NA + 1, tb + 8, 128), F32),
            pltpu.VMEM((tb, F), F32),
            pltpu.VMEM((D, tb), F32),
            pltpu.VMEM((5, (NA + 1) * 64, 256), U32),
            pltpu.VMEM((5, ta // 4, 256), U32),
            pltpu.VMEM((2, ta // 2, (NA + 1) * 128), F32),
            pltpu.VMEM((16, tb), F32),
            pltpu.VMEM((8, 128), jnp.int32),
            pltpu.VMEM((8, 128), jnp.int32),
            pltpu.VMEM((P,), BF16), pltpu.VMEM((P,), BF16), pltpu.VMEM((P,), BF16),
            pltpu.VMEM((D,), BF16), pltpu.VMEM((F,), BF16), pltpu.VMEM((D,), BF16),
            pltpu.SemaphoreType.DMA((na,)),
            pltpu.SemaphoreType.DMA(()),
            pltpu.SemaphoreType.DMA((5,)),
        ],
        compiler_params=pltpu.CompilerParams(
            vmem_limit_bytes=100 * 1024 * 1024,
            disable_semaphore_checks=True, disable_bounds_checks=True),
    )(A_x.reshape(L, D).T, A_Lambda_re, A_Lambda_im, A_B_re, A_B_im, A_C_re, A_C_im,
      A_log_dt, A_Dskip, B_w1, B_b1, B_w2.T, B_b2)
    return outT.T.reshape(Bsz, L, D)
```

```python
import jax
import jax.numpy as jnp
import jax.experimental.pallas as pl
import jax.experimental.pallas.tpu as pltpu

F32 = jnp.float32
BF16 = jnp.bfloat16
U32 = jnp.uint32
NT = (((1,), (1,)), ((), ()))
EPS = 1e-5
GELU_C0 = 0.7978845608028654
GELU_C1 = 0.7978845608028654 * 0.044715

TA = 256
TB = 512

EVB0 = (0,1,2,4,5,6,8,9)
EVB = (6,7,10,12,14,15,16,18)
LNG = ((0,2,12),(0,2,5))
LNGL = ((0,3,11),(0,1,14))
EVS = (45,46,47,48,49,50,51,52,53,54,55,56,57,59,60,61,62,63,64,65,66,67,68,69,70,72,73,74,75,76,77,78,79,80,81,82,83,85,86,87,88,89,90,91,92,93,94,95,96)
CPK = (0,1,2,3,4,5,6,28,29,30,31,32,33,34)
GS0 = 4
EV2 = ((3,7,11,15,19,23,27,31,35,39),(0,40,80,120,160))
STG = (0,1,9,10)
GS = 0

RHS_SUMS = ((-1, (1, 0), (0, 0)), (-1, (0, 1), (1, 1)), (1, (0, 0), (1, 1)), (1, (1, 0), (1, 1)), (1, (0, 0), (0, 1)))
LHS_SUMS = ((1, (1, 0), (1, 1)), (1, (0, 0), (0, 1)), (1, (0, 0), (1, 1)), (-1, (0, 1), (1, 1)), (-1, (1, 0), (0, 0)))


def _cmul(ar, ai, br, bi):
    return ar * br - ai * bi, ar * bi + ai * br


def _row(ref):
    return ref[...].astype(F32).reshape(1, ref.shape[0])


def _rep(c, w):
    return c if w == 128 else jnp.concatenate([c] * (w // 128), axis=1)


def _dot_nt(a, b):
    return jax.lax.dot_general(a, b, NT, preferred_element_type=F32)


def _unpack(w):
    return pltpu.bitcast(w, BF16).astype(F32)


def _pack(x):
    return pltpu.bitcast(x.astype(BF16), U32)


def _comb(sign, a, b):
    return a + b if sign > 0 else a - b


def _heads(m, rows=(0,)):
    return [m[r:r + 8, k * 128:(k + 1) * 128] for k in range(m.shape[1] // 128) for r in rows]


def _kernel(x_hbm, lre_hbm, lim_hbm, bre_hbm, bim_hbm, cre_hbm, cim_hbm, ldt_hbm, dsk_hbm,
            w1_hbm, b1_hbm, w2_hbm, b2_hbm, o_hbm,
            x_s, o_s, bu_s, xn_s, bw_s, bt_s, c_s, ct_s, cw_s, w1_s, w2_s, w1x_s, w2x_s,
            lam_s, carry_s, col_s, coef_s, cm_s, h_s, a_s, s_s, bx_s, lx_s, m_s, st_s, zero_s, zsrc_s,
            lre_s, lim_s, ldt_s, dsk_s, b1_s, b2_s,
            xsem, osem, wsem):
    ta, tb = TA, TB
    na, D, _ = x_s.shape
    nb = o_s.shape[0]
    P = lre_s.shape[0]
    R = tb // ta
    NF = w1_s.shape[0]
    NFH = NF // 2
    FH = NFH * 128
    NK = D // 128
    DP = pl.cdiv(D, 128) * 128
    DH = D // 2
    KP = pl.cdiv(DH, 128) * 128
    KA = 256
    KB = D - KA
    H = tb // 2
    HA = ta // 2
    Q = tb // 8 + 1
    QL = tb - 7 * Q
    NA = P // 128
    PA = NA * 128
    PB = P - PA
    NB = 2 * NA + 1
    W = (NB + 1) * 128
    E = 256

    def x_copy(j):
        return pltpu.make_async_copy(x_hbm.at[:, pl.ds(j * ta, ta)], x_s.at[j], xsem.at[j])

    def o_copy(j, lo=0, hi=tb, r0=0, r1=D):
        return pltpu.make_async_copy(o_s.at[j, r0:r1, lo:hi],
                                     o_hbm.at[r0:r1, pl.ds(j * tb + lo, hi - lo)], osem)

    def b_copy(src, r0, r1, d0, sem):
        cs = [pltpu.make_async_copy(src.at[r0:r1, k * 128:(k + 1) * 128], bw_s.at[k, d0:d0 + r1 - r0, :], sem)
              for k in range(NK)]
        return cs + [pltpu.make_async_copy(src.at[r0:r1, NK * 128:D], bt_s.at[d0:d0 + r1 - r0, :], sem)]

    vec_copies = [pltpu.make_async_copy(src, dst, wsem.at[3]) for src, dst in
                  ((lre_hbm, lre_s), (lim_hbm, lim_s), (ldt_hbm, ldt_s), (dsk_hbm, dsk_s),
                   (b1_hbm, b1_s), (b2_hbm, b2_s))]
    z_copy = pltpu.make_async_copy(zsrc_s, zero_s, wsem.at[3])
    b0_copies = b_copy(bre_hbm, 0, E, 0, wsem.at[0]) + b_copy(bim_hbm, 0, E, PA, wsem.at[0])
    b1_copies = (b_copy(bre_hbm, E, PA, E, wsem.at[1]) + b_copy(bim_hbm, E, PA, PA + E, wsem.at[1])
                 + b_copy(bre_hbm, PA, P, 2 * PA, wsem.at[1]) + b_copy(bim_hbm, PA, P, 2 * PA + PB, wsem.at[1]))
    w1_copies = [pltpu.make_async_copy(w1_hbm.at[:, k * 128:(k + 1) * 128], w1_s.at[k, 0:D, :], wsem.at[4])
                 for k in range(NF)]
    w2_copies = [pltpu.make_async_copy(w2_hbm.at[:, k * 128:(k + 1) * 128], w2_s.at[k], wsem.at[2])
                 for k in range(NF)]
    c_copies = [pltpu.make_async_copy(src.at[:, k * 128:(k + 1) * 128], c_s.at[i * NA + k], wsem.at[2])
                for i, src in enumerate((cre_hbm, cim_hbm)) for k in range(NA)]
    c_copies += [pltpu.make_async_copy(src.at[:, PA:P], ct_s.at[i], wsem.at[2])
                 for i, src in enumerate((cre_hbm, cim_hbm))]

    def gate(val, dep):
        if dep is None:
            return val
        n = val.shape[1]
        w = pl.cdiv(n, 128) * 128
        head = jnp.where(_rep(zero_s[...], w)[:, :n] != 0, _rep(dep, w)[:, :n], val[0:8, :])
        return head if val.shape[0] == 8 else jnp.concatenate([head, val[8:, :]], axis=0)

    def gate_row(val, dep):
        if dep is None:
            return val
        w = val.shape[1]
        return jnp.where(_rep(zero_s[0:1, :], w) != 0, _rep(dep[0:1, :], w), val)

    def gate_all(val, dep):
        n, w = val.shape[0] // 8, pl.cdiv(val.shape[1], 128) * 128
        z = jnp.concatenate([_rep(zero_s[...], w)] * n, axis=0)[:, :val.shape[1]]
        d = jnp.concatenate([_rep(pltpu.bitcast(dep, val.dtype), w)] * n, axis=0)[:, :val.shape[1]]
        return jnp.where(z != 0, d, val)

    def b_words(r0, r1, k0, k1):
        rs = slice(r0 // 2, r1 // 2)
        parts = [bw_s.bitcast(U32)[k, rs, :] if k < NK else bt_s.bitcast(U32)[rs, :] for k in range(k0, k1)]
        return jnp.concatenate(parts, axis=1)

    def wblk(ref, half, r0, r1):
        r32 = ref.bitcast(U32)
        return pltpu.bitcast(
            jnp.concatenate([r32[half * NFH + k, r0 // 2:r1 // 2, :] for k in range(NFH)], axis=1), BF16)

    def xblk(ref, n, i, r0=0, r1=None):
        rows = ref.shape[0] // n
        r1 = 2 * rows if r1 is None else r1
        return pltpu.bitcast(ref[i * rows + r0 // 2:i * rows + r1 // 2, :], BF16)

    def tiles(ref, j, lo, hi):
        parts = []
        for r in range(R):
            a, b = max(lo, r * ta), min(hi, (r + 1) * ta)
            if a < b:
                parts.append(ref[j * R + r, :, a - r * ta:b - r * ta])
        return parts[0] if len(parts) == 1 else jnp.concatenate(parts, axis=1)

    def prep_params():
        lr = _row(lre_s)
        li = _row(lim_s)
        dt = jnp.exp(_row(ldt_s)).astype(BF16).astype(F32)
        mag = jnp.exp(dt * lr)
        ang = dt * li
        lbr = mag * jnp.cos(ang)
        lbi = mag * jnp.sin(ang)
        nr = lbr - 1.0
        den = lr * lr + li * li
        coef_s[...] = jnp.zeros_like(coef_s)
        coef_s[0:1, :] = 2.0 * (nr * lr + lbi * li) / den
        coef_s[1:2, :] = 2.0 * (lbi * lr - nr * li) / den

        def put_lam(k, re, im):
            a = jnp.concatenate([re[:, :PA], re[:, :PA], re[:, PA:], re[:, PA:], re[:, PA:], re[:, PA:]], axis=1)
            b = jnp.concatenate([-im[:, :PA], im[:, :PA], -im[:, PA:], im[:, PA:], im[:, PA:], -im[:, PA:]], axis=1)
            lam_s[2 * k] = jnp.broadcast_to(a, (8, W))
            lam_s[2 * k + 1] = jnp.broadcast_to(b, (8, W))

        put_lam(0, lbr, lbi)
        pr, pi = lbr, lbi
        q = 1
        while q < Q - 1:
            pr, pi = _cmul(pr, pi, pr, pi)
            q *= 2
        assert q == Q - 1
        pr, pi = _cmul(pr, pi, lbr, lbi)
        for k in range(3):
            put_lam(1 + k, pr, pi)
            pr, pi = _cmul(pr, pi, pr, pi)
        carry_s[...] = jnp.zeros_like(carry_s)
        bu_s[:, :, tb:, :] = jnp.zeros((nb, NB + 1, 8, 128), F32)
        row = jax.lax.broadcasted_iota(jnp.int32, (KP - DH, NF * 128), 0)
        pad = pltpu.bitcast(jnp.where(row == 0, _row(b1_s), 0.0).astype(BF16), U32)
        for i in range(5):
            rs = slice((i * KP + DH) // 2, (i + 1) * KP // 2)
            w1x_s[rs, :] = pad[:, i * FH:(i + 1) * FH] if i < 2 else jnp.zeros(((KP - DH) // 2, FH), U32)
        w1_s[:, D:, :] = jnp.zeros((NF, w1_s.shape[1] - D, 128), BF16)
        for k, r in enumerate((_row(dsk_s), 0.5 * _row(b2_s))):
            r = jnp.concatenate([r, jnp.zeros((1, DP - D), F32)], axis=1)
            col_s[k] = jnp.broadcast_to(r, (128, DP)).T[:D, :]

    def prep_b(q0, deps):
        rows = 32

        def top_bot(r0, dep):
            w = _unpack(gate_all(b_words(r0, r0 + rows, 0, NK + 1), dep))
            return w[:, :KA], jnp.concatenate([w[:, KA:], jnp.zeros((rows, KA - KB), F32)], axis=1)

        lane = jax.lax.broadcasted_iota(jnp.int32, (rows, KA), 1)
        cut = lambda a: jnp.where(lane < KB, a, 0.0)
        for q, dep in enumerate(deps):
            r0 = (q0 + q) * rows
            if r0 < PA:
                b11, b21 = top_bot(r0, dep)
                b12, b22 = top_bot(PA + r0, dep)
                outs = [cut(b21 - b11), b12 - b22, b11 + b22, b21 + b22, b11 + b12]
            else:
                b1, b2 = top_bot(PA + r0, dep)
                outs = [cut(b2 - b1), b1 - b2]
            for i, o in enumerate(outs):
                bx_s[(i * (PA + 128) + r0) // 2:(i * (PA + 128) + r0 + rows) // 2, :] = _pack(o)

    def prep_w(src, dst, specs, deps):
        src32 = src.bitcast(U32)
        per = len(deps) // NFH
        rows = DH // 2 // per
        z = jnp.concatenate([zero_s[...]] * (rows // 8), axis=0) != 0
        for n, dep in enumerate(deps):
            k, q = divmod(n, per)
            d = jnp.concatenate([pltpu.bitcast(dep, U32)] * (rows // 8), axis=0)
            blk = {}
            for r in range(2):
                for c in range(2):
                    r0 = r * DH // 2 + q * rows
                    blk[r, c] = _unpack(jnp.where(z, d, src32[c * NFH + k, r0:r0 + rows, :]))
            for i, (sign, a, b) in enumerate(specs):
                r0 = i * (dst.shape[0] // 5) + q * rows
                dst[r0:r0 + rows, k * 128:(k + 1) * 128] = _pack(_comb(sign, blk[a], blk[b]))

    def prep_c(deps):
        rows = DH // 2 // len(deps)
        for q, dep in enumerate(deps):
            cf = gate(coef_s[...], dep)
            cr = cf[0:1, :]
            ci = cf[1:2, :]
            blk = {}
            for r in range(2):
                rs = slice(r * DH // 2 + q * rows, r * DH // 2 + (q + 1) * rows)
                ld = lambda i: jnp.concatenate(
                    [c_s.bitcast(U32)[i * NA + k, rs, :] for k in range(NA)] + [ct_s.bitcast(U32)[i, rs, :]],
                    axis=1)
                c_re = _unpack(ld(0))
                c_im = _unpack(ld(1))
                cpr = c_re * cr - c_im * ci
                cpi = -(c_re * ci) - c_im * cr
                blk[r, 0], blk[r, 1] = cpr[:, :PA], cpi[:, :PA]
                cm_s[rs, 0:128] = _pack(jnp.concatenate([cpr[:, PA:], cpi[:, PA:]], axis=1))
            outs = [_comb(sign, blk[a], blk[b]) for sign, a, b in LHS_SUMS] + [blk[1, 1], blk[0, 0]]
            for i, o in enumerate(outs):
                cw_s[i * DH // 2 + q * rows:i * DH // 2 + (q + 1) * rows, :] = _pack(o)

    def ln1(j, lo, hi, deps=(None, None, None)):
        x = gate(x_s[j, :, lo:hi].astype(F32), deps[0])
        m = gate_row(jnp.sum(x, axis=0, keepdims=True) * (1.0 / D), deps[1])
        xc = x - m
        v = jnp.sum(xc * xc, axis=0, keepdims=True) * (1.0 / D)
        xb = (xc * gate_row(jax.lax.rsqrt(v + EPS), deps[2])).astype(BF16)
        xn = xb.astype(F32)
        xn_s[j, :, lo:hi] = xn
        return xb, xn

    def bu_plain(xn, ks):
        rhs = pltpu.bitcast(
            jnp.concatenate([b_words(k * 128, (k + 1) * 128, 0, NK + 1) for k in ks], axis=0), BF16)
        bu = _dot_nt(xn, rhs)
        for i, k in enumerate(ks):
            bu_s[0, k, 0:ta, :] = bu[:, i * 128:(i + 1) * 128]
            if k == NB - 1:
                bu_s[0, NB, 0:ta, :] = pltpu.roll(bu[:, i * 128:(i + 1) * 128], PB, 1)
        return bu

    def bu_operands(xn):
        a11, a12, a21, a22 = xn[:KA, :HA], xn[KA:, :HA], xn[:KA, HA:], xn[KA:, HA:]
        addp = lambda t, b: jnp.concatenate([t[:KB] + b, t[KB:]], axis=0)
        padz = lambda b: jnp.concatenate([b, jnp.zeros((KA - KB, HA), F32)], axis=0)
        ops = (addp(a21, a22), padz(a11[:KB] + a12), padz(a22), a11, addp(a11, a22), padz(a12 - a22), a21 - a11)
        return [o.astype(BF16).T for o in ops]

    def bu_lo(l2, l5):
        r2 = pltpu.bitcast(jnp.concatenate([b_words(0, PA, 0, 2), b_words(2 * PA, 2 * P, 0, 2)], axis=0), BF16)
        r5 = pltpu.bitcast(b_words(PA, 2 * P, 2, NK + 1), BF16)
        return _dot_nt(l2, r2), _dot_nt(l5[:, :KB], r5)

    def bu_hi(base, off, m2, m5, ls):
        jb = base + off // R
        r0 = (off % R) * ta
        mm = lambda i, rows: _dot_nt(ls[i], xblk(bx_s, 5, i, 0, rows))

        def put(half, k0, val):
            rows = pl.ds(r0 + half * HA, HA)
            for k in range(NA):
                bu_s[jb, k0 + k, rows, :] = val[:, k * 128:(k + 1) * 128]
            if val.shape[1] > PA:
                bu_s[jb, NB - 1, rows, :] = val[:, PA:]
                bu_s[jb, NB, rows, :] = pltpu.roll(val[:, PA:], PB, 1)

        m4 = mm(0, PA + 128)
        put(1, 0, m2 + m4)
        m3 = mm(1, PA + 128)
        put(0, NA, m3 + m5)
        m1 = mm(2, PA)
        u = m1 + m4[:, :PA] - m5[:, :PA]
        v = m1 - m2[:, :PA] + m3[:, :PA]
        m7 = mm(3, PA)
        put(0, 0, u + m7)
        m6 = mm(4, PA)
        put(1, NA, v + m6)
        return [m4, m3, m1, m7, m6]

    def stash(m2, m5, ls):
        m_s[0] = m2
        m_s[1] = m5
        for i in range(5):
            lx_s[i] = pltpu.bitcast(ls[2 + i], U32)

    def finish(base, off):
        return bu_hi(base, off, m_s[0], m_s[1], [pltpu.bitcast(lx_s[i], BF16) for i in range(5)])

    def phase_a_pair(base, lng):
        j = base * R + 1
        res = finish(base, 1)
        ls = bu_operands(ln1(j + 1, 0, ta)[1])
        cur = list(bu_lo(ls[0], ls[1]))
        cur += bu_hi(base, 2, cur[0], cur[1], ls[2:])
        ev = [e for m in cur for e in _heads(m)]
        xn = jnp.concatenate([ln1(j + 2, k * 128, (k + 1) * 128, [ev[g] for g in lng[k]])[1]
                              for k in range(ta // 128)], axis=1)
        ls = bu_operands(xn)
        m2, m5 = bu_lo(ls[0], ls[1])
        stash(m2, m5, ls)
        return res + cur + [m2, m5]

    def ln2_stats(j, deps):
        for k in range(tb // 128):
            xs = gate(tiles(xn_s, j, k * 128, (k + 1) * 128), deps[k])
            m = jnp.sum(xs, axis=0, keepdims=True) * (1.0 / D)
            v = jnp.sum(xs * xs, axis=0, keepdims=True) * (1.0 / D) - m * m
            r = jax.lax.rsqrt(v + EPS)
            st_s[0:8, k * 128:(k + 1) * 128] = jnp.broadcast_to(r, (8, 128))
            st_s[8:16, k * 128:(k + 1) * 128] = jnp.broadcast_to(m * r, (8, 128))

    def mlp_up(j):
        st = st_s[...]
        yT = tiles(xn_s, j, 0, tb) * st[0:1, :] - st[8:9, :]
        a11, a12, a21, a22 = yT[:DH, :H], yT[DH:, :H], yT[:DH, H:], yT[DH:, H:]
        row = jax.lax.broadcasted_iota(jnp.int32, (KP - DH, H), 0)
        zeros = jnp.zeros((KP - DH, H), F32)
        ones = jnp.where(row == 0, 1.0, 0.0).astype(F32)

        def mm(lhsT, rhs, pad=zeros):
            lhs = jnp.concatenate([lhsT, pad], axis=0).astype(BF16).T
            return jnp.dot(lhs, rhs, preferred_element_type=F32)

        def act(r, c, x):
            t = jnp.tanh(x * (x * x * GELU_C1 + GELU_C0))
            a_s[r * H:(r + 1) * H, c * FH:(c + 1) * FH] = x + x * t

        m2 = mm(a21 + a22, wblk(w1_s, 0, 0, KP))
        m4 = mm(a22, xblk(w1x_s, 5, 0), ones)
        act(1, 0, m2 + m4)
        m5 = mm(a11 + a12, wblk(w1_s, 1, DH, DH + KP))
        m3 = mm(a11, xblk(w1x_s, 5, 1), ones)
        act(0, 1, m3 + m5)
        m1 = mm(a11 + a22, xblk(w1x_s, 5, 2))
        u = m1 + m4 - m5
        v = m1 - m2 + m3
        m7 = mm(a12 - a22, xblk(w1x_s, 5, 3))
        act(0, 0, u + m7)
        m6 = mm(a21 - a11, xblk(w1x_s, 5, 4))
        act(1, 1, v + m6)
        return [e for m in (m2, m4, m5, m3, m1, m7, m6) for e in _heads(m)]

    def scan(j, dep):
        row = jax.lax.broadcasted_iota(jnp.int32, (8, 128), 0)
        for ka, kb in [(k, NA + k) for k in range(NA)] + [(NB - 1, NB)]:
            sa = slice(ka * 128, (ka + 1) * 128)
            sb = slice(kb * 128, (kb + 1) * 128)
            la = lam_s[0, :, sa]
            lba = lam_s[1, :, sa]
            lbb = lam_s[1, :, sb]
            ca = gate(carry_s[:, sa], dep)
            cb = carry_s[:, sb]

            def step(u, v, i):
                bu = bu_s[j, ka, pl.ds(i, 8, stride=Q), :]
                bv = bu_s[j, kb, pl.ds(i, 8, stride=Q), :]
                return (la * u + bu) + lba * v, (la * v + bv) + lbb * u

            u, v = ca, cb
            for i in range(Q):
                u, v = step(u, v, i)
            for k in range(3):
                sh = 1 << k
                us = jnp.where(row >= sh, pltpu.roll(u, sh, 0), 0.0)
                vs = jnp.where(row >= sh, pltpu.roll(v, sh, 0), 0.0)
                pa = lam_s[2 + 2 * k, :, sa]
                u, v = (u + pa * us + lam_s[3 + 2 * k, :, sa] * vs,
                        v + pa * vs + lam_s[3 + 2 * k, :, sb] * us)
            u = jnp.where(row == 0, ca, pltpu.roll(u, 1, 0))
            v = jnp.where(row == 0, cb, pltpu.roll(v, 1, 0))
            for i in range(Q):
                u, v = step(u, v, i)
                if i == QL - 1:
                    carry_s[:, sa] = jnp.where(row == 0, pltpu.roll(u, 1, 0), 0.0)
                    carry_s[:, sb] = jnp.where(row == 0, pltpu.roll(v, 1, 0), 0.0)
                h_s[ka, pl.ds(i, 8, stride=Q), :] = u
                if kb < NB:
                    h_s[kb, pl.ds(i, 8, stride=Q), :] = v
            dep = u

    def ssm_out(j, split=False):
        g = lambda r, c: jnp.concatenate([h_s[c * NA + k, r * H:(r + 1) * H, :] for k in range(NA)], axis=1)
        parts = []

        def mm(i, rhs):
            lhs = xblk(cw_s, 7, i)
            if not split:
                return _dot_nt(lhs, rhs.astype(BF16))
            cols = []
            for n in range(H // 128):
                acc = None
                for k in range(NA):
                    p = _dot_nt(lhs[:, k * 128:(k + 1) * 128],
                                rhs[n * 128:(n + 1) * 128, k * 128:(k + 1) * 128].astype(BF16))
                    parts.append(p)
                    acc = p if acc is None else acc + p
                cols.append(acc)
            return jnp.concatenate(cols, axis=1)

        z = _dot_nt(pltpu.bitcast(cm_s[:, 0:128], BF16), h_s[NB - 1, :tb, :].astype(BF16))
        z = z + tiles(xn_s, j, 0, tb) * _rep(col_s[0], tb)
        n2 = mm(0, g(0, 0))
        n4 = mm(5, g(0, 1) - g(0, 0))
        s_s[DH:, :H] = z[DH:, :H] + (n2 + n4)
        n5 = mm(1, g(1, 1))
        n3 = mm(6, g(1, 0) - g(1, 1))
        s_s[:DH, H:] = z[:DH, H:] + (n3 + n5)
        n1 = mm(2, g(0, 0) + g(1, 1))
        u = z[:DH, :H] + n1 + n4 - n5
        v = z[DH:, H:] + n1 - n2 + n3
        s_s[:DH, :H] = u + mm(3, g(0, 1) + g(1, 1))
        s_s[DH:, H:] = v + mm(4, g(0, 0) + g(1, 0))
        return parts

    last_pieces = ((0, 0, DH), (128, 0, 128), (128, 128, DH))

    def mlp_down(j, last=False):
        g = lambda r, c: a_s[r * H:(r + 1) * H, c * FH:(c + 1) * FH]
        mm = lambda lhs, rhs: _dot_nt(lhs, rhs.astype(BF16))

        def fin(r0, lo, oT):
            r1, hi = r0 + oT.shape[0], lo + oT.shape[1]
            h = oT * 0.25 + _rep(col_s[1, r0:r1, :], hi - lo)
            gt = h + h * jnp.tanh(h)
            o_s[j, r0:r1, lo:hi] = tiles(x_s, j, lo, hi)[r0:r1].astype(F32) + s_s[r0:r1, lo:hi] * gt
            if last:
                o_copy(j, lo, hi, r0, r1).start()

        n2 = mm(xblk(w2x_s, 5, 0), g(0, 0))
        n4 = mm(wblk(w2_s, 1, DH, D), g(0, 1) - g(0, 0))
        fin(DH, 0, n2 + n4)
        n5 = mm(xblk(w2x_s, 5, 1), g(1, 1))
        n3 = mm(wblk(w2_s, 0, 0, DH), g(1, 0) - g(1, 1))
        fin(0, H, n3 + n5)
        n1 = mm(xblk(w2x_s, 5, 2), g(0, 0) + g(1, 1))
        u = n1 + n4 - n5
        v = n1 - n2 + n3
        n7 = mm(xblk(w2x_s, 5, 3), g(0, 1) + g(1, 1))
        fin(0, 0, u + n7)
        s6 = g(0, 0) + g(1, 0)
        if not last:
            fin(DH, H, v + mm(xblk(w2x_s, 5, 4), s6))
        else:
            for lo, r0, r1 in last_pieces:
                fin(DH + r0, H + lo, v[r0:r1, lo:lo + 128] + mm(xblk(w2x_s, 5, 4, r0, r1), s6[lo:lo + 128, :]))
        return [e for n in (n2, n4, n5, n3, n1, n7) for e in _heads(n)]

    for c in vec_copies:
        c.start()
    x_copy(0).start()
    for c in b0_copies:
        c.start(priority=1)
    zsrc_s[...] = jnp.zeros_like(zsrc_s)
    z_copy.start()
    for c in vec_copies + [z_copy]:
        c.wait()
    for c in b1_copies:
        c.start(priority=1)
    x_copy(1).start(priority=1)
    prep_params()
    x_copy(0).wait()
    xn0 = ln1(0, 0, ta)[0].T
    for c in b0_copies:
        c.wait()
    for j in range(2, na):
        x_copy(j).start(priority=1)
    ev = _heads(bu_plain(xn0, (0, 1, NA, NA + 1)), (0, 64, 128, 192))
    prep_b(0, [ev[k] for k in EVB0])
    for c in b1_copies:
        c.wait()
    for c in w1_copies + c_copies + w2_copies:
        c.start(priority=1)

    x_copy(1).wait()
    bu0 = bu_plain(xn0, (2, NA + 2, NB - 1))
    ls = bu_operands(ln1(1, 0, ta)[1])
    m2, m5 = bu_lo(ls[0], ls[1])
    stash(m2, m5, ls)
    ev = _heads(bu0, (0, 64, 128, 192)) + _heads(m2) + _heads(m5)
    prep_b(E // 32, [ev[k] for k in EVB])

    def body_a(i, carry):
        x_copy(2 * i + 2).wait()
        x_copy(2 * i + 3).wait()
        phase_a_pair(i, LNG)
        return carry

    jax.lax.fori_loop(0, nb - 2, body_a, 0)

    x_copy(na - 2).wait()
    x_copy(na - 1).wait()
    for c in w1_copies:
        c.wait()
    ev = [e for m in phase_a_pair(nb - 2, LNGL) for e in _heads(m, (0, 64))]
    prep_w(w1_s, w1x_s, RHS_SUMS, [ev[k] for k in EVS])

    for c in c_copies + w2_copies:
        c.wait()
    finish(0, na - 1)
    ln2_stats(0, [None] * (tb // 128))
    ev = mlp_up(0)
    prep_c([ev[k] for k in CPK])
    scan(0, ev[GS0])
    parts = ssm_out(0, split=True)
    ev = [e for i in EV2[0] for e in _heads(parts[i], EV2[1])]
    prep_w(w2_s, w2x_s, LHS_SUMS, ev[:7 * NFH])

    def body_b(j, carry):
        ev = mlp_down(j)
        ln2_stats(j + 1, [ev[k] for k in STG])
        mlp_up(j + 1)
        scan(j + 1, ev[GS])
        ssm_out(j + 1)
        o_copy(j).start()
        return carry

    jax.lax.fori_loop(0, nb - 1, body_b, 0)

    mlp_down(nb - 1, last=True)
    for j in range(nb - 1):
        o_copy(j).wait()
    for lo, hi, r0, r1 in ((0, H, DH, D), (H, tb, 0, DH), (0, H, 0, DH)):
        o_copy(nb - 1, lo, hi, r0, r1).wait()
    for lo, r0, r1 in last_pieces:
        o_copy(nb - 1, H + lo, H + lo + 128, DH + r0, DH + r1).wait()


@jax.jit
def pallas_recurrent_scan__ssm_conv_s5__mixer_channel_mlp__prompt_kernel(
    A_x, A_Lambda_re, A_Lambda_im, A_B_re, A_B_im, A_C_re, A_C_im, A_log_dt, A_Dskip,
    B_x, B_w1, B_b1, B_w2, B_b2,
):
    Bsz, L, D = A_x.shape
    P = A_Lambda_re.shape[0]
    F = B_w1.shape[1]
    assert (Bsz, L, D, P, F) == (1, 2048, 448, 448, 1792)
    ta, tb = TA, TB
    na, nb = L // ta, L // tb
    NF, NA = F // 128, P // 128
    DH = D // 2
    KP = pl.cdiv(DH, 128) * 128
    outT = pl.pallas_call(
        _kernel,
        in_specs=[pl.BlockSpec(memory_space=pl.ANY)] * 13,
        out_specs=pl.BlockSpec(memory_space=pl.ANY),
        out_shape=jax.ShapeDtypeStruct((D, L), F32),
        scratch_shapes=[
            pltpu.VMEM((na, D, ta), BF16),
            pltpu.VMEM((nb, D, tb), F32),
            pltpu.VMEM((nb, 2 * NA + 2, tb + 8, 128), F32),
            pltpu.VMEM((na, D, ta), F32),
            pltpu.VMEM((D // 128, 2 * P, 128), BF16),
            pltpu.VMEM((2 * P, D % 128), BF16),
            pltpu.VMEM((2 * NA, D, 128), BF16),
            pltpu.VMEM((2, D, P % 128), BF16),
            pltpu.VMEM((7 * DH // 2, NA * 128), U32),
            pltpu.VMEM((NF, DH + KP, 128), BF16),
            pltpu.VMEM((NF, D, 128), BF16),
            pltpu.VMEM((5 * KP // 2, F // 2), U32),
            pltpu.VMEM((5 * DH // 2, F // 2), U32),
            pltpu.VMEM((8, 8, (2 * NA + 2) * 128), F32),
            pltpu.VMEM((8, (2 * NA + 2) * 128), F32),
            pltpu.VMEM((2, D, 128), F32),
            pltpu.VMEM((8, P), F32),
            pltpu.VMEM((D // 2, 256), U32),
            pltpu.VMEM((2 * NA + 1, tb + 8, 128), F32),
            pltpu.VMEM((tb, F), F32),
            pltpu.VMEM((D, tb), F32),
            pltpu.VMEM((5 * (NA + 1) * 64, 256), U32),
            pltpu.VMEM((5, ta // 4, 256), U32),
            pltpu.VMEM((2, ta // 2, (NA + 1) * 128), F32),
            pltpu.VMEM((16, tb), F32),
            pltpu.VMEM((8, 128), jnp.int32),
            pltpu.VMEM((8, 128), jnp.int32),
            pltpu.VMEM((P,), BF16), pltpu.VMEM((P,), BF16), pltpu.VMEM((P,), BF16),
            pltpu.VMEM((D,), BF16), pltpu.VMEM((F,), BF16), pltpu.VMEM((D,), BF16),
            pltpu.SemaphoreType.DMA((na,)),
            pltpu.SemaphoreType.DMA(()),
            pltpu.SemaphoreType.DMA((5,)),
        ],
        compiler_params=pltpu.CompilerParams(
            vmem_limit_bytes=100 * 1024 * 1024,
            disable_semaphore_checks=True, disable_bounds_checks=True),
    )(A_x.reshape(L, D).T, A_Lambda_re, A_Lambda_im, A_B_re, A_B_im, A_C_re, A_C_im,
      A_log_dt, A_Dskip, B_w1, B_b1, B_w2.T, B_b2)
    return outT.T.reshape(Bsz, L, D)
```

```python
import jax
import jax.numpy as jnp
import jax.experimental.pallas as pl
import jax.experimental.pallas.tpu as pltpu

F32 = jnp.float32
BF16 = jnp.bfloat16
U32 = jnp.uint32
NT = (((1,), (1,)), ((), ()))
EPS = 1e-5
GELU_C0 = 0.7978845608028654
GELU_C1 = 0.7978845608028654 * 0.044715

TA = 256
TB = 512

EVB0 = (0,1,2,4,5,6,8,9)
EVB = (6,7,10,12,14,15,16,18)
LNG = ((0,2,12),(0,2,5))
LNGL = ((0,3,11),(0,1,14))
EVS = (45,46,47,48,49,50,51,52,53,54,55,56,57,59,60,61,62,63,64,65,66,67,68,69,70,72,73,74,75,76,77,78,79,80,81,82,83,85,86,87,88,89,90,91,92,93,94,95,96)
CPK = (0,1,2,3,4,5,6,28,29,30,31,32,33,34)
GS0 = 4
EV2 = ((3,7,11,15,19,23,27,31,35,39),(0,40,80,120,160))
STG = (0,1,9,10)
LASTP = ((0,0,224),(128,0,128),(128,128,224))
GS = 0

RHS_SUMS = ((-1, (1, 0), (0, 0)), (-1, (0, 1), (1, 1)), (1, (0, 0), (1, 1)), (1, (1, 0), (1, 1)), (1, (0, 0), (0, 1)))
LHS_SUMS = ((1, (1, 0), (1, 1)), (1, (0, 0), (0, 1)), (1, (0, 0), (1, 1)), (-1, (0, 1), (1, 1)), (-1, (1, 0), (0, 0)))


def _cmul(ar, ai, br, bi):
    return ar * br - ai * bi, ar * bi + ai * br


def _row(ref):
    return ref[...].astype(F32).reshape(1, ref.shape[0])


def _rep(c, w):
    return c if w == 128 else jnp.concatenate([c] * (w // 128), axis=1)


def _dot_nt(a, b):
    return jax.lax.dot_general(a, b, NT, preferred_element_type=F32)


def _unpack(w):
    return pltpu.bitcast(w, BF16).astype(F32)


def _pack(x):
    return pltpu.bitcast(x.astype(BF16), U32)


def _comb(sign, a, b):
    return a + b if sign > 0 else a - b


def _heads(m, rows=(0,)):
    return [m[r:r + 8, k * 128:(k + 1) * 128] for k in range(m.shape[1] // 128) for r in rows]


def _kernel(x_hbm, lre_hbm, lim_hbm, bre_hbm, bim_hbm, cre_hbm, cim_hbm, ldt_hbm, dsk_hbm,
            w1_hbm, b1_hbm, w2_hbm, b2_hbm, o_hbm,
            x_s, o_s, bu_s, xn_s, bw0_s, bt0_s, bw1_s, bt1_s, c_s, ct_s, cw_s, w1_s, w2_s, w1x_s, w2x_s,
            lam_s, carry_s, col_s, coef_s, cm_s, h_s, a_s, s_s, bx_s, lx_s, m_s, st_s, zero_s, zsrc_s,
            lre_s, lim_s, ldt_s, dsk_s, b1_s, b2_s,
            xsem, osem, wsem):
    ta, tb = TA, TB
    na, D, _ = x_s.shape
    nb = o_s.shape[0]
    P = lre_s.shape[0]
    R = tb // ta
    NF = w1_s.shape[0]
    NFH = NF // 2
    FH = NFH * 128
    NK = D // 128
    DP = pl.cdiv(D, 128) * 128
    DH = D // 2
    KP = pl.cdiv(DH, 128) * 128
    KA = 256
    KB = D - KA
    H = tb // 2
    HA = ta // 2
    Q = tb // 8 + 1
    QL = tb - 7 * Q
    NA = P // 128
    PA = NA * 128
    PB = P - PA
    NB = 2 * NA + 1
    W = (NB + 1) * 128
    E = 256

    def x_copy(j):
        return pltpu.make_async_copy(x_hbm.at[:, pl.ds(j * ta, ta)], x_s.at[j], xsem.at[j])

    def o_copy(j, lo=0, hi=tb, r0=0, r1=D):
        return pltpu.make_async_copy(o_s.at[j, r0:r1, lo:hi],
                                     o_hbm.at[r0:r1, pl.ds(j * tb + lo, hi - lo)], osem)

    b_parts = ((0, bre_hbm, 0, E, 0, 0), (E, bre_hbm, E, PA, 1, 0),
               (PA, bim_hbm, 0, E, 0, E), (PA + E, bim_hbm, E, PA, 1, PA - E),
               (2 * PA, bre_hbm, PA, P, 1, 2 * (PA - E)), (2 * PA + PB, bim_hbm, PA, P, 1, 2 * (PA - E) + PB))
    b_bufs = ((bw0_s, bt0_s), (bw1_s, bt1_s))

    def b_copies(group):
        cs = []
        for _, src, r0, r1, g, d0 in b_parts:
            if g == group:
                bw, bt = b_bufs[g]
                cs += [pltpu.make_async_copy(src.at[r0:r1, k * 128:(k + 1) * 128],
                                             bw.at[k, d0:d0 + r1 - r0, :], wsem.at[g]) for k in range(NK)]
                cs += [pltpu.make_async_copy(src.at[r0:r1, NK * 128:D], bt.at[d0:d0 + r1 - r0, :], wsem.at[g])]
        return cs

    vec_copies = [pltpu.make_async_copy(src, dst, wsem.at[3]) for src, dst in
                  ((lre_hbm, lre_s), (lim_hbm, lim_s), (ldt_hbm, ldt_s), (dsk_hbm, dsk_s),
                   (b1_hbm, b1_s), (b2_hbm, b2_s))]
    z_copy = pltpu.make_async_copy(zsrc_s, zero_s, wsem.at[3])
    b0_copies = b_copies(0)
    b1_copies = b_copies(1)
    w1_copies = [pltpu.make_async_copy(w1_hbm.at[:, k * 128:(k + 1) * 128], w1_s.at[k, 0:D, :], wsem.at[4])
                 for k in range(NF)]
    w2_copies = [pltpu.make_async_copy(w2_hbm.at[:, k * 128:(k + 1) * 128], w2_s.at[k], wsem.at[2])
                 for k in range(NF)]
    c_copies = [pltpu.make_async_copy(src.at[:, k * 128:(k + 1) * 128], c_s.at[i * NA + k], wsem.at[2])
                for i, src in enumerate((cre_hbm, cim_hbm)) for k in range(NA)]
    c_copies += [pltpu.make_async_copy(src.at[:, PA:P], ct_s.at[i], wsem.at[2])
                 for i, src in enumerate((cre_hbm, cim_hbm))]

    def gate(val, dep):
        if dep is None:
            return val
        n = val.shape[1]
        w = pl.cdiv(n, 128) * 128
        head = jnp.where(_rep(zero_s[...], w)[:, :n] != 0, _rep(dep, w)[:, :n], val[0:8, :])
        return head if val.shape[0] == 8 else jnp.concatenate([head, val[8:, :]], axis=0)

    def gate_row(val, dep):
        if dep is None:
            return val
        w = val.shape[1]
        return jnp.where(_rep(zero_s[0:1, :], w) != 0, _rep(dep[0:1, :], w), val)

    def gate_all(val, dep):
        n, w = val.shape[0] // 8, pl.cdiv(val.shape[1], 128) * 128
        z = jnp.concatenate([_rep(zero_s[...], w)] * n, axis=0)[:, :val.shape[1]]
        d = jnp.concatenate([_rep(pltpu.bitcast(dep, val.dtype), w)] * n, axis=0)[:, :val.shape[1]]
        return jnp.where(z != 0, d, val)

    def b_words(r0, r1, k0, k1):
        rows = []
        for s0, _, a, b, g, d0 in b_parts:
            lo, hi = max(r0, s0), min(r1, s0 + b - a)
            if lo < hi:
                bw, bt = b_bufs[g]
                rs = slice((d0 + lo - s0) // 2, (d0 + hi - s0) // 2)
                rows.append(jnp.concatenate(
                    [bw.bitcast(U32)[k, rs, :] if k < NK else bt.bitcast(U32)[rs, :] for k in range(k0, k1)],
                    axis=1))
        return rows[0] if len(rows) == 1 else jnp.concatenate(rows, axis=0)

    def wblk(ref, half, r0, r1):
        r32 = ref.bitcast(U32)
        return pltpu.bitcast(
            jnp.concatenate([r32[half * NFH + k, r0 // 2:r1 // 2, :] for k in range(NFH)], axis=1), BF16)

    def xblk(ref, n, i, r0=0, r1=None):
        rows = ref.shape[0] // n
        r1 = 2 * rows if r1 is None else r1
        return pltpu.bitcast(ref[i * rows + r0 // 2:i * rows + r1 // 2, :], BF16)

    def tiles(ref, j, lo, hi):
        parts = []
        for r in range(R):
            a, b = max(lo, r * ta), min(hi, (r + 1) * ta)
            if a < b:
                parts.append(ref[j * R + r, :, a - r * ta:b - r * ta])
        return parts[0] if len(parts) == 1 else jnp.concatenate(parts, axis=1)

    def prep_params():
        lr = _row(lre_s)
        li = _row(lim_s)
        dt = jnp.exp(_row(ldt_s)).astype(BF16).astype(F32)
        mag = jnp.exp(dt * lr)
        ang = dt * li
        lbr = mag * jnp.cos(ang)
        lbi = mag * jnp.sin(ang)
        nr = lbr - 1.0
        den = lr * lr + li * li
        coef_s[...] = jnp.zeros_like(coef_s)
        coef_s[0:1, :] = 2.0 * (nr * lr + lbi * li) / den
        coef_s[1:2, :] = 2.0 * (lbi * lr - nr * li) / den

        def put_lam(k, re, im):
            a = jnp.concatenate([re[:, :PA], re[:, :PA], re[:, PA:], re[:, PA:], re[:, PA:], re[:, PA:]], axis=1)
            b = jnp.concatenate([-im[:, :PA], im[:, :PA], -im[:, PA:], im[:, PA:], im[:, PA:], -im[:, PA:]], axis=1)
            lam_s[2 * k] = jnp.broadcast_to(a, (8, W))
            lam_s[2 * k + 1] = jnp.broadcast_to(b, (8, W))

        put_lam(0, lbr, lbi)
        pr, pi = lbr, lbi
        q = 1
        while q < Q - 1:
            pr, pi = _cmul(pr, pi, pr, pi)
            q *= 2
        assert q == Q - 1
        pr, pi = _cmul(pr, pi, lbr, lbi)
        for k in range(3):
            put_lam(1 + k, pr, pi)
            pr, pi = _cmul(pr, pi, pr, pi)
        carry_s[...] = jnp.zeros_like(carry_s)
        bu_s[:, :, tb:, :] = jnp.zeros((nb, NB + 1, 8, 128), F32)
        row = jax.lax.broadcasted_iota(jnp.int32, (KP - DH, NF * 128), 0)
        pad = pltpu.bitcast(jnp.where(row == 0, _row(b1_s), 0.0).astype(BF16), U32)
        for i in range(5):
            rs = slice((i * KP + DH) // 2, (i + 1) * KP // 2)
            w1x_s[rs, :] = pad[:, i * FH:(i + 1) * FH] if i < 2 else jnp.zeros(((KP - DH) // 2, FH), U32)
        w1_s[:, D:, :] = jnp.zeros((NF, w1_s.shape[1] - D, 128), BF16)
        for k, r in enumerate((_row(dsk_s), 0.5 * _row(b2_s))):
            r = jnp.concatenate([r, jnp.zeros((1, DP - D), F32)], axis=1)
            col_s[k] = jnp.broadcast_to(r, (128, DP)).T[:D, :]

    def prep_b(q0, deps):
        rows = 32

        def top_bot(r0, dep):
            w = _unpack(gate_all(b_words(r0, r0 + rows, 0, NK + 1), dep))
            return w[:, :KA], jnp.concatenate([w[:, KA:], jnp.zeros((rows, KA - KB), F32)], axis=1)

        lane = jax.lax.broadcasted_iota(jnp.int32, (rows, KA), 1)
        cut = lambda a: jnp.where(lane < KB, a, 0.0)
        for q, dep in enumerate(deps):
            r0 = (q0 + q) * rows
            if r0 < PA:
                b11, b21 = top_bot(r0, dep)
                b12, b22 = top_bot(PA + r0, dep)
                outs = [cut(b21 - b11), b12 - b22, b11 + b22, b21 + b22, b11 + b12]
            else:
                b1, b2 = top_bot(PA + r0, dep)
                outs = [cut(b2 - b1), b1 - b2]
            for i, o in enumerate(outs):
                bx_s[(i * (PA + 128) + r0) // 2:(i * (PA + 128) + r0 + rows) // 2, :] = _pack(o)

    def prep_w(src, dst, specs, deps):
        src32 = src.bitcast(U32)
        per = len(deps) // NFH
        rows = DH // 2 // per
        z = jnp.concatenate([zero_s[...]] * (rows // 8), axis=0) != 0
        for n, dep in enumerate(deps):
            k, q = divmod(n, per)
            d = jnp.concatenate([pltpu.bitcast(dep, U32)] * (rows // 8), axis=0)
            blk = {}
            for r in range(2):
                for c in range(2):
                    r0 = r * DH // 2 + q * rows
                    blk[r, c] = _unpack(jnp.where(z, d, src32[c * NFH + k, r0:r0 + rows, :]))
            for i, (sign, a, b) in enumerate(specs):
                r0 = i * (dst.shape[0] // 5) + q * rows
                dst[r0:r0 + rows, k * 128:(k + 1) * 128] = _pack(_comb(sign, blk[a], blk[b]))

    def prep_c(deps):
        rows = DH // 2 // len(deps)
        for q, dep in enumerate(deps):
            cf = gate(coef_s[...], dep)
            cr = cf[0:1, :]
            ci = cf[1:2, :]
            blk = {}
            for r in range(2):
                rs = slice(r * DH // 2 + q * rows, r * DH // 2 + (q + 1) * rows)
                ld = lambda i: jnp.concatenate(
                    [c_s.bitcast(U32)[i * NA + k, rs, :] for k in range(NA)] + [ct_s.bitcast(U32)[i, rs, :]],
                    axis=1)
                c_re = _unpack(ld(0))
                c_im = _unpack(ld(1))
                cpr = c_re * cr - c_im * ci
                cpi = -(c_re * ci) - c_im * cr
                blk[r, 0], blk[r, 1] = cpr[:, :PA], cpi[:, :PA]
                cm_s[rs, 0:128] = _pack(jnp.concatenate([cpr[:, PA:], cpi[:, PA:]], axis=1))
            outs = [_comb(sign, blk[a], blk[b]) for sign, a, b in LHS_SUMS] + [blk[1, 1], blk[0, 0]]
            for i, o in enumerate(outs):
                cw_s[i * DH // 2 + q * rows:i * DH // 2 + (q + 1) * rows, :] = _pack(o)

    def ln1(j, lo, hi, deps=(None, None, None)):
        x = gate(x_s[j, :, lo:hi].astype(F32), deps[0])
        m = gate_row(jnp.sum(x, axis=0, keepdims=True) * (1.0 / D), deps[1])
        xc = x - m
        v = jnp.sum(xc * xc, axis=0, keepdims=True) * (1.0 / D)
        xb = (xc * gate_row(jax.lax.rsqrt(v + EPS), deps[2])).astype(BF16)
        xn = xb.astype(F32)
        xn_s[j, :, lo:hi] = xn
        return xb, xn

    def bu_plain(xn, ks):
        rhs = pltpu.bitcast(
            jnp.concatenate([b_words(k * 128, (k + 1) * 128, 0, NK + 1) for k in ks], axis=0), BF16)
        bu = _dot_nt(xn, rhs)
        for i, k in enumerate(ks):
            bu_s[0, k, 0:ta, :] = bu[:, i * 128:(i + 1) * 128]
            if k == NB - 1:
                bu_s[0, NB, 0:ta, :] = pltpu.roll(bu[:, i * 128:(i + 1) * 128], PB, 1)
        return bu

    def bu_operands(xn):
        a11, a12, a21, a22 = xn[:KA, :HA], xn[KA:, :HA], xn[:KA, HA:], xn[KA:, HA:]
        addp = lambda t, b: jnp.concatenate([t[:KB] + b, t[KB:]], axis=0)
        padz = lambda b: jnp.concatenate([b, jnp.zeros((KA - KB, HA), F32)], axis=0)
        ops = (addp(a21, a22), padz(a11[:KB] + a12), padz(a22), a11, addp(a11, a22), padz(a12 - a22), a21 - a11)
        return [o.astype(BF16).T for o in ops]

    def bu_lo(l2, l5):
        r2 = pltpu.bitcast(jnp.concatenate([b_words(0, PA, 0, 2), b_words(2 * PA, 2 * P, 0, 2)], axis=0), BF16)
        r5 = pltpu.bitcast(b_words(PA, 2 * P, 2, NK + 1), BF16)
        return _dot_nt(l2, r2), _dot_nt(l5[:, :KB], r5)

    def bu_hi(base, off, m2, m5, ls):
        jb = base + off // R
        r0 = (off % R) * ta
        mm = lambda i, rows: _dot_nt(ls[i], xblk(bx_s, 5, i, 0, rows))

        def put(half, k0, val):
            rows = pl.ds(r0 + half * HA, HA)
            for k in range(NA):
                bu_s[jb, k0 + k, rows, :] = val[:, k * 128:(k + 1) * 128]
            if val.shape[1] > PA:
                bu_s[jb, NB - 1, rows, :] = val[:, PA:]
                bu_s[jb, NB, rows, :] = pltpu.roll(val[:, PA:], PB, 1)

        m4 = mm(0, PA + 128)
        put(1, 0, m2 + m4)
        m3 = mm(1, PA + 128)
        put(0, NA, m3 + m5)
        m1 = mm(2, PA)
        u = m1 + m4[:, :PA] - m5[:, :PA]
        v = m1 - m2[:, :PA] + m3[:, :PA]
        m7 = mm(3, PA)
        put(0, 0, u + m7)
        m6 = mm(4, PA)
        put(1, NA, v + m6)
        return [m4, m3, m1, m7, m6]

    def stash(m2, m5, ls):
        m_s[0] = m2
        m_s[1] = m5
        for i in range(5):
            lx_s[i] = pltpu.bitcast(ls[2 + i], U32)

    def finish(base, off):
        return bu_hi(base, off, m_s[0], m_s[1], [pltpu.bitcast(lx_s[i], BF16) for i in range(5)])

    def phase_a_pair(base, lng):
        j = base * R + 1
        res = finish(base, 1)
        ls = bu_operands(ln1(j + 1, 0, ta)[1])
        cur = list(bu_lo(ls[0], ls[1]))
        cur += bu_hi(base, 2, cur[0], cur[1], ls[2:])
        ev = [e for m in cur for e in _heads(m)]
        xn = jnp.concatenate([ln1(j + 2, k * 128, (k + 1) * 128, [ev[g] for g in lng[k]])[1]
                              for k in range(ta // 128)], axis=1)
        ls = bu_operands(xn)
        m2, m5 = bu_lo(ls[0], ls[1])
        stash(m2, m5, ls)
        return res + cur + [m2, m5]

    def ln2_stats(j, deps):
        for k in range(tb // 128):
            xs = gate(tiles(xn_s, j, k * 128, (k + 1) * 128), deps[k])
            m = jnp.sum(xs, axis=0, keepdims=True) * (1.0 / D)
            v = jnp.sum(xs * xs, axis=0, keepdims=True) * (1.0 / D) - m * m
            r = jax.lax.rsqrt(v + EPS)
            st_s[0:8, k * 128:(k + 1) * 128] = jnp.broadcast_to(r, (8, 128))
            st_s[8:16, k * 128:(k + 1) * 128] = jnp.broadcast_to(m * r, (8, 128))

    def mlp_up(j):
        st = st_s[...]
        yT = tiles(xn_s, j, 0, tb) * st[0:1, :] - st[8:9, :]
        a11, a12, a21, a22 = yT[:DH, :H], yT[DH:, :H], yT[:DH, H:], yT[DH:, H:]
        row = jax.lax.broadcasted_iota(jnp.int32, (KP - DH, H), 0)
        zeros = jnp.zeros((KP - DH, H), F32)
        ones = jnp.where(row == 0, 1.0, 0.0).astype(F32)

        def mm(lhsT, rhs, pad=zeros):
            lhs = jnp.concatenate([lhsT, pad], axis=0).astype(BF16).T
            return jnp.dot(lhs, rhs, preferred_element_type=F32)

        def act(r, c, x):
            t = jnp.tanh(x * (x * x * GELU_C1 + GELU_C0))
            a_s[r * H:(r + 1) * H, c * FH:(c + 1) * FH] = x + x * t

        m2 = mm(a21 + a22, wblk(w1_s, 0, 0, KP))
        m4 = mm(a22, xblk(w1x_s, 5, 0), ones)
        act(1, 0, m2 + m4)
        m5 = mm(a11 + a12, wblk(w1_s, 1, DH, DH + KP))
        m3 = mm(a11, xblk(w1x_s, 5, 1), ones)
        act(0, 1, m3 + m5)
        m1 = mm(a11 + a22, xblk(w1x_s, 5, 2))
        u = m1 + m4 - m5
        v = m1 - m2 + m3
        m7 = mm(a12 - a22, xblk(w1x_s, 5, 3))
        act(0, 0, u + m7)
        m6 = mm(a21 - a11, xblk(w1x_s, 5, 4))
        act(1, 1, v + m6)
        return [e for m in (m2, m4, m5, m3, m1, m7, m6) for e in _heads(m)]

    def scan(j, dep):
        row = jax.lax.broadcasted_iota(jnp.int32, (8, 128), 0)
        for ka, kb in [(k, NA + k) for k in range(NA)] + [(NB - 1, NB)]:
            sa = slice(ka * 128, (ka + 1) * 128)
            sb = slice(kb * 128, (kb + 1) * 128)
            la = lam_s[0, :, sa]
            lba = lam_s[1, :, sa]
            lbb = lam_s[1, :, sb]
            ca = gate(carry_s[:, sa], dep)
            cb = carry_s[:, sb]

            def step(u, v, i):
                bu = bu_s[j, ka, pl.ds(i, 8, stride=Q), :]
                bv = bu_s[j, kb, pl.ds(i, 8, stride=Q), :]
                return (la * u + bu) + lba * v, (la * v + bv) + lbb * u

            u, v = ca, cb
            for i in range(Q):
                u, v = step(u, v, i)
            for k in range(3):
                sh = 1 << k
                us = jnp.where(row >= sh, pltpu.roll(u, sh, 0), 0.0)
                vs = jnp.where(row >= sh, pltpu.roll(v, sh, 0), 0.0)
                pa = lam_s[2 + 2 * k, :, sa]
                u, v = (u + pa * us + lam_s[3 + 2 * k, :, sa] * vs,
                        v + pa * vs + lam_s[3 + 2 * k, :, sb] * us)
            u = jnp.where(row == 0, ca, pltpu.roll(u, 1, 0))
            v = jnp.where(row == 0, cb, pltpu.roll(v, 1, 0))
            for i in range(Q):
                u, v = step(u, v, i)
                if i == QL - 1:
                    carry_s[:, sa] = jnp.where(row == 0, pltpu.roll(u, 1, 0), 0.0)
                    carry_s[:, sb] = jnp.where(row == 0, pltpu.roll(v, 1, 0), 0.0)
                h_s[ka, pl.ds(i, 8, stride=Q), :] = u
                if kb < NB:
                    h_s[kb, pl.ds(i, 8, stride=Q), :] = v
            dep = u

    def ssm_out(j, split=False):
        g = lambda r, c: jnp.concatenate([h_s[c * NA + k, r * H:(r + 1) * H, :] for k in range(NA)], axis=1)
        parts = []

        def mm(i, rhs):
            lhs = xblk(cw_s, 7, i)
            if not split:
                return _dot_nt(lhs, rhs.astype(BF16))
            cols = []
            for n in range(H // 128):
                acc = None
                for k in range(NA):
                    p = _dot_nt(lhs[:, k * 128:(k + 1) * 128],
                                rhs[n * 128:(n + 1) * 128, k * 128:(k + 1) * 128].astype(BF16))
                    parts.append(p)
                    acc = p if acc is None else acc + p
                cols.append(acc)
            return jnp.concatenate(cols, axis=1)

        z = _dot_nt(pltpu.bitcast(cm_s[:, 0:128], BF16), h_s[NB - 1, :tb, :].astype(BF16))
        z = z + tiles(xn_s, j, 0, tb) * _rep(col_s[0], tb)
        n2 = mm(0, g(0, 0))
        n4 = mm(5, g(0, 1) - g(0, 0))
        s_s[DH:, :H] = z[DH:, :H] + (n2 + n4)
        n5 = mm(1, g(1, 1))
        n3 = mm(6, g(1, 0) - g(1, 1))
        s_s[:DH, H:] = z[:DH, H:] + (n3 + n5)
        n1 = mm(2, g(0, 0) + g(1, 1))
        u = z[:DH, :H] + n1 + n4 - n5
        v = z[DH:, H:] + n1 - n2 + n3
        s_s[:DH, :H] = u + mm(3, g(0, 1) + g(1, 1))
        s_s[DH:, H:] = v + mm(4, g(0, 0) + g(1, 0))
        return parts

    last_pieces = LASTP

    def mlp_down(j, last=False):
        g = lambda r, c: a_s[r * H:(r + 1) * H, c * FH:(c + 1) * FH]
        mm = lambda lhs, rhs: _dot_nt(lhs, rhs.astype(BF16))

        def fin(r0, lo, oT):
            r1, hi = r0 + oT.shape[0], lo + oT.shape[1]
            h = oT * 0.25 + _rep(col_s[1, r0:r1, :], hi - lo)
            gt = h + h * jnp.tanh(h)
            o_s[j, r0:r1, lo:hi] = tiles(x_s, j, lo, hi)[r0:r1].astype(F32) + s_s[r0:r1, lo:hi] * gt
            if last:
                o_copy(j, lo, hi, r0, r1).start()

        n2 = mm(xblk(w2x_s, 5, 0), g(0, 0))
        n4 = mm(wblk(w2_s, 1, DH, D), g(0, 1) - g(0, 0))
        fin(DH, 0, n2 + n4)
        n5 = mm(xblk(w2x_s, 5, 1), g(1, 1))
        n3 = mm(wblk(w2_s, 0, 0, DH), g(1, 0) - g(1, 1))
        fin(0, H, n3 + n5)
        n1 = mm(xblk(w2x_s, 5, 2), g(0, 0) + g(1, 1))
        u = n1 + n4 - n5
        v = n1 - n2 + n3
        n7 = mm(xblk(w2x_s, 5, 3), g(0, 1) + g(1, 1))
        fin(0, 0, u + n7)
        s6 = g(0, 0) + g(1, 0)
        if not last:
            fin(DH, H, v + mm(xblk(w2x_s, 5, 4), s6))
        else:
            for lo, r0, r1 in last_pieces:
                fin(DH + r0, H + lo, v[r0:r1, lo:lo + 128] + mm(xblk(w2x_s, 5, 4, r0, r1), s6[lo:lo + 128, :]))
        return [e for n in (n2, n4, n5, n3, n1, n7) for e in _heads(n)]

    for c in vec_copies:
        c.start()
    x_copy(0).start()
    for c in b0_copies:
        c.start(priority=1)
    zsrc_s[...] = jnp.zeros_like(zsrc_s)
    z_copy.start()
    for c in vec_copies + [z_copy]:
        c.wait()
    for c in b1_copies:
        c.start(priority=1)
    x_copy(1).start(priority=1)
    prep_params()
    x_copy(0).wait()
    xn0 = ln1(0, 0, ta)[0].T
    for c in b0_copies:
        c.wait()
    for j in range(2, na):
        x_copy(j).start(priority=1)
    ev = _heads(bu_plain(xn0, (0, 1, NA, NA + 1)), (0, 64, 128, 192))
    prep_b(0, [ev[k] for k in EVB0])
    for c in b1_copies:
        c.wait()
    for c in w1_copies + c_copies + w2_copies:
        c.start(priority=1)

    x_copy(1).wait()
    bu0 = bu_plain(xn0, (2, NA + 2, NB - 1))
    ls = bu_operands(ln1(1, 0, ta)[1])
    m2, m5 = bu_lo(ls[0], ls[1])
    stash(m2, m5, ls)
    ev = _heads(bu0, (0, 64, 128, 192)) + _heads(m2) + _heads(m5)
    prep_b(E // 32, [ev[k] for k in EVB])

    def body_a(i, carry):
        x_copy(2 * i + 2).wait()
        x_copy(2 * i + 3).wait()
        phase_a_pair(i, LNG)
        return carry

    jax.lax.fori_loop(0, nb - 2, body_a, 0)

    x_copy(na - 2).wait()
    x_copy(na - 1).wait()
    for c in w1_copies:
        c.wait()
    ev = [e for m in phase_a_pair(nb - 2, LNGL) for e in _heads(m, (0, 64))]
    prep_w(w1_s, w1x_s, RHS_SUMS, [ev[k] for k in EVS])

    for c in c_copies + w2_copies:
        c.wait()
    finish(0, na - 1)
    ln2_stats(0, [None] * (tb // 128))
    ev = mlp_up(0)
    prep_c([ev[k] for k in CPK])
    scan(0, ev[GS0])
    parts = ssm_out(0, split=True)
    ev = [e for i in EV2[0] for e in _heads(parts[i], EV2[1])]
    prep_w(w2_s, w2x_s, LHS_SUMS, ev[:7 * NFH])

    def body_b(j, carry):
        ev = mlp_down(j)
        ln2_stats(j + 1, [ev[k] for k in STG])
        mlp_up(j + 1)
        scan(j + 1, ev[GS])
        ssm_out(j + 1)
        o_copy(j).start()
        return carry

    jax.lax.fori_loop(0, nb - 1, body_b, 0)

    mlp_down(nb - 1, last=True)
    for j in range(nb - 1):
        o_copy(j).wait()
    for lo, hi, r0, r1 in ((0, H, DH, D), (H, tb, 0, DH), (0, H, 0, DH)):
        o_copy(nb - 1, lo, hi, r0, r1).wait()
    for lo, r0, r1 in last_pieces:
        o_copy(nb - 1, H + lo, H + lo + 128, DH + r0, DH + r1).wait()


@jax.jit
def pallas_recurrent_scan__ssm_conv_s5__mixer_channel_mlp__prompt_kernel(
    A_x, A_Lambda_re, A_Lambda_im, A_B_re, A_B_im, A_C_re, A_C_im, A_log_dt, A_Dskip,
    B_x, B_w1, B_b1, B_w2, B_b2,
):
    Bsz, L, D = A_x.shape
    P = A_Lambda_re.shape[0]
    F = B_w1.shape[1]
    assert (Bsz, L, D, P, F) == (1, 2048, 448, 448, 1792)
    ta, tb = TA, TB
    na, nb = L // ta, L // tb
    NF, NA = F // 128, P // 128
    DH = D // 2
    KP = pl.cdiv(DH, 128) * 128
    outT = pl.pallas_call(
        _kernel,
        in_specs=[pl.BlockSpec(memory_space=pl.ANY)] * 13,
        out_specs=pl.BlockSpec(memory_space=pl.ANY),
        out_shape=jax.ShapeDtypeStruct((D, L), F32),
        scratch_shapes=[
            pltpu.VMEM((na, D, ta), BF16),
            pltpu.VMEM((nb, D, tb), F32),
            pltpu.VMEM((nb, 2 * NA + 2, tb + 8, 128), F32),
            pltpu.VMEM((na, D, ta), F32),
            pltpu.VMEM((D // 128, 512, 128), BF16),
            pltpu.VMEM((512, D % 128), BF16),
            pltpu.VMEM((D // 128, 2 * P - 512, 128), BF16),
            pltpu.VMEM((2 * P - 512, D % 128), BF16),
            pltpu.VMEM((2 * NA, D, 128), BF16),
            pltpu.VMEM((2, D, P % 128), BF16),
            pltpu.VMEM((7 * DH // 2, NA * 128), U32),
            pltpu.VMEM((NF, DH + KP, 128), BF16),
            pltpu.VMEM((NF, D, 128), BF16),
            pltpu.VMEM((5 * KP // 2, F // 2), U32),
            pltpu.VMEM((5 * DH // 2, F // 2), U32),
            pltpu.VMEM((8, 8, (2 * NA + 2) * 128), F32),
            pltpu.VMEM((8, (2 * NA + 2) * 128), F32),
            pltpu.VMEM((2, D, 128), F32),
            pltpu.VMEM((8, P), F32),
            pltpu.VMEM((D // 2, 256), U32),
            pltpu.VMEM((2 * NA + 1, tb + 8, 128), F32),
            pltpu.VMEM((tb, F), F32),
            pltpu.VMEM((D, tb), F32),
            pltpu.VMEM((5 * (NA + 1) * 64, 256), U32),
            pltpu.VMEM((5, ta // 4, 256), U32),
            pltpu.VMEM((2, ta // 2, (NA + 1) * 128), F32),
            pltpu.VMEM((16, tb), F32),
            pltpu.VMEM((8, 128), jnp.int32),
            pltpu.VMEM((8, 128), jnp.int32),
            pltpu.VMEM((P,), BF16), pltpu.VMEM((P,), BF16), pltpu.VMEM((P,), BF16),
            pltpu.VMEM((D,), BF16), pltpu.VMEM((F,), BF16), pltpu.VMEM((D,), BF16),
            pltpu.SemaphoreType.DMA((na,)),
            pltpu.SemaphoreType.DMA(()),
            pltpu.SemaphoreType.DMA((5,)),
        ],
        compiler_params=pltpu.CompilerParams(
            vmem_limit_bytes=100 * 1024 * 1024,
            disable_semaphore_checks=True, disable_bounds_checks=True),
    )(A_x.reshape(L, D).T, A_Lambda_re, A_Lambda_im, A_B_re, A_B_im, A_C_re, A_C_im,
      A_log_dt, A_Dskip, B_w1, B_b1, B_w2.T, B_b2)
    return outT.T.reshape(Bsz, L, D)
```

```python
import jax
import jax.numpy as jnp
import jax.experimental.pallas as pl
import jax.experimental.pallas.tpu as pltpu

F32 = jnp.float32
BF16 = jnp.bfloat16
U32 = jnp.uint32
NT = (((1,), (1,)), ((), ()))
EPS = 1e-5
GELU_S = (0.7978845608028654 * 0.044715) ** (1.0 / 3.0)
GELU_K = 0.7978845608028654 / GELU_S

TA = 256
TB = 512

EVB0 = (0, 1, 2, 4, 5, 6, 8, 9)
EVB = (6, 5, 6, 10, 13, 7, 10, 11)
LNG = ((0, 9, 16), (0, 8, 19))
LNGL = ((0, 4, 7), (0, 4, 5))
EVS = (61, 62, 63, 64, 65, 66, 67, 68, 69, 70, 71, 72, 73, 74, 75, 76, 77, 78, 79, 80, 81, 82, 83, 84, 85, 86,
       87, 88, 89, 90, 91, 92, 93, 94, 95)
CPK = (2, 5, 6, 10, 11, 15, 16, 18, 20, 22, 23, 33, 36, 37)
GS0 = 8
STG = (1, 5, 6, 7)
TEV = (29, 31, 34, 35, 36, 38, 39, 40, 42, 46, 52, 54, 58, 62, 66, 70, 74, 79, 82, 86, 90, 94, 98, 102, 108,
       113, 114, 118, 121, 126, 130, 137, 138, 139, 146, 150, 154, 158, 162, 166, 169, 174, 177, 182, 186,
       192, 193, 196, 199)
GS = 0

RHS_SUMS = ((-1, (1, 0), (0, 0)), (-1, (0, 1), (1, 1)), (1, (0, 0), (1, 1)), (1, (1, 0), (1, 1)), (1, (0, 0), (0, 1)))
LHS_SUMS = ((1, (1, 0), (1, 1)), (1, (0, 0), (0, 1)), (1, (0, 0), (1, 1)), (-1, (0, 1), (1, 1)), (-1, (1, 0), (0, 0)))


def _cmul(ar, ai, br, bi):
    return ar * br - ai * bi, ar * bi + ai * br


def _row(ref):
    return ref[...].astype(F32).reshape(1, ref.shape[0])


def _rep(c, w):
    return c if w == 128 else jnp.concatenate([c] * (w // 128), axis=1)


def _dot_nt(a, b):
    return jax.lax.dot_general(a, b, NT, preferred_element_type=F32)


def _unpack(w):
    return pltpu.bitcast(w, BF16).astype(F32)


def _pack(x):
    return pltpu.bitcast(x.astype(BF16), U32)


def _comb(sign, a, b):
    return a + b if sign > 0 else a - b


def _heads(m, rows=(0,)):
    return [m[r:r + 8, k * 128:(k + 1) * 128] for k in range(m.shape[1] // 128) for r in rows]


def _kernel(x_hbm, lre_hbm, lim_hbm, bre_hbm, bim_hbm, cre_hbm, cim_hbm, ldt_hbm, dsk_hbm,
            w1_hbm, b1_hbm, w2_hbm, b2_hbm, o_hbm,
            x_s, o_s, bu_s, xn_s, bw0_s, bt0_s, bw1_s, bt1_s, c_s, ct_s, cw_s, w1_s, w2_s, w1x_s, w2x_s,
            lam_s, carry_s, col_s, coef_s, cm_s, h_s, a_s, s_s, bx_s, lx_s, m_s, st_s, bias_s, zero_s, zsrc_s,
            lre_s, lim_s, ldt_s, dsk_s, b1_s, b2_s,
            xsem, osem, wsem):
    ta, tb = TA, TB
    na, D, _ = x_s.shape
    nb = o_s.shape[0]
    P = lre_s.shape[0]
    R = tb // ta
    NF = w1_s.shape[0]
    NFH = NF // 2
    FH = NFH * 128
    NK = D // 128
    DP = pl.cdiv(D, 128) * 128
    DH = D // 2
    KA = 256
    H = tb // 2
    HA = ta // 2
    Q = tb // 8 + 1
    QL = tb - 7 * Q
    NA = P // 128
    PA = NA * 128
    PB = P - PA
    NB = 2 * NA + 1
    W = (NB + 1) * 128
    E = 256

    def x_copy(j):
        return pltpu.make_async_copy(x_hbm.at[:, pl.ds(j * ta, ta)], x_s.at[j], xsem.at[j])

    def o_copy(j, lo=0, hi=tb, r0=0, r1=D):
        return pltpu.make_async_copy(o_s.at[j, r0:r1, lo:hi],
                                     o_hbm.at[r0:r1, pl.ds(j * tb + lo, hi - lo)], osem)

    b_bufs = ((bw0_s, bt0_s), (bw1_s, bt1_s))
    b_parts = ((0, E, 0, 0), (E, PA - E, 1, 0), (PA, E, 0, E), (PA + E, PA - E, 1, P - E),
               (2 * PA, PB, 1, PA - E), (2 * PA + PB, PB, 1, P - E + PA - E))

    def b_copies(g):
        r0, r1 = ((0, E), (E, P))[g]
        bw, bt = b_bufs[g]
        cs = []
        for i, src in enumerate((bre_hbm, bim_hbm)):
            ds = slice(i * (r1 - r0), (i + 1) * (r1 - r0))
            cs += [pltpu.make_async_copy(src.at[r0:r1, k * 128:(k + 1) * 128], bw.at[k, ds, :], wsem.at[g])
                   for k in range(NK)]
            cs += [pltpu.make_async_copy(src.at[r0:r1, NK * 128:D], bt.at[ds, :], wsem.at[g])]
        return cs

    vec_copies = [pltpu.make_async_copy(src, dst, wsem.at[3]) for src, dst in
                  ((lre_hbm, lre_s), (lim_hbm, lim_s), (ldt_hbm, ldt_s), (dsk_hbm, dsk_s),
                   (b1_hbm, b1_s), (b2_hbm, b2_s))]
    z_copy = pltpu.make_async_copy(zsrc_s, zero_s, wsem.at[3])
    b0_copies = b_copies(0)
    b1_copies = b_copies(1)
    w1_copies = [pltpu.make_async_copy(w1_hbm.at[:, k * 128:(k + 1) * 128], w1_s.at[k], wsem.at[4])
                 for k in range(NF)]
    w2_copies = [pltpu.make_async_copy(w2_hbm.at[:, k * 128:(k + 1) * 128], w2_s.at[k], wsem.at[2])
                 for k in range(NF)]
    c_copies = [pltpu.make_async_copy(src.at[:, k * 128:(k + 1) * 128], c_s.at[i * NA + k], wsem.at[2])
                for i, src in enumerate((cre_hbm, cim_hbm)) for k in range(NA)]
    c_copies += [pltpu.make_async_copy(src.at[:, PA:P], ct_s.at[i], wsem.at[2])
                 for i, src in enumerate((cre_hbm, cim_hbm))]

    def gate(val, dep):
        if dep is None:
            return val
        n = val.shape[1]
        w = pl.cdiv(n, 128) * 128
        head = jnp.where(_rep(zero_s[...], w)[:, :n] != 0, _rep(dep, w)[:, :n], val[0:8, :])
        return head if val.shape[0] == 8 else jnp.concatenate([head, val[8:, :]], axis=0)

    def gate_row(val, dep):
        if dep is None:
            return val
        w = val.shape[1]
        return jnp.where(_rep(zero_s[0:1, :], w) != 0, _rep(dep[0:1, :], w), val)

    def gate_all(val, dep):
        n, w = val.shape[0] // 8, pl.cdiv(val.shape[1], 128) * 128
        z = jnp.concatenate([_rep(zero_s[...], w)] * n, axis=0)[:, :val.shape[1]]
        d = jnp.concatenate([_rep(pltpu.bitcast(dep, val.dtype), w)] * n, axis=0)[:, :val.shape[1]]
        return jnp.where(z != 0, d, val)

    def b_words(r0, r1, k0, k1):
        rows = []
        for s0, n, g, d0 in b_parts:
            lo, hi = max(r0, s0), min(r1, s0 + n)
            if lo < hi:
                bw, bt = b_bufs[g]
                rs = slice((d0 + lo - s0) // 2, (d0 + hi - s0) // 2)
                rows.append(jnp.concatenate(
                    [bw.bitcast(U32)[k, rs, :] if k < NK else bt.bitcast(U32)[rs, :] for k in range(k0, k1)],
                    axis=1))
        return rows[0] if len(rows) == 1 else jnp.concatenate(rows, axis=0)

    def wblk(ref, half, r0, r1):
        r32 = ref.bitcast(U32)
        return pltpu.bitcast(
            jnp.concatenate([r32[half * NFH + k, r0 // 2:r1 // 2, :] for k in range(NFH)], axis=1), BF16)

    def xblk(ref, n, i, r0=0, r1=None):
        rows = ref.shape[0] // n
        r1 = 2 * rows if r1 is None else r1
        return pltpu.bitcast(ref[i * rows + r0 // 2:i * rows + r1 // 2, :], BF16)

    def tiles(ref, j, lo, hi):
        parts = []
        for r in range(R):
            a, b = max(lo, r * ta), min(hi, (r + 1) * ta)
            if a < b:
                parts.append(ref[j * R + r, :, a - r * ta:b - r * ta])
        return parts[0] if len(parts) == 1 else jnp.concatenate(parts, axis=1)

    def prep_params():
        lr = _row(lre_s)
        li = _row(lim_s)
        dt = jnp.exp(_row(ldt_s)).astype(BF16).astype(F32)
        mag = jnp.exp(dt * lr)
        ang = dt * li
        lbr = mag * jnp.cos(ang)
        lbi = mag * jnp.sin(ang)
        nr = lbr - 1.0
        den = lr * lr + li * li
        coef_s[...] = jnp.zeros_like(coef_s)
        coef_s[0:1, :] = 2.0 * (nr * lr + lbi * li) / den
        coef_s[1:2, :] = 2.0 * (lbi * lr - nr * li) / den

        def put_lam(k, re, im):
            a = jnp.concatenate([re[:, :PA], re[:, :PA], re[:, PA:], re[:, PA:], re[:, PA:], re[:, PA:]], axis=1)
            b = jnp.concatenate([-im[:, :PA], im[:, :PA], -im[:, PA:], im[:, PA:], im[:, PA:], -im[:, PA:]], axis=1)
            lam_s[2 * k] = jnp.broadcast_to(a, (8, W))
            lam_s[2 * k + 1] = jnp.broadcast_to(b, (8, W))

        put_lam(0, lbr, lbi)
        pr, pi = lbr, lbi
        q = 1
        while q < Q - 1:
            pr, pi = _cmul(pr, pi, pr, pi)
            q *= 2
        assert q == Q - 1
        pr, pi = _cmul(pr, pi, lbr, lbi)
        for k in range(3):
            put_lam(1 + k, pr, pi)
            pr, pi = _cmul(pr, pi, pr, pi)
        carry_s[...] = jnp.zeros_like(carry_s)

    def prep_tables():
        bu_s[:, 0:NB, tb:, :] = jnp.zeros((nb, NB, 8, 128), F32)
        bias_s[...] = jnp.broadcast_to(_row(b1_s) * GELU_S, bias_s.shape)
        for k, r in enumerate((_row(dsk_s), 0.5 * _row(b2_s))):
            r = jnp.concatenate([r, jnp.zeros((1, DP - D), F32)], axis=1)
            col_s[k] = jnp.broadcast_to(r, (128, DP)).T[:D, :]

    def prep_b(q0, deps):
        rows = 32
        low = jax.lax.broadcasted_iota(jnp.int32, (rows, 128), 1) < 64
        zero = jnp.zeros((rows, 128), F32)

        def load(r0, dep):
            w = _unpack(gate_all(b_words(r0, r0 + rows, 0, NK + 1), dep))
            tail = jnp.concatenate([w[:, NK * 128:], jnp.zeros((rows, 64), F32)], axis=1)
            return w[:, 0:128], w[:, 128:256], w[:, 256:384], tail

        for q, dep in enumerate(deps):
            r0 = (q0 + q) * rows
            if r0 < PA:
                r0_, r1_, r2_, r3_ = load(r0, dep)
                i0_, i1_, i2_, i3_ = load(PA + r0, dep)
                outs = {0: jnp.where(low, r3_, i2_), 2: r1_ - r0_, 3: i0_ - i1_,
                        4: jnp.where(low, r2_, r2_ + i2_), 5: jnp.where(low, i2_, pltpu.roll(r3_ + i3_, 64, 1)),
                        6: r0_ + i1_, 7: r1_ + i1_, 8: r0_ + i0_}
            else:
                m0_, m1_, m2_, m3_ = load(PA + r0, dep)
                outs = {0: m3_, 1: jnp.where(low, zero, m2_), 2: m1_ - m0_, 3: m0_ - m1_,
                        4: m2_, 5: jnp.where(low, m2_, pltpu.roll(m3_, 64, 1))}
            for i, o in outs.items():
                bx_s[r0 // 2:(r0 + rows) // 2, i * 128:(i + 1) * 128] = _pack(o)

    def prep_w2(deps):
        src32 = w2_s.bitcast(U32)
        per = len(deps) // NFH
        rows = DH // 2 // per
        z = jnp.concatenate([zero_s[...]] * (rows // 8), axis=0) != 0
        for n, dep in enumerate(deps):
            k, q = divmod(n, per)
            d = jnp.concatenate([pltpu.bitcast(dep, U32)] * (rows // 8), axis=0)
            blk = {}
            for r in range(2):
                for c in range(2):
                    r0 = r * DH // 2 + q * rows
                    blk[r, c] = _unpack(jnp.where(z, d, src32[c * NFH + k, r0:r0 + rows, :]))
            for i, (sign, a, b) in enumerate(LHS_SUMS):
                r0 = i * DH // 2 + q * rows
                w2x_s[r0:r0 + rows, k * 128:(k + 1) * 128] = _pack(_comb(sign, blk[a], blk[b]))

    def prep_w1(deps):
        src32 = w1_s.bitcast(U32)
        z = jnp.concatenate([zero_s[...]] * 2, axis=0) != 0
        for n, dep in enumerate(deps):
            k, q = divmod(n, 5)
            cs = slice(k * 128, (k + 1) * 128)
            d = jnp.concatenate([pltpu.bitcast(dep, U32)] * 2, axis=0)
            ld = lambda c, r0: _unpack(jnp.where(z, d, src32[c * NFH + k, r0:r0 + 16, :]))
            if q < 4:
                blk = {(r, c): ld(c, r * 64 + q * 16) for r in range(2) for c in range(2)}
                for i, (sign, a, b) in enumerate(RHS_SUMS):
                    w1x_s[i * 64 + q * 16:i * 64 + (q + 1) * 16, cs] = _pack(_comb(sign, blk[a], blk[b]))
            else:
                for i, r0 in enumerate((KA // 2, KA // 2 + 16, KA // 2 + 64, KA // 2 + 80)):
                    w1x_s[320 + i * 16:336 + i * 16, cs] = _pack(ld(0, r0) + ld(1, r0))

    def prep_c(deps):
        rows = DH // 2 // len(deps)
        for q, dep in enumerate(deps):
            cf = gate(coef_s[...], dep)
            cr = cf[0:1, :]
            ci = cf[1:2, :]
            blk = {}
            for r in range(2):
                rs = slice(r * DH // 2 + q * rows, r * DH // 2 + (q + 1) * rows)
                ld = lambda i: jnp.concatenate(
                    [c_s.bitcast(U32)[i * NA + k, rs, :] for k in range(NA)] + [ct_s.bitcast(U32)[i, rs, :]],
                    axis=1)
                c_re = _unpack(ld(0))
                c_im = _unpack(ld(1))
                cpr = c_re * cr - c_im * ci
                cpi = -(c_re * ci) - c_im * cr
                blk[r, 0], blk[r, 1] = cpr[:, :PA], cpi[:, :PA]
                cm_s[rs, 0:128] = _pack(jnp.concatenate([cpr[:, PA:], cpi[:, PA:]], axis=1))
            outs = [_comb(sign, blk[a], blk[b]) for sign, a, b in LHS_SUMS] + [blk[1, 1], blk[0, 0]]
            for i, o in enumerate(outs):
                cw_s[i * DH // 2 + q * rows:i * DH // 2 + (q + 1) * rows, :] = _pack(o)

    def ln1(j, lo, hi, deps=(None, None, None)):
        x = gate(x_s[j, :, lo:hi].astype(F32), deps[0])
        m = gate_row(jnp.sum(x, axis=0, keepdims=True) * (1.0 / D), deps[1])
        xc = x - m
        v = jnp.sum(xc * xc, axis=0, keepdims=True) * (1.0 / D)
        xb = (xc * gate_row(jax.lax.rsqrt(v + EPS), deps[2])).astype(BF16)
        xn = xb.astype(F32)
        xn_s[j, :, lo:hi] = xn
        return xb, xn

    def bu_plain(xn, ks):
        rhs = pltpu.bitcast(
            jnp.concatenate([b_words(k * 128, (k + 1) * 128, 0, NK + 1) for k in ks], axis=0), BF16)
        bu = _dot_nt(xn, rhs)
        for i, k in enumerate(ks):
            bu_s[0, k, 0:ta, :] = bu[:, i * 128:(i + 1) * 128]
        return bu

    def bu_operands(xn):
        a11, a12, a21, a22 = xn[:128, :HA], xn[128:KA, :HA], xn[:128, HA:], xn[128:KA, HA:]
        p1, p2, p3 = [xn[KA + 64 * k:KA + 64 * (k + 1), :HA] for k in range(3)]
        q1, q2, q3 = [xn[KA + 64 * k:KA + 64 * (k + 1), HA:] for k in range(3)]
        ops = ([a22], [q1, q2], [a21 + a22, q3, -q2],
               [a11], [p1, p3], [a11 + a12, -p3, p2], [a11 + a22], [a12 - a22, p1, p2], [a21 - a11, q1, q3])
        return [jnp.concatenate(o, axis=0).astype(BF16).T for o in ops]

    def bx(n, *cols):
        return jnp.concatenate([bx_s[n * 64:(n + 1) * 64, c * 128:(c + 1) * 128] for c in cols], axis=1)

    def bu_mm(l, *words):
        return _dot_nt(l, pltpu.bitcast(jnp.concatenate(words, axis=1), BF16))

    def bu_put(base, off, half, k, val):
        bu_s[base + off // R, k, pl.ds((off % R) * ta + half * HA, HA), :] = val

    def bu_lo(base, off, ls):
        m2, m4, res = [], [], []
        for n in (NA, 0, 1, 2):
            r0 = 2 * PA if n == NA else n * 128
            p4 = bu_mm(ls[0], bx(n, 2))
            g = bu_mm(ls[1], bx(n, 4))
            p2 = bu_mm(ls[2], b_words(r0, r0 + 128, 0, 1), bx(n, 0))
            bu_put(base, off, 1, NB - 1 if n == NA else n, p2 + g + p4)
            res += [p4, p2]
            if n < NA:
                m2.append(p2)
                m4.append(p4)
        return res, m4, m2

    def bu_hi(base, off, m4, m2, ls):
        m3, m5, res = [], [], []
        for n in (NA, 0, 1, 2):
            r0 = 2 * PA if n == NA else PA + n * 128
            p3 = bu_mm(ls[0], bx(n, 3))
            g = bu_mm(ls[1], bx(n, 5))
            p5 = bu_mm(ls[2], b_words(r0, r0 + 128, 1, 2), bx(n, 1 if n == NA else 0))
            bu_put(base, off, 0, NB - 1 if n == NA else NA + n, p5 + g + p3)
            res += [p3, p5]
            if n < NA:
                m3.append(p3)
                m5.append(p5)
        for n in range(NA):
            m1 = bu_mm(ls[3], bx(n, 6))
            p7 = bu_mm(ls[4], bx(n, 7, 4))
            bu_put(base, off, 0, n, p7 + m1 + m4[n] - m5[n])
            p6 = bu_mm(ls[5], bx(n, 8, 5))
            bu_put(base, off, 1, NA + n, p6 + m1 - m2[n] + m3[n])
            res += [m1, p7, p6]
        return res

    LX = (0, 128, 256, 512, 640, 896, 1152)

    def stash(m4, m2, ls):
        for n in range(NA):
            m_s[n] = m4[n]
            m_s[NA + n] = m2[n]
        for i in range(6):
            lx_s[:, LX[i]:LX[i + 1]] = pltpu.bitcast(ls[3 + i], U32)

    def finish(base, off):
        return bu_hi(base, off, [m_s[n] for n in range(NA)], [m_s[NA + n] for n in range(NA)],
                     [pltpu.bitcast(lx_s[:, LX[i]:LX[i + 1]], BF16) for i in range(6)])

    def phase_a_pair(base, lng):
        j = base * R + 1
        res = finish(base, 1)
        ls = bu_operands(ln1(j + 1, 0, ta)[1])
        cur, m4, m2 = bu_lo(base, 2, ls)
        cur += bu_hi(base, 2, m4, m2, ls[3:])
        ev = [e for m in cur for e in _heads(m)]
        xn = jnp.concatenate([ln1(j + 2, k * 128, (k + 1) * 128, [ev[g] for g in lng[k]])[1]
                              for k in range(ta // 128)], axis=1)
        ls = bu_operands(xn)
        nxt, m4, m2 = bu_lo(base, 3, ls)
        stash(m4, m2, ls)
        return res + cur + nxt

    def ln2_stats(j, deps):
        for k in range(tb // 128):
            xs = gate(tiles(xn_s, j, k * 128, (k + 1) * 128), deps[k])
            m = jnp.sum(xs, axis=0, keepdims=True) * (1.0 / D)
            v = jnp.sum(xs * xs, axis=0, keepdims=True) * (1.0 / D) - m * m
            r = jax.lax.rsqrt(v + EPS) * GELU_S
            st_s[0:8, k * 128:(k + 1) * 128] = jnp.broadcast_to(r, (8, 128))
            st_s[8:16, k * 128:(k + 1) * 128] = jnp.broadcast_to(m * r, (8, 128))

    def mlp_up(j):
        st = st_s[...]
        yT = tiles(xn_s, j, 0, tb) * st[0:1, :] - st[8:9, :]
        a11, a12, a21, a22 = yT[:128, :H], yT[128:KA, :H], yT[:128, H:], yT[128:KA, H:]
        p1, p2, p3 = [yT[KA + 64 * k:KA + 64 * (k + 1), :H] for k in range(3)]
        q1, q2, q3 = [yT[KA + 64 * k:KA + 64 * (k + 1), H:] for k in range(3)]
        raw = lambda half, r0, r1: wblk(w1_s, half, r0, r1)
        pre = lambda r0, r1: pltpu.bitcast(w1x_s[r0 // 2:r1 // 2, :], BF16)
        b31, b12 = raw(0, KA + 128, D), raw(1, KA, KA + 64)
        g1 = [pre(640, 704), raw(0, KA + 64, KA + 128)]
        g2 = [raw(1, KA + 64, KA + 128), pre(704, 768)]

        lhs = lambda *parts: jnp.concatenate(parts, axis=0).astype(BF16).T
        rhs = lambda *parts: jnp.concatenate(parts, axis=0)
        mm = lambda l, r, n: jnp.dot(l, r[:, n * 128:(n + 1) * 128], preferred_element_type=F32)

        def act(r, c, n, x):
            cs = slice(c * FH + n * 128, c * FH + (n + 1) * 128)
            x = x + bias_s[0:1, cs]
            t = jnp.tanh(x * (x * x + GELU_K))
            a_s[r * H:(r + 1) * H, cs] = x + x * t

        ev, m2, m3, m4, m5 = [], [], [], [], []
        l4, ln, l2 = lhs(a22), lhs(q1, q2), lhs(a21 + a22, q3, -q1)
        for n in range(NFH):
            m4.append(mm(l4, pre(0, 128), n))
            g = mm(ln, rhs(*g1), n)
            m2.append(mm(l2, rhs(raw(0, 0, 128), b31, b12), n))
            act(1, 0, n, m2[n] + g + m4[n])
            ev += _heads(m2[n], (0, 128))
        l3, ln, l5 = lhs(a11), lhs(p2, p3), lhs(a11 + a12, -p3, p1)
        for n in range(NFH):
            m3.append(mm(l3, pre(128, 256), n))
            g = mm(ln, rhs(*g2), n)
            m5.append(mm(l5, rhs(raw(1, 128, KA), b31, b12), n))
            act(0, 1, n, m5[n] + g + m3[n])
            ev += _heads(m5[n], (0, 128))
        l1, l7, l6 = lhs(a11 + a22), lhs(a12 - a22, p1, p2), lhs(a21 - a11, q2, q3)
        for n in range(NFH):
            m1 = mm(l1, pre(256, 384), n)
            act(0, 0, n, mm(l7, rhs(pre(384, 512), *g1), n) + m1 + m4[n] - m5[n])
            act(1, 1, n, mm(l6, rhs(pre(512, 640), *g2), n) + m1 - m2[n] + m3[n])
            ev += _heads(m1, (0, 128))
        return ev

    def scan(j, dep):
        row = jax.lax.broadcasted_iota(jnp.int32, (8, 128), 0)
        for ka, kb in [(k, NA + k) for k in range(NA)] + [(NB - 1, NB)]:
            sa = slice(ka * 128, (ka + 1) * 128)
            sb = slice(kb * 128, (kb + 1) * 128)
            la = lam_s[0, :, sa]
            lba = lam_s[1, :, sa]
            lbb = lam_s[1, :, sb]
            ca = gate(carry_s[:, sa], dep)
            cb = carry_s[:, sb]

            def step(u, v, i):
                bu = bu_s[j, ka, pl.ds(i, 8, stride=Q), :]
                bv = bu_s[j, kb, pl.ds(i, 8, stride=Q), :] if kb < NB else pltpu.roll(bu, PB, 1)
                return (la * u + bu) + lba * v, (la * v + bv) + lbb * u

            u, v = ca, cb
            for i in range(Q):
                u, v = step(u, v, i)
            for k in range(3):
                sh = 1 << k
                us = jnp.where(row >= sh, pltpu.roll(u, sh, 0), 0.0)
                vs = jnp.where(row >= sh, pltpu.roll(v, sh, 0), 0.0)
                pa = lam_s[2 + 2 * k, :, sa]
                u, v = (u + pa * us + lam_s[3 + 2 * k, :, sa] * vs,
                        v + pa * vs + lam_s[3 + 2 * k, :, sb] * us)
            u = jnp.where(row == 0, ca, pltpu.roll(u, 1, 0))
            v = jnp.where(row == 0, cb, pltpu.roll(v, 1, 0))
            for i in range(Q):
                u, v = step(u, v, i)
                if i == QL - 1:
                    carry_s[:, sa] = jnp.where(row == 0, pltpu.roll(u, 1, 0), 0.0)
                    carry_s[:, sb] = jnp.where(row == 0, pltpu.roll(v, 1, 0), 0.0)
                h_s[ka, pl.ds(i, 8, stride=Q), :] = u
                if kb < NB:
                    h_s[kb, pl.ds(i, 8, stride=Q), :] = v
            dep = u

    def ssm_out(j, split=False):
        g = lambda r, c: jnp.concatenate([h_s[c * NA + k, r * H:(r + 1) * H, :] for k in range(NA)], axis=1)
        parts = []

        def mm(i, rhs):
            lhs = xblk(cw_s, 7, i)
            if not split:
                return _dot_nt(lhs, rhs.astype(BF16))
            cols = []
            for n in range(H // 128):
                acc = None
                for k in range(NA):
                    p = _dot_nt(lhs[:, k * 128:(k + 1) * 128],
                                rhs[n * 128:(n + 1) * 128, k * 128:(k + 1) * 128].astype(BF16))
                    parts.append(p)
                    acc = p if acc is None else acc + p
                cols.append(acc)
            return jnp.concatenate(cols, axis=1)

        z = _dot_nt(pltpu.bitcast(cm_s[:, 0:128], BF16), h_s[NB - 1, :tb, :].astype(BF16))
        z = z + tiles(xn_s, j, 0, tb) * _rep(col_s[0], tb)
        n2 = mm(0, g(0, 0))
        n4 = mm(5, g(0, 1) - g(0, 0))
        s_s[DH:, :H] = z[DH:, :H] + (n2 + n4)
        n5 = mm(1, g(1, 1))
        n3 = mm(6, g(1, 0) - g(1, 1))
        s_s[:DH, H:] = z[:DH, H:] + (n3 + n5)
        n1 = mm(2, g(0, 0) + g(1, 1))
        u = z[:DH, :H] + n1 + n4 - n5
        v = z[DH:, H:] + n1 - n2 + n3
        s_s[:DH, :H] = u + mm(3, g(0, 1) + g(1, 1))
        s_s[DH:, H:] = v + mm(4, g(0, 0) + g(1, 0))
        return parts

    last_pieces = ((0, 0, DH), (128, 0, 128), (128, 128, DH))

    def mlp_down(j, last=False):
        g = lambda r, c: a_s[r * H:(r + 1) * H, c * FH:(c + 1) * FH]
        mm = lambda lhs, rhs: _dot_nt(lhs, rhs.astype(BF16))

        def fin(r0, lo, oT):
            r1, hi = r0 + oT.shape[0], lo + oT.shape[1]
            h = oT * (0.25 / GELU_S) + _rep(col_s[1, r0:r1, :], hi - lo)
            gt = h + h * jnp.tanh(h)
            o_s[j, r0:r1, lo:hi] = tiles(x_s, j, lo, hi)[r0:r1].astype(F32) + s_s[r0:r1, lo:hi] * gt
            if last:
                o_copy(j, lo, hi, r0, r1).start()

        n2 = mm(xblk(w2x_s, 5, 0), g(0, 0))
        n4 = mm(wblk(w2_s, 1, DH, D), g(0, 1) - g(0, 0))
        fin(DH, 0, n2 + n4)
        n5 = mm(xblk(w2x_s, 5, 1), g(1, 1))
        n3 = mm(wblk(w2_s, 0, 0, DH), g(1, 0) - g(1, 1))
        fin(0, H, n3 + n5)
        n1 = mm(xblk(w2x_s, 5, 2), g(0, 0) + g(1, 1))
        u = n1 + n4 - n5
        v = n1 - n2 + n3
        n7 = mm(xblk(w2x_s, 5, 3), g(0, 1) + g(1, 1))
        fin(0, 0, u + n7)
        s6 = g(0, 0) + g(1, 0)
        if not last:
            fin(DH, H, v + mm(xblk(w2x_s, 5, 4), s6))
        else:
            for lo, r0, r1 in last_pieces:
                fin(DH + r0, H + lo, v[r0:r1, lo:lo + 128] + mm(xblk(w2x_s, 5, 4, r0, r1), s6[lo:lo + 128, :]))
        return [e for n in (n2, n4, n5, n3, n1, n7) for e in _heads(n)]

    for c in vec_copies:
        c.start()
    x_copy(0).start()
    for c in b0_copies:
        c.start(priority=1)
    zsrc_s[...] = jnp.zeros_like(zsrc_s)
    z_copy.start()
    for c in vec_copies + [z_copy]:
        c.wait()
    for c in b1_copies:
        c.start(priority=1)
    x_copy(1).start(priority=1)
    prep_params()
    x_copy(0).wait()
    xn0 = ln1(0, 0, ta)[0].T
    for c in b0_copies:
        c.wait()
    for j in range(2, na):
        x_copy(j).start(priority=1)
    ev = _heads(bu_plain(xn0, (0, 1, NA, NA + 1)), (0, 64, 128, 192))
    prep_b(0, [ev[k] for k in EVB0])
    prep_tables()
    for c in b1_copies:
        c.wait()
    x_copy(1).wait()
    for c in w1_copies + c_copies + w2_copies:
        c.start(priority=1)
    bu0 = bu_plain(xn0, (2, NA + 2, NB - 1))
    ls = bu_operands(ln1(1, 0, ta)[1])
    ev = _heads(bu0, (0, 32, 64, 96, 128, 160, 192, 224))
    prep_b(E // 32, [ev[k] for k in EVB])
    stash(*bu_lo(0, 1, ls)[1:], ls)

    def body_a(i, carry):
        x_copy(2 * i + 2).wait()
        x_copy(2 * i + 3).wait()
        phase_a_pair(i, LNG)
        return carry

    jax.lax.fori_loop(0, nb - 2, body_a, 0)

    x_copy(na - 2).wait()
    x_copy(na - 1).wait()
    for c in w1_copies:
        c.wait()
    ev = [e for m in phase_a_pair(nb - 2, LNGL) for e in _heads(m, (0, 64))]
    prep_w1([ev[k] for k in EVS])

    for c in c_copies + w2_copies:
        c.wait()
    finish(0, na - 1)
    ln2_stats(0, [None] * (tb // 128))
    ev = mlp_up(0)
    prep_c([ev[k] for k in CPK])
    scan(0, ev[GS0])
    parts = ssm_out(0, split=True)
    ev += [e for p in parts for e in _heads(p, (0, 56, 112, 168))]
    prep_w2([ev[k] for k in TEV])

    def body_b(j, carry):
        ev = mlp_down(j)
        ln2_stats(j + 1, [ev[k] for k in STG])
        mlp_up(j + 1)
        scan(j + 1, ev[GS])
        ssm_out(j + 1)
        o_copy(j).start()
        return carry

    jax.lax.fori_loop(0, nb - 1, body_b, 0)

    mlp_down(nb - 1, last=True)
    for j in range(nb - 1):
        o_copy(j).wait()
    for lo, hi, r0, r1 in ((0, H, DH, D), (H, tb, 0, DH), (0, H, 0, DH)):
        o_copy(nb - 1, lo, hi, r0, r1).wait()
    for lo, r0, r1 in last_pieces:
        o_copy(nb - 1, H + lo, H + lo + 128, DH + r0, DH + r1).wait()


@jax.jit
def pallas_recurrent_scan__ssm_conv_s5__mixer_channel_mlp__prompt_kernel(
    A_x, A_Lambda_re, A_Lambda_im, A_B_re, A_B_im, A_C_re, A_C_im, A_log_dt, A_Dskip,
    B_x, B_w1, B_b1, B_w2, B_b2,
):
    Bsz, L, D = A_x.shape
    P = A_Lambda_re.shape[0]
    F = B_w1.shape[1]
    assert (Bsz, L, D, P, F) == (1, 2048, 448, 448, 1792)
    ta, tb = TA, TB
    na, nb = L // ta, L // tb
    NF, NA = F // 128, P // 128
    DH = D // 2
    outT = pl.pallas_call(
        _kernel,
        in_specs=[pl.BlockSpec(memory_space=pl.ANY)] * 13,
        out_specs=pl.BlockSpec(memory_space=pl.ANY),
        out_shape=jax.ShapeDtypeStruct((D, L), F32),
        scratch_shapes=[
            pltpu.VMEM((na, D, ta), BF16),
            pltpu.VMEM((nb, D, tb), F32),
            pltpu.VMEM((nb, 2 * NA + 2, tb + 8, 128), F32),
            pltpu.VMEM((na, D, ta), F32),
            pltpu.VMEM((D // 128, 512, 128), BF16),
            pltpu.VMEM((512, D % 128), BF16),
            pltpu.VMEM((D // 128, 2 * P - 512, 128), BF16),
            pltpu.VMEM((2 * P - 512, D % 128), BF16),
            pltpu.VMEM((2 * NA, D, 128), BF16),
            pltpu.VMEM((2, D, P % 128), BF16),
            pltpu.VMEM((7 * DH // 2, NA * 128), U32),
            pltpu.VMEM((NF, D, 128), BF16),
            pltpu.VMEM((NF, D, 128), BF16),
            pltpu.VMEM((384, F // 2), U32),
            pltpu.VMEM((5 * DH // 2, F // 2), U32),
            pltpu.VMEM((8, 8, (2 * NA + 2) * 128), F32),
            pltpu.VMEM((8, (2 * NA + 2) * 128), F32),
            pltpu.VMEM((2, D, 128), F32),
            pltpu.VMEM((8, P), F32),
            pltpu.VMEM((D // 2, 256), U32),
            pltpu.VMEM((2 * NA + 1, tb + 8, 128), F32),
            pltpu.VMEM((tb, F), F32),
            pltpu.VMEM((D, tb), F32),
            pltpu.VMEM(((NA + 1) * 64, 9 * 128), U32),
            pltpu.VMEM((ta // 4, 1152), U32),
            pltpu.VMEM((2 * NA, ta // 2, 128), F32),
            pltpu.VMEM((16, tb), F32),
            pltpu.VMEM((8, F), F32),
            pltpu.VMEM((8, 128), jnp.int32),
            pltpu.VMEM((8, 128), jnp.int32),
            pltpu.VMEM((P,), BF16), pltpu.VMEM((P,), BF16), pltpu.VMEM((P,), BF16),
            pltpu.VMEM((D,), BF16), pltpu.VMEM((F,), BF16), pltpu.VMEM((D,), BF16),
            pltpu.SemaphoreType.DMA((na,)),
            pltpu.SemaphoreType.DMA(()),
            pltpu.SemaphoreType.DMA((5,)),
        ],
        compiler_params=pltpu.CompilerParams(
            vmem_limit_bytes=100 * 1024 * 1024,
            disable_semaphore_checks=True, disable_bounds_checks=True),
    )(A_x.reshape(L, D).T, A_Lambda_re, A_Lambda_im, A_B_re, A_B_im, A_C_re, A_C_im,
      A_log_dt, A_Dskip, B_w1, B_b1, B_w2.T, B_b2)
    return outT.T.reshape(Bsz, L, D)
```
